```python
import jax
import jax.numpy as jnp

def _softmax(x, axis=-1):
    return jax.nn.softmax(x, axis=axis)

def _gelu(x):
    return jax.nn.gelu(x, approximate=True)

def _silu(x):
    return jax.nn.silu(x)

def _sigmoid(x):
    return jax.nn.sigmoid(x)

def _layernorm(x, axis=-1, eps=1e-05):
    m = jnp.mean(x, axis=axis, keepdims=True)
    v = jnp.var(x, axis=axis, keepdims=True)
    return (x - m) / jnp.sqrt(v + eps)

def _scatter_add(tgt, idx, src, axis=0):
    return tgt.at[idx].add(src)

def _segment_sum(src, seg, n):
    return jax.ops.segment_sum(src, seg, n)

class _Rng:

    def __init__(self, key):
        self._k = key

    def _next(self):
        self._k, sub = jax.random.split(self._k)
        return sub

    def normal(self, shape):
        return jax.random.normal(self._next(), shape, dtype=jnp.bfloat16)

    def randint(self, lo, hi, shape):
        return jax.random.randint(self._next(), shape, lo, hi, dtype=jnp.int32)

    def uniform(self, shape, lo=0.0, hi=1.0):
        return jax.random.uniform(self._next(), shape, jnp.bfloat16, lo, hi)

    def permutation(self, n):
        return jax.random.permutation(self._next(), n)
kernel_name = 'adaLN_cond__linear_kernel_hedgehog__moe_arch_mod__prompt'

def setup_inputs():
    _rng = _Rng(jax.random.key(int.from_bytes(__import__("os").urandom(4), "little")))
    _w = lambda a: (lambda t: t.astype(jnp.bfloat16) if jnp.issubdtype(t.dtype, jnp.floating) else t)(jnp.asarray(a))

    def _A_setup():
        B, S, D, H = (1, 2048, 1024, 32)
        Dh = D // H
        return {'x': _w((lambda *s: _rng.normal(s) * 0.05)(B, S, D)), 'wqkv': _w((lambda *s: _rng.normal(s) * 0.05)(D, 3 * D)), 'w_phi': _w((lambda *s: _rng.normal(s) * 0.05)(H, Dh, Dh) * Dh ** (-0.5)), 'wo': _w((lambda *s: _rng.normal(s) * 0.05)(D, D))}
    _A_in = _A_setup()

    def _B_setup():
        B, S, D, F, C = (1, 2048, 1024, 3584, 2)
        return {'x': _w((lambda *s: _rng.normal(s) * 0.05)(B, S, D)), 'w_r': _w((lambda *s: _rng.normal(s) * 0.05)(D)), 'w_gate': _w((lambda *s: _rng.normal(s) * 0.05)(D, F)), 'w_up': _w((lambda *s: _rng.normal(s) * 0.05)(D, F)), 'w_down': _w((lambda *s: _rng.normal(s) * 0.05)(F, D))}
    _B_in = _B_setup()
    return {'A_x': _A_in['x'], 'A_wqkv': _A_in['wqkv'], 'A_w_phi': _A_in['w_phi'], 'A_wo': _A_in['wo'], 'B_x': _B_in['x'], 'B_w_r': _B_in['w_r'], 'B_w_gate': _B_in['w_gate'], 'B_w_up': _B_in['w_up'], 'B_w_down': _B_in['w_down'], 'c': _w((lambda *s: _rng.normal(s) * 0.05)(1, 1024)), 'w_mod': _w((lambda *s: _rng.normal(s) * 0.05)(1024, 6 * 1024) * 1024 ** (-0.5))}

def reference(A_x, A_wqkv, A_w_phi, A_wo, B_x, B_w_r, B_w_gate, B_w_up, B_w_down, c, w_mod):

    def _A_ref(x, wqkv, w_phi, wo):
        B, S, D = x.shape
        H = 32
        Dh = D // H
        qkv = (lambda x, *d: x.transpose(*d))((x @ wqkv).reshape(B, S, 3, H, Dh), 2, 0, 3, 1, 4)
        q, k, v = (qkv[0], qkv[1], qkv[2])
        pq = jnp.einsum('bhsd,hdf->bhsf', q, w_phi)
        pk = jnp.einsum('bhsd,hdf->bhsf', k, w_phi)
        phi_q = jnp.concatenate([_softmax(pq, axis=-1), _softmax(-pq, axis=-1)], axis=-1)
        phi_k = jnp.concatenate([_softmax(pk, axis=-1), _softmax(-pk, axis=-1)], axis=-1)
        kv = jnp.einsum('bhsf,bhsd->bhfd', phi_k, v)
        z = jnp.einsum('bhsf->bhf', phi_k)
        num = jnp.einsum('bhqf,bhfd->bhqd', phi_q, kv)
        den = jnp.einsum('bhqf,bhf->bhq', phi_q, z)[..., None] + 1e-06
        o = num / den
        return (lambda x, *d: x.transpose(*d))(o, 0, 2, 1, 3).reshape(B, S, D) @ wo

    def _B_ref(x, w_r, w_gate, w_up, w_down):
        B, S, D = x.shape
        C = 2
        r = x @ w_r
        idx = jnp.argsort(-r, axis=-1)[:, :C]
        idx_e = jnp.repeat(idx.reshape(B, C, 1), D, axis=2)
        x_sel = jnp.take_along_axis(x, idx_e, axis=1)
        g = _silu(x_sel @ w_gate)
        u = x_sel @ w_up
        y = g * u @ w_down
        r_sel = _sigmoid(jnp.take_along_axis(r, idx, axis=1))
        y = y * r_sel.reshape(B, C, 1)
        b_off = (jnp.arange(B) * S).reshape(B, 1)
        flat_idx = (idx + b_off).reshape(B * C)
        zero = (x * 0.0).reshape(B * S, D)
        upd = _scatter_add(zero, flat_idx, y.reshape(B * C, D), axis=0)
        return x + upd.reshape(B, S, D)
    x = A_x
    mod = (_silu(c) @ w_mod).reshape(c.shape[0], 6, 1, -1)
    sa, ca, ga, sb, cb, gb = (mod[:, 0].copy(), mod[:, 1].copy(), mod[:, 2].copy(), mod[:, 3].copy(), mod[:, 4].copy(), mod[:, 5].copy())
    h = _layernorm(x, axis=-1) * (1 + ca) + sa
    x = x + ga * _A_ref(h, A_wqkv, A_w_phi, A_wo)
    h = _layernorm(x, axis=-1) * (1 + cb) + sb
    x = x + gb * _B_ref(h, B_w_r, B_w_gate, B_w_up, B_w_down)
    return x
```

```python
import math

import jax
import jax.numpy as jnp
from jax import lax
import jax.experimental.pallas as pl
import jax.experimental.pallas.tpu as pltpu

F32 = jnp.float32
BF16 = jnp.bfloat16
U32 = jnp.uint32

HEADS = 32
HEAD_DIM = 32
PAIR = 2 * HEAD_DIM
KV_ROWS = PAIR + 16
LN_EPS = 1e-5
DEN_EPS = 1e-6
LOG2E = math.log2(math.e)

TILE = 256
CHUNK = 256

NT_DIMS = (((1,), (1,)), ((), ()))


def _dot(a, b):
    return jnp.dot(a, b, preferred_element_type=F32)


def _dot_nt(a, b):
    return lax.dot_general(a, b, NT_DIMS, preferred_element_type=F32)


def _pack(v):
    return pltpu.bitcast(v.astype(BF16), U32)


def _unpack(v):
    return pltpu.bitcast(v, BF16)


def _recip(d):
    r = pltpu.reciprocal(d, approx=True)
    return r * (2.0 - d * r)


def _sigmoid(v):
    return 1.0 / (1.0 + jnp.exp(-v))


def _rows(v, n):
    return jnp.concatenate([v] * (n // 8), axis=0) if n > 8 else v


def _layernorm(x):
    inv_d = 1.0 / x.shape[-1]
    xc = x - jnp.sum(x, axis=-1, keepdims=True) * inv_d
    var = jnp.sum(xc * xc, axis=-1, keepdims=True) * inv_d
    return xc * lax.rsqrt(var + LN_EPS)


def _head_reduce(op, tiles):
    while len(tiles) > 1:
        tiles = [op(tiles[i], tiles[i + 1]) for i in range(0, len(tiles), 2)]
    m = tiles[0]
    m = op(m, pltpu.roll(m, 4, 0))
    return op(m, pltpu.roll(m, 2, 0))


def _feature_map(p):
    tiles = [p[8 * j:8 * j + 8] for j in range(PAIR // 8)]
    hi = _head_reduce(jnp.maximum, tiles)
    lo = _head_reduce(jnp.minimum, tiles)
    e_pos = [jnp.exp2(t - hi) for t in tiles]
    e_neg = [jnp.exp2(lo - t) for t in tiles]
    r_pos = _recip(_head_reduce(jnp.add, e_pos))
    r_neg = _recip(_head_reduce(jnp.add, e_neg))
    phi = [e * r_pos for e in e_pos] + [e * r_neg for e in e_neg]
    return jnp.concatenate(phi, axis=0).astype(BF16)


def _kernel(x_hbm, wqkv_hbm, wphi_hbm, wo_hbm, wr_hbm, wg_hbm, wu_hbm, wd_hbm, c_hbm, wmod_hbm,
            out_hbm,
            x_v, wqkv_v, wphi_v, wo_v, wr_v, wg_v, wu_v, wd_v, c_v, wmod_v,
            wqt_v, wkt_v, wvt_v, mod_v, h_v, kv_v, kvm_v, x1_v, out_v, r_v,
            sem, x_sem, out_sem):
    seq, d = x_v.shape
    n_tiles = seq // TILE
    n_pairs = HEADS // 2

    def copy(src, dst, s):
        return pltpu.make_async_copy(src, dst, s)

    def tile_rows(t):
        return pl.ds(pl.multiple_of(t * TILE, TILE), TILE)

    def x_copy(t):
        return copy(x_hbm.at[tile_rows(t)], x_v.at[tile_rows(t)], x_sem.at[t])

    def out_copy(t):
        return copy(out_v.at[tile_rows(t)], out_hbm.at[tile_rows(t)], out_sem.at[t])

    def cols(ref, i, n=1):
        return ref.at[:, pl.ds(i * d, n * d)]

    c_cp = copy(c_hbm, c_v, sem.at[0])
    wphi_cp = copy(wphi_hbm, wphi_v, sem.at[1])
    wr_cp = copy(wr_hbm, wr_v, sem.at[2])
    mod_a_cp = copy(cols(wmod_hbm, 0, 2), cols(wmod_v, 0, 2), sem.at[3])
    mod_b_cp = copy(cols(wmod_hbm, 2, 4), cols(wmod_v, 2, 4), sem.at[4])
    wq_cp = copy(cols(wqkv_hbm, 0), cols(wqkv_v, 0), sem.at[5])
    wk_cp = copy(cols(wqkv_hbm, 1), cols(wqkv_v, 1), sem.at[6])
    wv_cp = copy(cols(wqkv_hbm, 2), cols(wqkv_v, 2), sem.at[7])
    wo_cp = copy(wo_hbm, wo_v, sem.at[8])
    wg_cp = copy(wg_hbm, wg_v, sem.at[9])
    wu_cp = copy(wu_hbm, wu_v, sem.at[10])
    wd_cp = copy(wd_hbm, wd_v, sem.at[11])

    for cp in (c_cp, wphi_cp, wr_cp, wk_cp, wv_cp, x_copy(0), mod_a_cp):
        cp.start()

    def fold(col, dst):
        row = lax.broadcasted_iota(jnp.int32, (128, 128), 0)
        lane = lax.broadcasted_iota(jnp.int32, (128, 128), 1)
        same_head = (2 * (row // PAIR) + row % 2) == lane // HEAD_DIM
        row_f = lax.broadcasted_iota(jnp.int32, (128, HEAD_DIM), 0)
        lane_f = lax.broadcasted_iota(jnp.int32, (128, HEAD_DIM), 1)
        pick = jnp.where((row_f % PAIR) // 2 == lane_f, 1.0, 0.0).astype(BF16)
        for g in range(d // 128):
            wphi = wphi_v[4 * g:4 * g + 4].reshape(128, HEAD_DIM)
            a = jnp.where(same_head, _dot_nt(pick, wphi), 0.0).astype(BF16)
            w = wqkv_v[:, col * d + g * 128:col * d + (g + 1) * 128]
            dst[g * 64:(g + 1) * 64, :] = _pack(_dot_nt(a, w) * LOG2E)

    def modulation(lo, hi):
        cf = c_v[...].astype(F32)
        act = jnp.broadcast_to(cf * _sigmoid(cf), (16, d)).astype(BF16)
        for i in range(lo, hi):
            mod_v[:, i * d:(i + 1) * d] = _dot(act, wmod_v[:, i * d:(i + 1) * d])[0:8]

    def mod(i, n):
        return _rows(mod_v[:, i * d:(i + 1) * d], n)

    def normed_tile(t):
        x = x_v[tile_rows(t), :].astype(F32)
        h = _layernorm(x) * (1.0 + mod(1, TILE)) + mod(0, TILE)
        h_v[pl.ds(pl.multiple_of(t * (TILE // 2), TILE // 2), TILE // 2), :] = _pack(h)

    def load_h(t):
        return _unpack(h_v[pl.ds(pl.multiple_of(t * (TILE // 2), TILE // 2), TILE // 2), :])

    wphi_cp.wait()
    wk_cp.wait()
    fold(1, wkt_v)
    wv_cp.wait()
    for g in range(d // 128):
        wv = wqkv_v[:, 2 * d + g * 128:2 * d + (g + 1) * 128]
        wvt_v[g * 64:(g + 1) * 64, :] = _pack(wv.T)
    c_cp.wait()
    mod_a_cp.wait()
    for t in range(1, n_tiles):
        x_copy(t).start()
    for cp in (wq_cp, wo_cp, mod_b_cp, wg_cp, wu_cp, wd_cp):
        cp.start()
    modulation(0, 2)
    x_copy(0).wait()
    normed_tile(0)
    kv_v[...] = jnp.zeros(kv_v.shape, F32)

    def phase1(t, carry):
        nxt = jnp.minimum(t + 1, n_tiles - 1)

        @pl.when(t + 1 < n_tiles)
        def _():
            x_copy(nxt).wait()

        h = load_h(t)
        ones = jnp.ones((KV_ROWS - PAIR, TILE), BF16)
        for m in range(d // CHUNK):
            rows = slice(m * CHUNK // 2, (m + 1) * CHUNK // 2)
            pk = _dot_nt(_unpack(wkt_v[rows, :]), h)
            v = _dot_nt(_unpack(wvt_v[rows, :]), h).astype(BF16)
            for j in range(CHUNK // PAIR):
                p = m * (CHUNK // PAIR) + j
                phi = _feature_map(pk[j * PAIR:(j + 1) * PAIR])
                lhs = jnp.concatenate([v[j * PAIR:(j + 1) * PAIR], ones], axis=0)
                kv_v[p] += _dot_nt(lhs, phi)
        normed_tile(nxt)
        return carry

    lax.fori_loop(0, n_tiles, phase1, 0)

    wq_cp.wait()
    fold(0, wqt_v)
    mod_b_cp.wait()
    modulation(2, 6)
    row = lax.broadcasted_iota(jnp.int32, (KV_ROWS, 128), 0)
    lane = lax.broadcasted_iota(jnp.int32, (KV_ROWS, 128), 1)
    own_head = jnp.where(row < PAIR, row // HEAD_DIM, (row - PAIR) // 8) == lane % 2
    for p in range(n_pairs):
        kvm_v[p] = _pack(jnp.where(own_head, kv_v[p], 0.0))
    wo_cp.wait()
    wr_cp.wait()
    w_r = jnp.broadcast_to(wr_v[...].astype(F32).reshape(1, d), (8, d))

    def phase2(t, carry):
        h = load_h(t)
        o_t = []
        for m in range(d // CHUNK):
            rows = slice(m * CHUNK // 2, (m + 1) * CHUNK // 2)
            pq = _dot_nt(_unpack(wqt_v[rows, :]), h)
            for j in range(CHUNK // PAIR):
                p = m * (CHUNK // PAIR) + j
                phi = _feature_map(pq[j * PAIR:(j + 1) * PAIR])
                res = _dot(_unpack(kvm_v[p]), phi)
                inv0 = _recip(res[PAIR:PAIR + 8] + DEN_EPS)
                inv1 = _recip(res[PAIR + 8:PAIR + 16] + DEN_EPS)
                inv = jnp.concatenate([_rows(inv0, HEAD_DIM), _rows(inv1, HEAD_DIM)], axis=0)
                o_t.append((res[:PAIR] * inv).astype(BF16))
        attn = _dot(jnp.concatenate(o_t, axis=0).T, wo_v[...])
        x1 = x_v[tile_rows(t), :].astype(F32) + mod(2, TILE) * attn
        h2 = _layernorm(x1) * (1.0 + mod(4, TILE)) + mod(3, TILE)
        x1_v[tile_rows(t), :] = x1
        out_v[tile_rows(t), :] = (x1 + mod(5, TILE) * h2).astype(BF16)
        score = jnp.sum(h2 * _rows(w_r, TILE), axis=-1, keepdims=True)
        lane_id = lax.broadcasted_iota(jnp.int32, (8, 128), 1)
        packed = jnp.full((8, 128), -jnp.inf, F32)
        for g in range(TILE // 8):
            packed = jnp.where(lane_id == g, score[8 * g:8 * g + 8], packed)
        r_v[pl.ds(pl.multiple_of(t * 8, 8), 8), :] = packed
        out_copy(t).start()
        return carry

    lax.fori_loop(0, n_tiles, phase2, 0)

    scores = r_v[...]
    row = lax.broadcasted_iota(jnp.int32, scores.shape, 0)
    lane = lax.broadcasted_iota(jnp.int32, scores.shape, 1)
    token = jnp.where(lane < TILE // 8, (row // 8) * TILE + lane * 8 + row % 8, seq)

    def arg_top(s, valid):
        best = jnp.max(jnp.where(valid, s, -jnp.inf))
        first = jnp.min(jnp.where(valid & (s == best), token, seq).astype(F32))
        return jnp.minimum(first.astype(jnp.int32), seq - 1)

    i0 = arg_top(scores, token < seq)
    i1 = arg_top(scores, (token < seq) & (token != i0))

    sub = lax.broadcasted_iota(jnp.int32, (16, d), 0)
    x1 = jnp.where(sub == 0, x1_v[pl.ds(i0, 1), :], x1_v[pl.ds(i1, 1), :])
    h2 = _layernorm(x1) * (1.0 + mod(4, 16)) + mod(3, 16)
    gate = _sigmoid(jnp.sum(h2 * _rows(w_r, 16), axis=-1, keepdims=True))
    xs = h2.astype(BF16)
    wg_cp.wait()
    wu_cp.wait()
    wd_cp.wait()
    g = _dot(xs, wg_v[...])
    u = _dot(xs, wu_v[...])
    y = _dot((g * _sigmoid(g) * u).astype(BF16), wd_v[...])
    routed = x1 + mod(5, 16) * (h2 + y * gate)

    for t in range(n_tiles):
        out_copy(t).wait()

    def patch(k, i):
        base = pl.multiple_of((i // 16) * 16, 16)
        old = out_v[pl.ds(base, 16), :].astype(F32)
        out_v[pl.ds(base, 16), :] = jnp.where(sub == i - base, routed[k:k + 1], old).astype(BF16)
        return base, copy(out_v.at[pl.ds(base, 16)], out_hbm.at[pl.ds(base, 16)], sem.at[12 + k])

    base0, patch0 = patch(0, i0)
    base1, patch1 = patch(1, i1)
    patch0.start()

    @pl.when(base1 != base0)
    def _():
        patch1.start()
        patch1.wait()

    patch0.wait()


@jax.jit
def pallas_adaLN_cond__linear_kernel_hedgehog__moe_arch_mod__prompt_kernel(
    A_x: jax.Array,
    A_wqkv: jax.Array,
    A_w_phi: jax.Array,
    A_wo: jax.Array,
    B_x: jax.Array,
    B_w_r: jax.Array,
    B_w_gate: jax.Array,
    B_w_up: jax.Array,
    B_w_down: jax.Array,
    c: jax.Array,
    w_mod: jax.Array,
):
    del B_x
    batch, seq, d = A_x.shape
    assert batch == 1 and d == HEADS * HEAD_DIM and seq % TILE == 0
    n_tiles = seq // TILE
    operands = (A_x.reshape(seq, d), A_wqkv, A_w_phi, A_wo, B_w_r, B_w_gate, B_w_up, B_w_down,
                c, w_mod)
    scratch = [pltpu.VMEM(a.shape, a.dtype) for a in operands] + [
        pltpu.VMEM((d // 2, d), U32),
        pltpu.VMEM((d // 2, d), U32),
        pltpu.VMEM((d // 2, d), U32),
        pltpu.VMEM((8, w_mod.shape[1]), F32),
        pltpu.VMEM((seq // 2, d), U32),
        pltpu.VMEM((HEADS // 2, KV_ROWS, 128), F32),
        pltpu.VMEM((HEADS // 2, KV_ROWS // 2, 128), U32),
        pltpu.VMEM((seq, d), F32),
        pltpu.VMEM((seq, d), BF16),
        pltpu.VMEM((n_tiles * 8, 128), F32),
        pltpu.SemaphoreType.DMA((14,)),
        pltpu.SemaphoreType.DMA((n_tiles,)),
        pltpu.SemaphoreType.DMA((n_tiles,)),
    ]
    out = pl.pallas_call(
        _kernel,
        out_shape=jax.ShapeDtypeStruct((seq, d), A_x.dtype),
        in_specs=[pl.BlockSpec(memory_space=pl.ANY)] * len(operands),
        out_specs=pl.BlockSpec(memory_space=pl.ANY),
        scratch_shapes=scratch,
        compiler_params=pltpu.CompilerParams(vmem_limit_bytes=110 * 2**20),
        name="adaln_hedgehog_mod",
    )(*operands)
    return out.reshape(batch, seq, d)
```

```python
import contextlib
import math

import jax
import jax.numpy as jnp
from jax import lax
import jax.experimental.pallas as pl
import jax.experimental.pallas.tpu as pltpu

F32 = jnp.float32
BF16 = jnp.bfloat16
I32 = jnp.int32

HEADS = 32
HEAD_DIM = 32
PAIR = 2 * HEAD_DIM
TERMS = 7
LN_EPS = 1e-5
DEN_EPS = 1e-6
LOG2E = math.log2(math.e)

TILE = 256
HALF = TILE // 2
CHUNK = 128
SCOPES = True
FLAGS = {"XLA_TPU_EVENLY_DISTRIBUTE_CRITICAL_NODES": True}

NT_DIMS = (((1,), (1,)), ((), ()))


def _scope(name):
    return jax.named_scope(name) if SCOPES else contextlib.nullcontext()


def _dot(a, b):
    return jnp.dot(a, b, preferred_element_type=F32)


def _dot_nt(a, b):
    return lax.dot_general(a, b, NT_DIMS, preferred_element_type=F32)


def _pack(v):
    return pltpu.bitcast(v.astype(BF16), I32)


def _pack_heads(v):
    starts = range(0, v.shape[0], PAIR)
    first = jnp.concatenate([v[s:s + HEAD_DIM] for s in starts], axis=0)
    second = jnp.concatenate([v[s + HEAD_DIM:s + PAIR] for s in starts], axis=0)
    return pltpu.pack_elementwise([first, second], packed_dtype=BF16).astype(I32)


def _unpack(v):
    return pltpu.bitcast(v, BF16)


def _recip(d):
    r = pltpu.reciprocal(d, approx=True)
    return r * (2.0 - d * r)


def _sigmoid(v):
    return 1.0 / (1.0 + jnp.exp(-v))


def _rows(v, n):
    return jnp.concatenate([v] * (n // 8), axis=0) if n > 8 else v


def _layernorm(x):
    inv_d = 1.0 / x.shape[-1]
    xc = x - jnp.sum(x, axis=-1, keepdims=True) * inv_d
    var = jnp.sum(xc * xc, axis=-1, keepdims=True) * inv_d
    return xc * lax.rsqrt(var + LN_EPS)


def _lhs_terms(a11, a12, a21, a22):
    return [a11 + a22, a21 + a22, a11, a22, a11 + a12, a21 - a11, a12 - a22]


def _rhs_terms(b11, b12, b21, b22):
    return [b11 + b22, b11, b12 - b22, b21 - b11, b22, b11 + b12, b21 + b22]


def _block_matmul(product):
    m1 = product(0)
    m4 = product(3)
    c11 = m1 + m4
    c11 = c11 + product(6)
    m5 = product(4)
    c11 = c11 - m5
    m3 = product(2)
    c12 = m3 + m5
    c22 = m1 + m3
    m2 = product(1)
    c21 = m2 + m4
    c22 = c22 - m2
    c22 = c22 + product(5)
    return c11, c12, c21, c22


def _head_reduce(op, tiles):
    while len(tiles) > 1:
        tiles = [op(tiles[i], tiles[i + 1]) for i in range(0, len(tiles), 2)]
    m = tiles[0]
    m = op(m, pltpu.roll(m, 4, 0))
    return op(m, pltpu.roll(m, 2, 0))


def _feature_map(p):
    tiles = [p[8 * j:8 * j + 8] for j in range(PAIR // 8)]
    hi = _head_reduce(jnp.maximum, tiles)
    lo = _head_reduce(jnp.minimum, tiles)
    e_pos = [jnp.exp2(t - hi) for t in tiles]
    e_neg = [jnp.exp2(lo - t) for t in tiles]
    r_pos = _recip(_head_reduce(jnp.add, e_pos))
    r_neg = _recip(_head_reduce(jnp.add, e_neg))
    return [e * r_pos for e in e_pos] + [e * r_neg for e in e_neg]


def _kernel(x_hbm, wqkv_hbm, wphi_hbm, wo_hbm, wr_hbm, wg_hbm, wu_hbm, wd_hbm, c_hbm, wmod_hbm,
            out_hbm,
            x_v, wqkv_v, wphi_v, wo_v, wr_v, wg_v, wu_v, wd_v, c_v, wmod_v,
            wq_s, wk_s, wv_s, wo_s, h_even, h_odd, o_even, o_odd, x1_even, x1_odd,
            mod_v, kv_v, kvm_v, z_v, out_v, r_v, sem, out_sem):
    seq, d = x_v.shape
    hd = d // 2
    n_tiles = seq // TILE
    n_pairs = HEADS // 2
    n_chunks = hd // CHUNK
    chunk_pairs = CHUNK // PAIR
    h_rows = HALF // 2
    w_rows = hd // 2
    h_s, o_s, x1_s = (h_even, h_odd), (o_even, o_odd), (x1_even, x1_odd)

    def rows(start, size):
        return pl.ds(start if isinstance(start, int) else pl.multiple_of(start, size), size)

    def copy(src, dst, s):
        return pltpu.make_async_copy(src, dst, s)

    def token_copy(src, dst, first, count, s):
        span = pl.ds(first if isinstance(first, int) else pl.multiple_of(first, TILE), count)
        return copy(src.at[span], dst.at[span], s)

    def cols(ref, i, n=1):
        return ref.at[:, pl.ds(i * d, n * d)]

    c_cp = copy(c_hbm, c_v, sem.at[0])
    wphi_cp = copy(wphi_hbm, wphi_v, sem.at[1])
    wr_cp = copy(wr_hbm, wr_v, sem.at[2])
    shift_cp = copy(cols(wmod_hbm, 0), cols(wmod_v, 0), sem.at[3])
    scale_cp = copy(cols(wmod_hbm, 1), cols(wmod_v, 1), sem.at[4])
    mod_b_cp = copy(cols(wmod_hbm, 2, 4), cols(wmod_v, 2, 4), sem.at[5])
    wq_cp = copy(cols(wqkv_hbm, 0), cols(wqkv_v, 0), sem.at[6])
    wk_cp = copy(cols(wqkv_hbm, 1), cols(wqkv_v, 1), sem.at[7])
    wv_cp = copy(cols(wqkv_hbm, 2), cols(wqkv_v, 2), sem.at[8])
    wo_cp = copy(wo_hbm, wo_v, sem.at[9])
    wg_cp = copy(wg_hbm, wg_v, sem.at[10])
    wu_cp = copy(wu_hbm, wu_v, sem.at[11])
    wd_cp = copy(wd_hbm, wd_v, sem.at[12])
    x0_cp = token_copy(x_hbm, x_v, 0, TILE, sem.at[13])
    x1_cp = token_copy(x_hbm, x_v, TILE, TILE, sem.at[14])
    x_rest_cp = token_copy(x_hbm, x_v, 2 * TILE, seq - 2 * TILE, sem.at[15])

    def store_terms(dst, g, terms):
        for i, term in enumerate(terms):
            dst[i * w_rows + g * 64:i * w_rows + (g + 1) * 64, :] = _pack_heads(term)

    def store_lhs_terms(dst, g, group):
        top, bottom = group(g), group(g + hd // 128)
        store_terms(dst, g, _lhs_terms(top[:, :hd], top[:, hd:], bottom[:, :hd], bottom[:, hd:]))

    def fold(col, dst, g):
        row = lax.broadcasted_iota(I32, (128, 128), 0)
        lane = lax.broadcasted_iota(I32, (128, 128), 1)
        same_head = row // HEAD_DIM == lane // HEAD_DIM
        row_f = lax.broadcasted_iota(I32, (128, HEAD_DIM), 0)
        lane_f = lax.broadcasted_iota(I32, (128, HEAD_DIM), 1)
        pick = jnp.where(row_f % HEAD_DIM == lane_f, 1.0, 0.0).astype(BF16)

        def group(g):
            wphi = wphi_v[4 * g:4 * g + 4].reshape(128, HEAD_DIM)
            a = jnp.where(same_head, _dot_nt(pick, wphi), 0.0).astype(BF16)
            return _dot_nt(a, wqkv_v[:, col * d + g * 128:col * d + (g + 1) * 128]) * LOG2E

        store_lhs_terms(dst, g, group)

    def value_terms(g):
        store_lhs_terms(
            wv_s, g, lambda g: wqkv_v[:, 2 * d + g * 128:2 * d + (g + 1) * 128].astype(F32).T)

    def output_terms(g):
        top = wo_v[g * 128:(g + 1) * 128, :].astype(F32)
        bottom = wo_v[hd + g * 128:hd + (g + 1) * 128, :].astype(F32)
        store_terms(wo_s, g, _rhs_terms(top[:, :hd], top[:, hd:], bottom[:, :hd], bottom[:, hd:]))

    def modulation(i):
        cf = c_v[...].astype(F32)
        act = jnp.broadcast_to(cf * _sigmoid(cf), (16, d)).astype(BF16)
        m = _dot(act, wmod_v[:, i * d:(i + 1) * d])[0:8]
        mod_v[:, i * d:(i + 1) * d] = 1.0 + m if i % 3 == 1 else m

    def mod(i, n):
        return _rows(mod_v[:, i * d:(i + 1) * d], n)

    def first_token(i, parity):
        return (2 * i + parity) * TILE

    def normed_piece(i, parity, k):
        def normed(start):
            x = x_v[rows(first_token(i, parity) + start + 16 * k, 16), :].astype(F32)
            return _layernorm(x) * mod(1, 16) + mod(0, 16)

        ha, hb = normed(0), normed(HALF)
        for j, term in enumerate(_rhs_terms(ha[:, :hd], hb[:, :hd], ha[:, hd:], hb[:, hd:])):
            h_s[parity][rows((i * TERMS + j) * h_rows + 8 * k, 8), :] = _pack(term)

    def project(w_s, i, parity, m):
        def product(j):
            w = w_s[j * w_rows + m * CHUNK // 2:j * w_rows + (m + 1) * CHUNK // 2, :]
            h = h_s[parity][rows((i * TERMS + j) * h_rows, h_rows), :]
            return _dot_nt(_unpack(w), _unpack(h))

        c11, c12, c21, c22 = _block_matmul(product)
        halves = (jnp.concatenate([c11, c12], axis=1), jnp.concatenate([c21, c22], axis=1))
        return [(side * (n_pairs // 2) + m * chunk_pairs + j, block[j * PAIR:(j + 1) * PAIR])
                for side, block in enumerate(halves) for j in range(chunk_pairs)]

    def share(m, total):
        return range(m * total // n_chunks, (m + 1) * total // n_chunks)

    def key_features(pk):
        out = []
        for p, pk_p in pk:
            phi = jnp.concatenate(_feature_map(pk_p), axis=0)
            z_v[p * 128:(p + 1) * 128, :] += phi[:, :HALF] + phi[:, HALF:]
            out.append(phi.astype(BF16))
        return out

    def accumulate_kv(phi, v):
        for phi_p, (p, v_p) in zip(phi, v):
            kv_v[p * PAIR:(p + 1) * PAIR, :] += _dot_nt(v_p.astype(BF16), phi_p)

    def summarize(i, parity, between):
        for m in range(n_chunks):
            pk = project(wk_s, i, parity, m)
            v = project(wv_s, i, parity, m)
            accumulate_kv(key_features(pk), v)
            between(m)

    def normalize(i, parity):
        def pieces(m):
            for k in share(m, HALF // 16):
                normed_piece(i, parity, k)
        return pieces

    def read_out(parity, m, pq):
        o_t = []
        for p, pq_p in pq:
            phi = _feature_map(pq_p)
            z = [z_v[p * 128 + 8 * j:p * 128 + 8 * j + 8, :] for j in range(len(phi))]
            den = _head_reduce(
                jnp.add, [f * jnp.concatenate([zj, zj], axis=1) for f, zj in zip(phi, z)])
            num = _dot(_unpack(kvm_v[p * HEAD_DIM:(p + 1) * HEAD_DIM, :]),
                       jnp.concatenate(phi, axis=0).astype(BF16))
            o_t.append(num * _rows(_recip(den + DEN_EPS), PAIR))
        top = jnp.concatenate(o_t[:chunk_pairs], axis=0)
        bottom = jnp.concatenate(o_t[chunk_pairs:], axis=0)
        terms = _lhs_terms(top[:, :HALF], bottom[:, :HALF], top[:, HALF:], bottom[:, HALF:])
        for j, term in enumerate(terms):
            o_s[parity][j * h_rows:(j + 1) * h_rows, m * CHUNK:(m + 1) * CHUNK] = pltpu.bitcast(
                term.astype(BF16).T, I32)

    def residual(i, parity, g):
        def product(j):
            o = o_s[parity][j * h_rows:(j + 1) * h_rows, :]
            w = wo_s[j * w_rows:(j + 1) * w_rows, g * 128:(g + 1) * 128]
            return _dot(_unpack(o), _unpack(w))

        for b, attn in enumerate(_block_matmul(product)):
            r0 = (b // 2) * HALF
            c0 = (b % 2) * hd + g * 128
            x = x_v[rows(first_token(i, parity) + r0, HALF), c0:c0 + 128].astype(F32)
            gate = _rows(mod_v[:, 2 * d + c0:2 * d + c0 + 128], HALF)
            x1_s[parity][rows(i * TILE + r0, HALF), c0:c0 + 128] = x + gate * attn

    def finish(i, parity, groups):
        lane = lax.broadcasted_iota(I32, (8, 128), 1)
        slot = rows((2 * i + parity) * 8, 8)
        packed = r_v[slot, :]
        for g in groups:
            x1 = x1_s[parity][rows(i * TILE + 16 * g, 16), :]
            h2 = _layernorm(x1) * mod(4, 16) + mod(3, 16)
            out_v[rows(first_token(i, parity) + 16 * g, 16), :] = (
                x1 + mod(5, 16) * h2).astype(BF16)
            score = jnp.sum(h2 * mod(6, 16), axis=-1, keepdims=True)
            for s in range(2):
                packed = jnp.where(lane == 2 * g + s, score[8 * s:8 * s + 8], packed)
        r_v[slot, :] = packed

    def attend(i, parity, prev=None, done=None):
        for m in range(n_chunks):
            pq = project(wq_s, i, parity, m)
            if prev is not None:
                for g in share(m, hd // 128):
                    residual(*prev, g)
            read_out(parity, m, pq)
            if done is not None:
                finish(*done, share(m, TILE // 16))

    def out_copy(i):
        return token_copy(out_v, out_hbm, first_token(i, 0), 2 * TILE, out_sem.at[i])

    for cp in (c_cp, wphi_cp, wk_cp, x0_cp, scale_cp, shift_cp, wv_cp, x1_cp):
        cp.start()
    kv_v[...] = jnp.zeros(kv_v.shape, F32)
    z_v[...] = jnp.zeros(z_v.shape, F32)
    r_v[...] = jnp.full(r_v.shape, -jnp.inf, F32)
    with _scope("wait_wk"):
        wphi_cp.wait()
        wk_cp.wait()
    with _scope("fold_k"):
        for g in range(hd // 128):
            fold(1, wk_s, g)
    with _scope("mod_a"):
        c_cp.wait()
        scale_cp.wait()
        modulation(1)
        shift_cp.wait()
        modulation(0)
    with _scope("k0"):
        x0_cp.wait()
        for k in range(HALF // 16):
            normed_piece(0, 0, k)
        phi0 = [key_features(project(wk_s, 0, 0, m)) for m in range(n_chunks)]
    with _scope("v0"):
        wv_cp.wait()
        x1_cp.wait()
        for cp in (x_rest_cp, wq_cp, wo_cp, wr_cp, mod_b_cp):
            cp.start()
        for m in range(n_chunks):
            for g in share(m, hd // 128):
                value_terms(g)
        for m in range(n_chunks):
            accumulate_kv(phi0[m], project(wv_s, 0, 0, m))
            normalize(0, 1)(m)
        x_rest_cp.wait()

    def phase1(i, carry):
        for step, cp in enumerate((wg_cp, wu_cp, wd_cp)):
            pl.when(i == step)(cp.start)
        summarize(i, 1, normalize(i + 1, 0))
        summarize(i + 1, 0, normalize(i + 1, 1))
        return carry

    last = n_tiles // 2 - 1
    with _scope("phase1"):
        lax.fori_loop(0, last, phase1, 0)

    with _scope("tile7"):
        for cp in (wq_cp, wo_cp, wr_cp, mod_b_cp):
            cp.wait()
        mod_v[:, 6 * d:7 * d] = jnp.broadcast_to(wr_v[...].astype(F32).reshape(1, d), (8, d))

        def prepare(m):
            for g in share(m, hd // 128):
                output_terms(g)
                fold(0, wq_s, g)

        summarize(last, 1, prepare)

    with _scope("mid"):
        row = lax.broadcasted_iota(I32, (PAIR, 128), 0)
        lane = lax.broadcasted_iota(I32, (PAIR, 128), 1)
        for p in range(n_pairs):
            kv = jnp.where(row % 2 == lane % 2, kv_v[p * PAIR:(p + 1) * PAIR, :], 0.0)
            kvm_v[p * HEAD_DIM:(p + 1) * HEAD_DIM, :] = _pack(kv)
            z = jnp.sum(z_v[p * 128:(p + 1) * 128, :], axis=1, keepdims=True)
            z_v[p * 128:(p + 1) * 128, :] = jnp.broadcast_to(z, (128, 128))
        pq = project(wq_s, 0, 0, 0)
        for m in range(n_chunks):
            ahead = project(wq_s, 0, 0, m + 1) if m + 1 < n_chunks else None
            for j in share(m, 4):
                modulation(2 + j)
            read_out(0, m, pq)
            pq = ahead
        attend(0, 1, prev=(0, 0))

    def phase2(i, carry):
        attend(i, 0, prev=(i - 1, 1), done=(i - 1, 0))
        attend(i, 1, prev=(i, 0), done=(i - 1, 1))
        out_copy(i - 1).start()
        return carry

    with _scope("phase2"):
        lax.fori_loop(1, last + 1, phase2, 0)
    with _scope("last"):
        for m in range(n_chunks):
            for g in share(m, hd // 128):
                residual(last, 1, g)
            finish(last, 0, share(m, TILE // 16))
        finish(last, 1, range(TILE // 16))
        out_copy(last).start()

    with _scope("route"):
        scores = r_v[...]
        row = lax.broadcasted_iota(I32, scores.shape, 0)
        lane = lax.broadcasted_iota(I32, scores.shape, 1)
        token = jnp.where(lane < TILE // 8, (row // 8) * TILE + lane * 8 + row % 8, seq)

        def arg_top(valid):
            best = jnp.max(jnp.where(valid, scores, -jnp.inf))
            first = jnp.min(jnp.where(valid & (scores == best), token, seq).astype(F32))
            return jnp.minimum(first.astype(I32), seq - 1)

        i0 = arg_top(token < seq)
        i1 = arg_top((token < seq) & (token != i0))

        def residual_row(i):
            local = pl.ds((i // (2 * TILE)) * TILE + i % TILE, 1)
            return jnp.where((i // TILE) % 2 == 0, x1_even[local, :], x1_odd[local, :])

        sub = lax.broadcasted_iota(I32, (16, d), 0)
        x1 = jnp.where(sub == 0, residual_row(i0), residual_row(i1))
        h2 = _layernorm(x1) * mod(4, 16) + mod(3, 16)
        gate = _sigmoid(jnp.sum(h2 * mod(6, 16), axis=-1, keepdims=True))
        xs = h2.astype(BF16)
        for cp in (wg_cp, wu_cp, wd_cp):
            cp.wait()
    with _scope("ffn"):
        g = _dot(xs, wg_v[...])
        u = _dot(xs, wu_v[...])
        y = _dot((g * _sigmoid(g) * u).astype(BF16), wd_v[...])
        routed = x1 + mod(5, 16) * (h2 + y * gate)

    for i in range(last + 1):
        out_copy(i).wait()

    def patch(k, i):
        base = pl.multiple_of((i // 16) * 16, 16)
        old = out_v[pl.ds(base, 16), :].astype(F32)
        out_v[pl.ds(base, 16), :] = jnp.where(sub == i - base, routed[k:k + 1], old).astype(BF16)
        return base, copy(out_v.at[pl.ds(base, 16)], out_hbm.at[pl.ds(base, 16)], sem.at[16 + k])

    base0, patch0 = patch(0, i0)
    base1, patch1 = patch(1, i1)
    patch0.start()

    @pl.when(base1 != base0)
    def _():
        patch1.start()
        patch1.wait()

    patch0.wait()


@jax.jit
def pallas_adaLN_cond__linear_kernel_hedgehog__moe_arch_mod__prompt_kernel(
    A_x: jax.Array,
    A_wqkv: jax.Array,
    A_w_phi: jax.Array,
    A_wo: jax.Array,
    B_x: jax.Array,
    B_w_r: jax.Array,
    B_w_gate: jax.Array,
    B_w_up: jax.Array,
    B_w_down: jax.Array,
    c: jax.Array,
    w_mod: jax.Array,
):
    del B_x
    batch, seq, d = A_x.shape
    assert batch == 1 and d == HEADS * HEAD_DIM and seq == 8 * TILE
    n_tiles = seq // TILE
    operands = (A_x.reshape(seq, d), A_wqkv, A_w_phi, A_wo, B_w_r, B_w_gate, B_w_up, B_w_down,
                c, w_mod)
    weight_terms = pltpu.VMEM((TERMS * d // 4, d // 2), I32)
    normed_terms = pltpu.VMEM((n_tiles // 2 * TERMS * HALF // 2, d // 2), I32)
    readout_terms = pltpu.VMEM((TERMS * HALF // 2, d // 2), I32)
    residual_rows = pltpu.VMEM((seq // 2, d), F32)
    scratch = [pltpu.VMEM(a.shape, a.dtype) for a in operands] + [
        weight_terms, weight_terms, weight_terms, weight_terms,
        normed_terms, normed_terms, readout_terms, readout_terms, residual_rows, residual_rows,
        pltpu.VMEM((8, 7 * d), F32),
        pltpu.VMEM((HEADS // 2 * PAIR, 128), F32),
        pltpu.VMEM((HEADS // 2 * HEAD_DIM, 128), I32),
        pltpu.VMEM((HEADS // 2 * 128, 128), F32),
        pltpu.VMEM((seq, d), BF16),
        pltpu.VMEM((n_tiles * 8, 128), F32),
        pltpu.SemaphoreType.DMA((18,)),
        pltpu.SemaphoreType.DMA((n_tiles // 2,)),
    ]
    out = pl.pallas_call(
        _kernel,
        out_shape=jax.ShapeDtypeStruct((seq, d), A_x.dtype),
        in_specs=[pl.BlockSpec(memory_space=pl.ANY)] * len(operands),
        out_specs=pl.BlockSpec(memory_space=pl.ANY),
        scratch_shapes=scratch,
        compiler_params=pltpu.CompilerParams(vmem_limit_bytes=110 * 2**20, flags=FLAGS or None),
        name="adaln_hedgehog_mod",
    )(*operands)
    return out.reshape(batch, seq, d)
```

```python
import contextlib
import math

import jax
import jax.numpy as jnp
from jax import lax
import jax.experimental.pallas as pl
import jax.experimental.pallas.tpu as pltpu

F32 = jnp.float32
BF16 = jnp.bfloat16
I32 = jnp.int32

HEADS = 32
HEAD_DIM = 32
PAIR = 2 * HEAD_DIM
TERMS = 7
LN_EPS = 1e-5
DEN_EPS = 1e-6
LOG2E = math.log2(math.e)

TILE = 256
HALF = TILE // 2
CHUNK = 128
SCOPES = True
ONLY = None
LN_GATES = (7, 7)
FIN_GATES = (4, 4, 7, 7)
PIN_START = True
FLAGS = {"XLA_TPU_EVENLY_DISTRIBUTE_CRITICAL_NODES": True}

NT_DIMS = (((1,), (1,)), ((), ()))


def _scope(name):
    return jax.named_scope(name) if SCOPES else contextlib.nullcontext()


def _dot(a, b):
    return jnp.dot(a, b, preferred_element_type=F32)


def _dot_nt(a, b):
    return lax.dot_general(a, b, NT_DIMS, preferred_element_type=F32)


def _pack(v):
    return pltpu.bitcast(v.astype(BF16), I32)


def _pack_heads(v):
    starts = range(0, v.shape[0], PAIR)
    first = jnp.concatenate([v[s:s + HEAD_DIM] for s in starts], axis=0)
    second = jnp.concatenate([v[s + HEAD_DIM:s + PAIR] for s in starts], axis=0)
    return pltpu.pack_elementwise([first, second], packed_dtype=BF16).astype(I32)


def _unpack(v):
    return pltpu.bitcast(v, BF16)


def _recip(d):
    r = pltpu.reciprocal(d, approx=True)
    return r * (2.0 - d * r)


def _sigmoid(v):
    return 1.0 / (1.0 + jnp.exp(-v))


def _rows(v, n):
    return jnp.concatenate([v] * (n // 8), axis=0) if n > 8 else v


def _centered(x, after=None):
    inv_d = 1.0 / x.shape[-1]
    if after is not None:
        head = x[:, :128] + _rows(pltpu.bitcast(after, F32), x.shape[0])
        x = jnp.concatenate([head, x[:, 128:]], axis=1)
    xc = x - jnp.sum(x, axis=-1, keepdims=True) * inv_d
    var = jnp.sum(xc * xc, axis=-1, keepdims=True) * inv_d
    return xc, lax.rsqrt(var + LN_EPS)


def _lhs_terms(a11, a12, a21, a22):
    return [a11 + a22, a21 + a22, a11, a22, a11 + a12, a21 - a11, a12 - a22]


def _rhs_terms(b11, b12, b21, b22):
    return [b11 + b22, b11, b12 - b22, b21 - b11, b22, b11 + b12, b21 + b22]


def _block_matmul(product):
    m1 = product(0, 0)
    m4 = product(1, 3)
    c11 = m1 + m4
    c11 = c11 + product(2, 6)
    m5 = product(3, 4)
    c11 = c11 - m5
    m3 = product(4, 2)
    c12 = m3 + m5
    c22 = m1 + m3
    m2 = product(5, 1)
    c21 = m2 + m4
    c22 = c22 - m2
    c22 = c22 + product(6, 5)
    return c11, c12, c21, c22


def _head_reduce(op, tiles):
    while len(tiles) > 1:
        tiles = [op(tiles[i], tiles[i + 1]) for i in range(0, len(tiles), 2)]
    m = tiles[0]
    m = op(m, pltpu.roll(m, 4, 0))
    return op(m, pltpu.roll(m, 2, 0))


def _feature_map(p):
    tiles = [p[8 * j:8 * j + 8] for j in range(PAIR // 8)]
    hi = _head_reduce(jnp.maximum, tiles)
    lo = _head_reduce(jnp.minimum, tiles)
    e_pos = [jnp.exp2(t - hi) for t in tiles]
    e_neg = [jnp.exp2(lo - t) for t in tiles]
    r_pos = _recip(_head_reduce(jnp.add, e_pos))
    r_neg = _recip(_head_reduce(jnp.add, e_neg))
    return [e * r_pos for e in e_pos] + [e * r_neg for e in e_neg]


SHIFT_A, SCALE_A, GATE_A, SHIFT_B, SCALE_B, GATE_B, ROUTER, OUT_SCALE, OUT_SHIFT, SCORE = range(10)


def _kernel(x_hbm, wqkv_hbm, wphi_hbm, wo_hbm, wr_hbm, wg_hbm, wu_hbm, wd_hbm, c_hbm, wmod_hbm,
            out_hbm,
            x_v, wqkv_v, wphi_v, wo_v, wr_v, wg_v, wu_v, wd_v, c_v, wmod_v,
            wq_s, wk_s, wv_s, wo_s, h_s, o_s, x1_v, mod_v, kv_v, kvm_v, z_v, out_v, r_v, zero_v,
            sem, out_sem):
    seq, d = x_v.shape
    hd = d // 2
    n_tiles = seq // TILE
    n_pairs = HEADS // 2
    n_chunks = hd // CHUNK
    chunk_pairs = CHUNK // PAIR
    h_rows = HALF // 2
    w_rows = hd // 2

    def copy(src, dst, s):
        return pltpu.make_async_copy(src, dst, s)

    def rows(start, size):
        return pl.ds(start if isinstance(start, int) else pl.multiple_of(start, 8), size)

    def token_rows(start, size):
        return pl.ds(start if isinstance(start, int) else pl.multiple_of(start, 16), size)

    def token_copy(src, dst, first, count, s):
        span = pl.ds(first if isinstance(first, int) else pl.multiple_of(first, TILE), count)
        return copy(src.at[span], dst.at[span], s)

    def cols(ref, i, n=1):
        return ref.at[:, pl.ds(i * d, n * d)]

    c_cp = copy(c_hbm, c_v, sem.at[0])
    wphi_cp = copy(wphi_hbm, wphi_v, sem.at[1])
    wr_cp = copy(wr_hbm, wr_v, sem.at[2])
    shift_cp = copy(cols(wmod_hbm, 0), cols(wmod_v, 0), sem.at[3])
    scale_cp = copy(cols(wmod_hbm, 1), cols(wmod_v, 1), sem.at[4])
    mod_b_cp = copy(cols(wmod_hbm, 2, 4), cols(wmod_v, 2, 4), sem.at[5])
    wq_cp = copy(cols(wqkv_hbm, 0), cols(wqkv_v, 0), sem.at[6])
    wk_cp = copy(cols(wqkv_hbm, 1), cols(wqkv_v, 1), sem.at[7])
    wv_cp = copy(cols(wqkv_hbm, 2), cols(wqkv_v, 2), sem.at[8])
    wo_cp = copy(wo_hbm, wo_v, sem.at[9])
    wg_cp = copy(wg_hbm, wg_v, sem.at[10])
    wu_cp = copy(wu_hbm, wu_v, sem.at[11])
    wd_cp = copy(wd_hbm, wd_v, sem.at[12])
    x0_cp = token_copy(x_hbm, x_v, 0, TILE, sem.at[13])
    x1_cp = token_copy(x_hbm, x_v, TILE, TILE, sem.at[14])
    x_rest_cp = token_copy(x_hbm, x_v, 2 * TILE, seq - 2 * TILE, sem.at[15])

    def first_token(t):
        return (2 * t[0] + t[1]) * TILE

    def out_copy(i):
        return token_copy(out_v, out_hbm, first_token((i, 0)), 2 * TILE, out_sem.at[i])

    def token(values):
        tiles = [pltpu.bitcast(v[r:r + 8, c:c + 128], I32) for v in values
                 for r in range(0, v.shape[0], 8) for c in range(0, v.shape[1], 128)]
        while len(tiles) > 1:
            tiles = [tiles[j] | tiles[j + 1] if j + 1 < len(tiles) else tiles[j]
                     for j in range(0, len(tiles), 2)]
        return tiles[0] & zero_v[...]

    def gated(w, gates, step):
        for before, zero in gates:
            if before == step:
                top = jnp.concatenate([w[:8, :128] | zero, w[:8, 128:]], axis=1)
                w = jnp.concatenate([top, w[8:]], axis=0)
        return w

    def spill_over(gates):
        return [(before - TERMS, zero) for before, zero in gates if before >= TERMS]

    def store_terms(dst, g, terms):
        for i, term in enumerate(terms):
            dst[i * w_rows + g * 64:i * w_rows + (g + 1) * 64, :] = _pack_heads(term)

    def store_lhs_terms(dst, g, group):
        top, bottom = group(g), group(g + hd // 128)
        store_terms(dst, g, _lhs_terms(top[:, :hd], top[:, hd:], bottom[:, :hd], bottom[:, hd:]))

    def fold(col, dst, g):
        row = lax.broadcasted_iota(I32, (128, 128), 0)
        lane = lax.broadcasted_iota(I32, (128, 128), 1)
        same_head = row // HEAD_DIM == lane // HEAD_DIM
        row_f = lax.broadcasted_iota(I32, (128, HEAD_DIM), 0)
        lane_f = lax.broadcasted_iota(I32, (128, HEAD_DIM), 1)
        pick = jnp.where(row_f % HEAD_DIM == lane_f, 1.0, 0.0).astype(BF16)

        def group(g):
            wphi = wphi_v[4 * g:4 * g + 4].reshape(128, HEAD_DIM)
            a = jnp.where(same_head, _dot_nt(pick, wphi), 0.0).astype(BF16)
            return _dot_nt(a, wqkv_v[:, col * d + g * 128:col * d + (g + 1) * 128]) * LOG2E

        store_lhs_terms(dst, g, group)

    def value_terms(g):
        store_lhs_terms(
            wv_s, g, lambda g: wqkv_v[:, 2 * d + g * 128:2 * d + (g + 1) * 128].astype(F32).T)

    def output_terms(g):
        top = wo_v[g * 128:(g + 1) * 128, :].astype(F32)
        bottom = wo_v[hd + g * 128:hd + (g + 1) * 128, :].astype(F32)
        store_terms(wo_s, g, _rhs_terms(top[:, :hd], top[:, hd:], bottom[:, :hd], bottom[:, hd:]))

    def vec(i):
        return mod_v[:, i * d:(i + 1) * d]

    def modulation(i):
        cf = c_v[...].astype(F32)
        act = jnp.broadcast_to(cf * _sigmoid(cf), (16, d)).astype(BF16)
        m = _dot(act, wmod_v[:, i * d:(i + 1) * d])[0:8]
        mod_v[:, i * d:(i + 1) * d] = 1.0 + m if i in (SCALE_A, SCALE_B) else m

    def derived_vectors():
        router = jnp.broadcast_to(wr_v[...].astype(F32).reshape(1, d), (8, d))
        for i, v in ((ROUTER, router), (OUT_SCALE, vec(GATE_B) * vec(SCALE_B)),
                     (OUT_SHIFT, vec(GATE_B) * vec(SHIFT_B)), (SCORE, router * vec(SCALE_B))):
            mod_v[:, i * d:(i + 1) * d] = v

    def normed_piece(t, k, after=None):
        def normed(start):
            x = x_v[token_rows(first_token(t) + start + 16 * k, 16), :]
            xc, rstd = _centered(x.astype(F32), after)
            return xc * rstd * _rows(vec(SCALE_A), 16) + _rows(vec(SHIFT_A), 16)

        ha, hb = normed(0), normed(HALF)
        packed = [_pack(term)
                  for term in _rhs_terms(ha[:, :hd], hb[:, :hd], ha[:, hd:], hb[:, hd:])]
        for j, term in enumerate(packed):
            h_s[t[1]][rows((t[0] * TERMS + j) * h_rows + 8 * k, 8), :] = term
        return token(packed)

    def project(w_s, t, m, gates=()):
        def product(step, j):
            w = w_s[j * w_rows + m * CHUNK // 2:j * w_rows + (m + 1) * CHUNK // 2, :]
            h = h_s[t[1]][rows((t[0] * TERMS + j) * h_rows, h_rows), :]
            return _dot_nt(_unpack(gated(w, gates, step)), _unpack(h))

        c11, c12, c21, c22 = _block_matmul(product)
        halves = (jnp.concatenate([c11, c12], axis=1), jnp.concatenate([c21, c22], axis=1))
        return [(side * (n_pairs // 2) + m * chunk_pairs + j, block[j * PAIR:(j + 1) * PAIR])
                for side, block in enumerate(halves) for j in range(chunk_pairs)]

    def key_features(pk):
        out = []
        for p, pk_p in pk:
            phi = jnp.concatenate(_feature_map(pk_p), axis=0)
            z_v[p * 128:(p + 1) * 128, :] += phi[:, :HALF] + phi[:, HALF:]
            out.append(phi.astype(BF16))
        return out

    def accumulate_kv(phi, v):
        for phi_p, (p, v_p) in zip(phi, v):
            kv_v[p * PAIR:(p + 1) * PAIR, :] += _dot_nt(v_p.astype(BF16), phi_p)

    def summarize(t, state, side):
        pending, start = state
        for m in range(n_chunks):
            gates = side(m, start)
            pk = project(wk_s, t, m, gates)
            if pending is not None:
                accumulate_kv(*pending)
            v = project(wv_s, t, m, spill_over(gates))
            pending = (key_features(pk), v)
            start = token([v[-1][1][-8:, -128:]]) if PIN_START else None
        return pending, start

    def normalize(t):
        def pieces(m, after=None):
            return [(before, normed_piece(t, 2 * m + j, after)) for j, before in enumerate(LN_GATES)]
        return pieces

    def read_out(t, m, pq):
        o_t = []
        for p, pq_p in pq:
            phi = _feature_map(pq_p)
            z = [z_v[p * 128 + 8 * j:p * 128 + 8 * j + 8, :] for j in range(len(phi))]
            den = _head_reduce(
                jnp.add, [f * jnp.concatenate([zj, zj], axis=1) for f, zj in zip(phi, z)])
            num = _dot(_unpack(kvm_v[p * HEAD_DIM:(p + 1) * HEAD_DIM, :]),
                       jnp.concatenate(phi, axis=0).astype(BF16))
            o_t.append(num * _rows(_recip(den + DEN_EPS), PAIR))
        top = jnp.concatenate(o_t[:chunk_pairs], axis=0)
        bottom = jnp.concatenate(o_t[chunk_pairs:], axis=0)
        terms = _lhs_terms(top[:, :HALF], bottom[:, :HALF], top[:, HALF:], bottom[:, HALF:])
        for j, term in enumerate(terms):
            o_s[t[1]][j * h_rows:(j + 1) * h_rows, m * CHUNK:(m + 1) * CHUNK] = pltpu.bitcast(
                term.astype(BF16).T, I32)

    def residual(t, g, gates=()):
        def product(step, j):
            o = o_s[t[1]][j * h_rows:(j + 1) * h_rows, :]
            w = wo_s[j * w_rows:(j + 1) * w_rows, g * 128:(g + 1) * 128]
            return _dot(_unpack(gated(o, gates, step)), _unpack(w))

        for b, attn in enumerate(_block_matmul(product)):
            r0 = (b // 2) * HALF
            c0 = (b % 2) * hd + g * 128
            gate = _rows(mod_v[:, GATE_A * d + c0:GATE_A * d + c0 + 128], HALF)
            x = x_v[token_rows(first_token(t) + r0, HALF), c0:c0 + 128].astype(F32)
            x1_v[t[1]][rows(t[0] * TILE + r0, HALF), c0:c0 + 128] = x + gate * attn
        return token([attn[-8:]])

    def finish(t, g, after=None):
        x1 = x1_v[t[1]][rows(t[0] * TILE + 16 * g, 16), :]
        xc, rstd = _centered(x1, after)
        out = x1 + (xc * rstd * _rows(vec(OUT_SCALE), 16) + _rows(vec(OUT_SHIFT), 16))
        out_v[token_rows(first_token(t) + 16 * g, 16), :] = out.astype(BF16)
        score = jnp.sum(xc * _rows(vec(SCORE), 16), axis=-1, keepdims=True) * rstd
        lane = lax.broadcasted_iota(I32, (8, 128), 1)
        slot = rows((2 * t[0] + t[1]) * 8, 8)
        packed = r_v[slot, :]
        for s in range(2):
            packed = jnp.where(lane == 2 * g + s, score[8 * s:8 * s + 8], packed)
        r_v[slot, :] = packed
        return token([packed, out[:, -128:]])

    def finishing(t):
        def pieces(m, after=None):
            return [(before, finish(t, 4 * m + j, after)) for j, before in enumerate(FIN_GATES)]
        return pieces

    def no_side(m, after=None):
        return []

    def attend(t, start, side, middle):
        gates = side(0, start)
        pq = project(wq_s, t, 0, gates)
        for m in range(n_chunks):
            ahead = None
            if m + 1 < n_chunks:
                start = token([pq[-1][1][-8:, -128:]]) if m == 0 else start
                gates = spill_over(gates) + side(m + 1, start if PIN_START else None)
                ahead = project(wq_s, t, m + 1, gates)
                start = middle(m, spill_over(gates))
                gates = []
                read_out(t, m, pq)
            else:
                read_out(t, m, pq)
                start = middle(m, [])
            pq = ahead
        return start if PIN_START else None

    def prologue():
        wphi_cp.wait()
        wk_cp.wait()
        for g in range(n_chunks):
            fold(1, wk_s, g)
        scale_cp.wait()
        modulation(SCALE_A)
        shift_cp.wait()
        modulation(SHIFT_A)
        x0_cp.wait()
        for k in range(HALF // 16):
            normed_piece((0, 0), k)

    def first_tile():
        phi0 = [key_features(project(wk_s, (0, 0), m)) for m in range(n_chunks)]
        wv_cp.wait()
        x1_cp.wait()
        for cp in (x_rest_cp, wq_cp, wo_cp, wr_cp, mod_b_cp):
            cp.start()
        for g in range(n_chunks):
            value_terms(g)
        pending = None
        for m in range(n_chunks):
            v = project(wv_s, (0, 0), m)
            normalize((0, 1))(m)
            if pending is not None:
                accumulate_kv(*pending)
            pending = (phi0[m], v)
        accumulate_kv(*pending)
        x_rest_cp.wait()

    last = n_tiles // 2 - 1

    def summarize_tiles():
        def body(i, carry):
            for step, cp in enumerate((wg_cp, wu_cp, wd_cp)):
                pl.when(i == step)(cp.start)
            state = summarize((i, 1), (None, None), normalize((i + 1, 0)))
            state = summarize((i + 1, 0), state, normalize((i + 1, 1)))
            accumulate_kv(*state[0])
            return carry
        lax.fori_loop(0, last, body, 0)

    def last_summary():
        for cp in (wq_cp, wo_cp, wr_cp, mod_b_cp):
            cp.wait()

        def prepare(m, after):
            output_terms(m)
            fold(0, wq_s, m)
            return []

        accumulate_kv(*summarize((last, 1), (None, None), prepare)[0])

    def first_read_outs():
        row = lax.broadcasted_iota(I32, (PAIR, 128), 0)
        lane = lax.broadcasted_iota(I32, (PAIR, 128), 1)
        for p in range(n_pairs):
            kv = jnp.where(row % 2 == lane % 2, kv_v[p * PAIR:(p + 1) * PAIR, :], 0.0)
            kvm_v[p * HEAD_DIM:(p + 1) * HEAD_DIM, :] = _pack(kv)
            z = jnp.sum(z_v[p * 128:(p + 1) * 128, :], axis=1, keepdims=True)
            z_v[p * 128:(p + 1) * 128, :] = jnp.broadcast_to(z, (128, 128))
        attend((0, 0), None, no_side, lambda m, gates: modulation(GATE_A + m))
        derived_vectors()
        attend((0, 1), None, no_side, lambda m, gates: residual((0, 0), m, gates))

    def attend_tiles():
        def body(i, carry):
            start = attend((i, 0), None, finishing((i - 1, 0)),
                           lambda m, gates: residual((i - 1, 1), m, gates))
            attend((i, 1), start, finishing((i - 1, 1)),
                   lambda m, gates: residual((i, 0), m, gates))
            out_copy(i - 1).start()
            return carry
        lax.fori_loop(1, last + 1, body, 0)

    def last_tile():
        gates, start = [], None
        for m in range(n_chunks):
            gates = spill_over(gates) + finishing((last, 0))(m, start)
            start = residual((last, 1), m, gates)
        for g in range(TILE // 16):
            finish((last, 1), g)
        out_copy(last).start()

    def route():
        scores = r_v[...]
        row = lax.broadcasted_iota(I32, scores.shape, 0)
        lane = lax.broadcasted_iota(I32, scores.shape, 1)
        index = jnp.where(lane < TILE // 8, (row // 8) * TILE + lane * 8 + row % 8, seq)

        def arg_top(valid):
            best = jnp.max(jnp.where(valid, scores, -jnp.inf))
            first = jnp.min(jnp.where(valid & (scores == best), index, seq).astype(F32))
            return jnp.minimum(first.astype(I32), seq - 1)

        i0 = arg_top(index < seq)
        i1 = arg_top((index < seq) & (index != i0))

        sub = lax.broadcasted_iota(I32, (16, d), 0)
        def residual_row(i):
            local = pl.ds((i // (2 * TILE)) * TILE + i % TILE, 1)
            return jnp.where((i // TILE) % 2 == 0, x1_v[0][local, :], x1_v[1][local, :])

        x1 = jnp.where(sub == 0, residual_row(i0), residual_row(i1))
        xc, rstd = _centered(x1)
        h2 = xc * rstd * _rows(vec(SCALE_B), 16) + _rows(vec(SHIFT_B), 16)
        gate = _sigmoid(jnp.sum(h2 * _rows(vec(ROUTER), 16), axis=-1, keepdims=True))
        xs = h2.astype(BF16)
        for cp in (wg_cp, wu_cp, wd_cp):
            cp.wait()
        g = _dot(xs, wg_v[...])
        u = _dot(xs, wu_v[...])
        y = _dot((g * _sigmoid(g) * u).astype(BF16), wd_v[...])
        routed = x1 + _rows(vec(GATE_B), 16) * (h2 + y * gate)

        for i in range(last + 1):
            out_copy(i).wait()

        def patch(k, i):
            base = pl.multiple_of((i // 16) * 16, 16)
            old = out_v[pl.ds(base, 16), :].astype(F32)
            out_v[pl.ds(base, 16), :] = jnp.where(
                sub == i - base, routed[k:k + 1], old).astype(BF16)
            return base, copy(out_v.at[pl.ds(base, 16)], out_hbm.at[pl.ds(base, 16)],
                              sem.at[16 + k])

        base0, patch0 = patch(0, i0)
        base1, patch1 = patch(1, i1)
        patch0.start()

        @pl.when(base1 != base0)
        def _():
            patch1.start()
            patch1.wait()

        patch0.wait()

    for cp in (c_cp, wphi_cp, wk_cp, x0_cp, scale_cp, shift_cp, wv_cp, x1_cp):
        cp.start()
    kv_v[...] = jnp.zeros(kv_v.shape, F32)
    z_v[...] = jnp.zeros(z_v.shape, F32)
    r_v[...] = jnp.full(r_v.shape, -jnp.inf, F32)
    c_cp.wait()
    words = pltpu.bitcast(jnp.broadcast_to(c_v[:, :128].astype(F32), (8, 128)), I32)
    zero_v[...] = jnp.minimum(lax.shift_right_logical(words, 1), 0)
    steps = (prologue, first_tile, summarize_tiles, last_summary, first_read_outs, attend_tiles,
             last_tile, route)
    for k, step in enumerate(steps):
        if ONLY is None or ONLY == k:
            with _scope(step.__name__):
                step()


@jax.jit
def pallas_adaLN_cond__linear_kernel_hedgehog__moe_arch_mod__prompt_kernel(
    A_x: jax.Array,
    A_wqkv: jax.Array,
    A_w_phi: jax.Array,
    A_wo: jax.Array,
    B_x: jax.Array,
    B_w_r: jax.Array,
    B_w_gate: jax.Array,
    B_w_up: jax.Array,
    B_w_down: jax.Array,
    c: jax.Array,
    w_mod: jax.Array,
):
    del B_x
    batch, seq, d = A_x.shape
    assert batch == 1 and d == HEADS * HEAD_DIM and seq == 8 * TILE
    n_tiles = seq // TILE
    operands = (A_x.reshape(seq, d), A_wqkv, A_w_phi, A_wo, B_w_r, B_w_gate, B_w_up, B_w_down,
                c, w_mod)
    weight_terms = pltpu.VMEM((TERMS * d // 4, d // 2), I32)
    scratch = [pltpu.VMEM(a.shape, a.dtype) for a in operands] + [
        weight_terms, weight_terms, weight_terms, weight_terms,
        [pltpu.VMEM((n_tiles // 2 * TERMS * HALF // 2, d // 2), I32)] * 2,
        [pltpu.VMEM((TERMS * HALF // 2, d // 2), I32)] * 2,
        [pltpu.VMEM((seq // 2, d), F32)] * 2,
        pltpu.VMEM((8, 10 * d), F32),
        pltpu.VMEM((HEADS // 2 * PAIR, 128), F32),
        pltpu.VMEM((HEADS // 2 * HEAD_DIM, 128), I32),
        pltpu.VMEM((HEADS // 2 * 128, 128), F32),
        pltpu.VMEM((seq, d), BF16),
        pltpu.VMEM((n_tiles * 8, 128), F32),
        pltpu.VMEM((8, 128), I32),
        pltpu.SemaphoreType.DMA((18,)),
        pltpu.SemaphoreType.DMA((n_tiles // 2,)),
    ]
    out = pl.pallas_call(
        _kernel,
        out_shape=jax.ShapeDtypeStruct((seq, d), A_x.dtype),
        in_specs=[pl.BlockSpec(memory_space=pl.ANY)] * len(operands),
        out_specs=pl.BlockSpec(memory_space=pl.ANY),
        scratch_shapes=scratch,
        compiler_params=pltpu.CompilerParams(vmem_limit_bytes=110 * 2**20, flags=FLAGS or None),
        name="adaln_hedgehog_mod",
    )(*operands)
    return out.reshape(batch, seq, d)
```

```python
import contextlib
import functools
import math

import jax
import jax.numpy as jnp
from jax import lax
import jax.experimental.pallas as pl
import jax.experimental.pallas.tpu as pltpu

F32 = jnp.float32
BF16 = jnp.bfloat16
I32 = jnp.int32

HEADS = 32
HEAD_DIM = 32
PAIR = 2 * HEAD_DIM
TERMS = 7
LN_EPS = 1e-5
DEN_EPS = 1e-6
LOG2E = math.log2(math.e)

TILE = 256
HALF = TILE // 2
CHUNK = 128
SCOPES = True
ONLY = None
LN_PLAN = ((0, 1, 2), (3, 4, 5), (6, 7), ())
TR_PLAN = ((), (), (), (0, 1, 2, 3, 4, 5, 6))
LN_GATE = 7
FFN_CHUNK = 512
FIRST_SPLIT = True
FIN_GATES = (4, 4, 7, 7)
PIN_START = True
FLAGS = {"XLA_TPU_EVENLY_DISTRIBUTE_CRITICAL_NODES": True}

NT_DIMS = (((1,), (1,)), ((), ()))


def _scope(name):
    return jax.named_scope(name) if SCOPES else contextlib.nullcontext()


def _dot(a, b):
    return jnp.dot(a, b, preferred_element_type=F32)


def _dot_nt(a, b):
    return lax.dot_general(a, b, NT_DIMS, preferred_element_type=F32)


def _pack(v):
    return pltpu.bitcast(v.astype(BF16), I32)


def _pack_heads(v):
    starts = range(0, v.shape[0], PAIR)
    first = jnp.concatenate([v[s:s + HEAD_DIM] for s in starts], axis=0)
    second = jnp.concatenate([v[s + HEAD_DIM:s + PAIR] for s in starts], axis=0)
    return pltpu.pack_elementwise([first, second], packed_dtype=BF16).astype(I32)


def _unpack(v):
    return pltpu.bitcast(v, BF16)


def _recip(d):
    r = pltpu.reciprocal(d, approx=True)
    return r * (2.0 - d * r)


def _sigmoid(v):
    return 1.0 / (1.0 + jnp.exp(-v))


def _rows(v, n):
    return jnp.concatenate([v] * (n // 8), axis=0) if n > 8 else v


def _centered(x, after=None):
    inv_d = 1.0 / x.shape[-1]
    if after is not None:
        head = x[:, :128] + _rows(pltpu.bitcast(after, F32), x.shape[0])
        x = jnp.concatenate([head, x[:, 128:]], axis=1)
    xc = x - jnp.sum(x, axis=-1, keepdims=True) * inv_d
    var = jnp.sum(xc * xc, axis=-1, keepdims=True) * inv_d
    return xc, lax.rsqrt(var + LN_EPS)


def _lhs_terms(a11, a12, a21, a22):
    return [a11 + a22, a21 + a22, a11, a22, a11 + a12, a21 - a11, a12 - a22]


def _rhs_terms(b11, b12, b21, b22):
    return [b11 + b22, b11, b12 - b22, b21 - b11, b22, b11 + b12, b21 + b22]


def _block_matmul(product):
    m1 = product(0, 0)
    m4 = product(1, 3)
    c11 = m1 + m4
    c11 = c11 + product(2, 6)
    m5 = product(3, 4)
    c11 = c11 - m5
    m3 = product(4, 2)
    c12 = m3 + m5
    c22 = m1 + m3
    m2 = product(5, 1)
    c21 = m2 + m4
    c22 = c22 - m2
    c22 = c22 + product(6, 5)
    return c11, c12, c21, c22


def _head_reduce(op, tiles):
    while len(tiles) > 1:
        tiles = [op(tiles[i], tiles[i + 1]) for i in range(0, len(tiles), 2)]
    m = tiles[0]
    m = op(m, pltpu.roll(m, 4, 0))
    return op(m, pltpu.roll(m, 2, 0))


def _feature_map(p):
    tiles = [p[8 * j:8 * j + 8] for j in range(PAIR // 8)]
    hi = _head_reduce(jnp.maximum, tiles)
    lo = _head_reduce(jnp.minimum, tiles)
    e_pos = [jnp.exp2(t - hi) for t in tiles]
    e_neg = [jnp.exp2(lo - t) for t in tiles]
    r_pos = _recip(_head_reduce(jnp.add, e_pos))
    r_neg = _recip(_head_reduce(jnp.add, e_neg))
    return [e * r_pos for e in e_pos] + [e * r_neg for e in e_neg]


SHIFT_A, SCALE_A, GATE_A, SHIFT_B, SCALE_B, GATE_B, ROUTER, OUT_SCALE, OUT_SHIFT, SCORE = range(10)


def _kernel(x_hbm, wqkv_hbm, wphi_hbm, wo_hbm, wr_hbm, wg_hbm, wu_hbm, wd_hbm, c_hbm, wmod_hbm,
            out_hbm,
            x_v, wqkv_v, wphi_v, wo_v, wr_v, wg_v, wu_v, wd_v, c_v, wmod_v,
            wq_s, wk_s, wv_s, wo_s, n_s, h_s, o_s, x1_v, mod_v, kv_v, kvm_v, z_v, out_v, r_v, zero_v, act_v, phi_s,
            sem, out_sem):
    seq, d = x_v.shape
    hd = d // 2
    n_tiles = seq // TILE
    n_pairs = HEADS // 2
    n_chunks = hd // CHUNK
    chunk_pairs = CHUNK // PAIR
    h_rows = HALF // 2
    w_rows = hd // 2

    def copy(src, dst, s):
        return pltpu.make_async_copy(src, dst, s)

    def rows(start, size):
        return pl.ds(start if isinstance(start, int) else pl.multiple_of(start, 8), size)

    def token_rows(start, size):
        return pl.ds(start if isinstance(start, int) else pl.multiple_of(start, 16), size)

    def token_copy(src, dst, first, count, s):
        span = pl.ds(first if isinstance(first, int) else pl.multiple_of(first, TILE), count)
        return copy(src.at[span], dst.at[span], s)

    def cols(ref, i, n=1):
        return ref.at[:, pl.ds(i * d, n * d)]

    c_cp = copy(c_hbm, c_v, sem.at[0])
    wphi_cp = copy(wphi_hbm, wphi_v, sem.at[1])
    wr_cp = copy(wr_hbm, wr_v, sem.at[2])
    mod_a_cps = [copy(wmod_hbm.at[:, pl.ds(j * hd, hd)], wmod_v.at[:, pl.ds(j * hd, hd)],
                      sem.at[18 + j]) for j in range(4)]
    mod_b_cp = copy(cols(wmod_hbm, 2, 4), cols(wmod_v, 2, 4), sem.at[5])
    wq_cp = copy(cols(wqkv_hbm, 0), cols(wqkv_v, 0), sem.at[6])
    wk_cp = copy(cols(wqkv_hbm, 1), cols(wqkv_v, 1), sem.at[7])
    wv_cp = copy(cols(wqkv_hbm, 2), cols(wqkv_v, 2), sem.at[8])
    wo_cp = copy(wo_hbm, wo_v, sem.at[9])
    wg_cp = copy(wg_hbm, wg_v, sem.at[10])
    wu_cp = copy(wu_hbm, wu_v, sem.at[11])
    wd_cp = copy(wd_hbm, wd_v, sem.at[12])
    x0_cp = token_copy(x_hbm, x_v, 0, TILE, sem.at[13])
    x1_cp = token_copy(x_hbm, x_v, TILE, TILE, sem.at[14])
    x_rest_cp = token_copy(x_hbm, x_v, 2 * TILE, seq - 2 * TILE, sem.at[15])

    def first_token(t):
        return (2 * t[0] + t[1]) * TILE

    def out_copy(i):
        return token_copy(out_v, out_hbm, first_token((i, 0)), 2 * TILE, out_sem.at[i])

    def token(values):
        tiles = [pltpu.bitcast(v[r:r + 8, c:c + 128], I32) for v in values
                 for r in range(0, v.shape[0], 8) for c in range(0, v.shape[1], 128)]
        while len(tiles) > 1:
            tiles = [tiles[j] | tiles[j + 1] if j + 1 < len(tiles) else tiles[j]
                     for j in range(0, len(tiles), 2)]
        return tiles[0] & zero_v[...]

    def gated(w, gates, step):
        for before, zero in gates:
            if before == step:
                top = jnp.concatenate([w[:8, :128] | zero, w[:8, 128:]], axis=1)
                w = jnp.concatenate([top, w[8:]], axis=0)
        return w

    def spill_over(gates):
        return [(before - TERMS, zero) for before, zero in gates if before >= TERMS]

    def store_terms(dst, g, terms):
        packed = [_pack_heads(term) for term in terms]
        for i, term in enumerate(packed):
            dst[i * w_rows + g * 64:i * w_rows + (g + 1) * 64, :] = term
        return token([term[-8:] for term in packed])

    def store_lhs_terms(dst, g, group):
        top, bottom = group(g), group(g + hd // 128)
        return store_terms(
            dst, g, _lhs_terms(top[:, :hd], top[:, hd:], bottom[:, :hd], bottom[:, hd:]))

    def feature_blocks():
        row = lax.broadcasted_iota(I32, (128, 128), 0)
        lane = lax.broadcasted_iota(I32, (128, 128), 1)
        same_head = row // HEAD_DIM == lane // HEAD_DIM
        row_f = lax.broadcasted_iota(I32, (128, HEAD_DIM), 0)
        lane_f = lax.broadcasted_iota(I32, (128, HEAD_DIM), 1)
        pick = jnp.where(row_f % HEAD_DIM == lane_f, 1.0, 0.0).astype(BF16)
        for g in range(d // 128):
            wphi = wphi_v[4 * g:4 * g + 4].reshape(128, HEAD_DIM)
            phi_s[g * 64:(g + 1) * 64, :] = _pack(jnp.where(same_head, _dot_nt(pick, wphi), 0.0))

    def fold(col, dst, g):
        def group(g):
            w = wqkv_v[:, col * d + g * 128:col * d + (g + 1) * 128]
            return _dot_nt(_unpack(phi_s[g * 64:(g + 1) * 64, :]), w) * LOG2E

        return store_lhs_terms(dst, g, group)

    def value_terms(g):
        return store_lhs_terms(
            wv_s, g, lambda g: wqkv_v[:, 2 * d + g * 128:2 * d + (g + 1) * 128].astype(F32).T)

    def output_terms(g):
        top = wo_v[g * 128:(g + 1) * 128, :].astype(F32)
        bottom = wo_v[hd + g * 128:hd + (g + 1) * 128, :].astype(F32)
        return store_terms(
            wo_s, g, _rhs_terms(top[:, :hd], top[:, hd:], bottom[:, :hd], bottom[:, hd:]))

    def vec(i):
        return mod_v[:, i * d:(i + 1) * d]

    def modulation(c0):
        m = _dot(_unpack(act_v[...]), wmod_v[:, c0:c0 + hd])[0:8]
        mod_v[:, c0:c0 + hd] = 1.0 + m if c0 // d in (SCALE_A, SCALE_B) else m

    def modulation_rounds(i):
        partial = {}

        def one(c0, half):
            span = slice(half * hd, (half + 1) * hd)
            m = _dot(_unpack(act_v[:, span]), wmod_v[span, c0:c0 + 128])[0:8]
            if half == 0:
                partial[c0] = 1.0 + m if i in (SCALE_A, SCALE_B) else m
            else:
                mod_v[:, c0:c0 + 128] = partial[c0] + m

        return [functools.partial(one, c0, half)
                for c0 in range(i * d, (i + 1) * d, 128) for half in range(2)]

    def derived_vectors():
        router = jnp.broadcast_to(wr_v[...].astype(F32).reshape(1, d), (8, d))
        for i, v in ((ROUTER, router), (OUT_SCALE, vec(GATE_B) * vec(SCALE_B)),
                     (OUT_SHIFT, vec(GATE_B) * vec(SHIFT_B)), (SCORE, router * vec(SCALE_B))):
            mod_v[:, i * d:(i + 1) * d] = v

    def normed_rows(t, r0, after=None):
        xc, rstd = _centered(x_v[token_rows(first_token(t) + r0, 16), :].astype(F32), after)
        return xc * rstd

    def normed_piece(t, k, after=None, normed_rows=normed_rows):
        def normed(start):
            xn = normed_rows(t, start + 16 * k, after)
            return xn * _rows(vec(SCALE_A), 16) + _rows(vec(SHIFT_A), 16)

        ha, hb = normed(0), normed(HALF)
        packed = [_pack(term)
                  for term in _rhs_terms(ha[:, :hd], hb[:, :hd], ha[:, hd:], hb[:, hd:])]
        for j, term in enumerate(packed):
            n_s[j * h_rows + 8 * k:j * h_rows + 8 * k + 8, :] = term
        return token(packed)

    def transposed_term(t, j):
        term = pltpu.bitcast(_unpack(n_s[j * h_rows:(j + 1) * h_rows, :]).T, I32)
        h_s[t[1]][rows((t[0] * TERMS + j) * w_rows, w_rows), :] = term
        return token([term[r:r + 8] for r in range(56, w_rows, 64)])

    fillers = []

    def fill():
        if fillers:
            fillers.pop(0)()

    def project(w_s, t, m, gates=()):
        def product(step, j):
            w = w_s[j * w_rows + m * CHUNK // 2:j * w_rows + (m + 1) * CHUNK // 2, :]
            h = h_s[t[1]][rows((t[0] * TERMS + j) * w_rows, w_rows), :]
            out = _dot(_unpack(gated(w, gates, step)), _unpack(h))
            fill()
            return out

        c11, c12, c21, c22 = _block_matmul(product)
        halves = (jnp.concatenate([c11, c12], axis=1), jnp.concatenate([c21, c22], axis=1))
        return [(side * (n_pairs // 2) + m * chunk_pairs + j, block[j * PAIR:(j + 1) * PAIR])
                for side, block in enumerate(halves) for j in range(chunk_pairs)]

    def key_features(pk):
        out = []
        for p, pk_p in pk:
            phi = jnp.concatenate(_feature_map(pk_p), axis=0)
            z_v[p * 128:(p + 1) * 128, :] += phi[:, :HALF] + phi[:, HALF:]
            out.append(phi.astype(BF16))
        return out

    def accumulate_kv(phi, v):
        for phi_p, (p, v_p) in zip(phi, v):
            kv_v[p * PAIR:(p + 1) * PAIR, :] += _dot_nt(v_p.astype(BF16), phi_p)

    def summarize(t, state, side):
        pending, start = state
        for m in range(n_chunks):
            gates = side(m, start)
            pk = project(wk_s, t, m, gates)
            if pending is not None:
                accumulate_kv(*pending)
            v = project(wv_s, t, m, spill_over(gates))
            pending = (key_features(pk), v)
            start = token([v[-1][1][-8:, -128:]]) if PIN_START else None
        return pending, start

    def normalize(t):
        def pieces(m, after=None):
            span = range(m * 4 // n_chunks, (m + 1) * 4 // n_chunks)
            done = [normed_piece(t, k, after) for j in span for k in LN_PLAN[j]]
            done += [transposed_term(t, k) for j in span for k in TR_PLAN[j]]
            return [(LN_GATE, zero) for zero in done]
        return pieces

    def read_out(t, m, pq):
        o_t = []
        for p, pq_p in pq:
            phi = _feature_map(pq_p)
            z = [z_v[p * 128 + 8 * j:p * 128 + 8 * j + 8, :] for j in range(len(phi))]
            den = _head_reduce(
                jnp.add, [f * jnp.concatenate([zj, zj], axis=1) for f, zj in zip(phi, z)])
            num = _dot(_unpack(kvm_v[p * HEAD_DIM:(p + 1) * HEAD_DIM, :]),
                       jnp.concatenate(phi, axis=0).astype(BF16))
            o_t.append(num * _rows(_recip(den + DEN_EPS), PAIR))
        top = jnp.concatenate(o_t[:chunk_pairs], axis=0)
        bottom = jnp.concatenate(o_t[chunk_pairs:], axis=0)
        terms = _lhs_terms(top[:, :HALF], bottom[:, :HALF], top[:, HALF:], bottom[:, HALF:])
        for j, term in enumerate(terms):
            o_s[t[1]][j * h_rows:(j + 1) * h_rows, m * CHUNK:(m + 1) * CHUNK] = pltpu.bitcast(
                term.astype(BF16).T, I32)

    def residual(t, g, gates=()):
        def product(step, j):
            o = o_s[t[1]][j * h_rows:(j + 1) * h_rows, :]
            w = wo_s[j * w_rows:(j + 1) * w_rows, g * 128:(g + 1) * 128]
            out = _dot(_unpack(gated(o, gates, step)), _unpack(w))
            fill()
            return out

        for b, attn in enumerate(_block_matmul(product)):
            r0 = (b // 2) * HALF
            c0 = (b % 2) * hd + g * 128
            gate = _rows(mod_v[:, GATE_A * d + c0:GATE_A * d + c0 + 128], HALF)
            x = x_v[token_rows(first_token(t) + r0, HALF), c0:c0 + 128].astype(F32)
            x1_v[t[1]][rows(t[0] * TILE + r0, HALF), c0:c0 + 128] = x + gate * attn
        return token([attn[-8:]])

    def finish(t, g, after=None):
        x1 = x1_v[t[1]][rows(t[0] * TILE + 16 * g, 16), :]
        xc, rstd = _centered(x1, after)
        out = x1 + (xc * rstd * _rows(vec(OUT_SCALE), 16) + _rows(vec(OUT_SHIFT), 16))
        out_v[token_rows(first_token(t) + 16 * g, 16), :] = out.astype(BF16)
        score = jnp.sum(xc * _rows(vec(SCORE), 16), axis=-1, keepdims=True) * rstd
        lane = lax.broadcasted_iota(I32, (8, 128), 1)
        slot = rows((2 * t[0] + t[1]) * 8, 8)
        packed = r_v[slot, :]
        for s in range(2):
            packed = jnp.where(lane == 2 * g + s, score[8 * s:8 * s + 8], packed)
        r_v[slot, :] = packed
        return token([packed, out[:, -128:]])

    def finishing(t):
        def pieces(m, after=None):
            return [(before, finish(t, 4 * m + j, after)) for j, before in enumerate(FIN_GATES)]
        return pieces

    def no_side(m, after=None):
        return []

    def attend(t, start, side, middle):
        gates = side(0, start)
        pq = project(wq_s, t, 0, gates)
        for m in range(n_chunks):
            ahead = None
            if m + 1 < n_chunks:
                start = token([pq[-1][1][-8:, -128:]]) if m == 0 else start
                gates = spill_over(gates) + side(m + 1, start if PIN_START else None)
                ahead = project(wq_s, t, m + 1, gates)
                start = middle(m, spill_over(gates))
                gates = []
                read_out(t, m, pq)
            else:
                read_out(t, m, pq)
                start = middle(m, [])
            pq = ahead
        return start if PIN_START else None

    def prologue():
        cf = c_v[...].astype(F32)
        act_v[...] = _pack(jnp.broadcast_to(cf * _sigmoid(cf), (16, d)))
        wphi_cp.wait()
        feature_blocks()
        x0_cp.wait()
        mod_a_cps[0].start()
        for r0 in range(0, TILE, 16):
            x1_v[0][r0:r0 + 16, :] = normed_rows((0, 0), r0)
        wk_cp.wait()
        mod_a_cps[1].start()
        for g in range(n_chunks):
            fold(1, wk_s, g)
            if g == 1:
                mod_a_cps[2].start()
        for cp, j, ahead in zip(mod_a_cps, range(4), (mod_a_cps[3], wv_cp, x1_cp, None)):
            cp.wait()
            if ahead is not None:
                ahead.start()
            modulation(j * hd)
        for k in range(HALF // 16):
            normed_piece((0, 0), k, normed_rows=lambda t, r0, after: x1_v[0][r0:r0 + 16, :])
        for j in range(TERMS):
            transposed_term((0, 0), j)

    def first_tile():
        phi, gates = [], []
        for m in range(n_chunks):
            if m == 2:
                wv_cp.wait()
                for cp in (x_rest_cp, wq_cp, wo_cp, wr_cp, mod_b_cp):
                    cp.start()
            phi.append(key_features(project(wk_s, (0, 0), m, gates)))
            if m >= 2:
                gates = [(0, value_terms(m - 2))]
        x1_cp.wait()
        pending, start = None, None
        for m in range(n_chunks):
            v = project(wv_s, (0, 0), m, gates)
            gates = [(0, zero) for _, zero in normalize((0, 1))(m, start)]
            if m + 2 < n_chunks:
                gates.append((0, value_terms(m + 2)))
            if pending is not None:
                accumulate_kv(*pending)
            pending = (phi[m], v)
            start = token([v[-1][1][-8:, -128:]])
        accumulate_kv(*pending)
        x_rest_cp.wait()

    last = n_tiles // 2 - 1

    def summarize_tiles():
        def body(i, carry):
            for step, cp in enumerate((wg_cp, wu_cp, wd_cp)):
                pl.when(i == step)(cp.start)
            state = summarize((i, 1), (None, None), normalize((i + 1, 0)))
            state = summarize((i + 1, 0), state, normalize((i + 1, 1)))
            accumulate_kv(*state[0])
            return carry
        lax.fori_loop(0, last, body, 0)

    def last_summary():
        for cp in (wq_cp, wo_cp, wr_cp, mod_b_cp):
            cp.wait()

        def prepare(m, after):
            fold(0, wq_s, m)
            return [(LN_GATE, output_terms(m))]

        accumulate_kv(*summarize((last, 1), (None, None), prepare)[0])

    def first_read_outs():
        row = lax.broadcasted_iota(I32, (PAIR, 128), 0)
        lane = lax.broadcasted_iota(I32, (PAIR, 128), 1)
        for p in range(n_pairs):
            kv = jnp.where(row % 2 == lane % 2, kv_v[p * PAIR:(p + 1) * PAIR, :], 0.0)
            kvm_v[p * HEAD_DIM:(p + 1) * HEAD_DIM, :] = _pack(kv)
            z = jnp.sum(z_v[p * 128:(p + 1) * 128, :], axis=1, keepdims=True)
            z_v[p * 128:(p + 1) * 128, :] = jnp.broadcast_to(z, (128, 128))
        for i in (GATE_A, SHIFT_B, SCALE_B, GATE_B):
            fillers.extend(modulation_rounds(i))
        attend((0, 0), None, no_side, lambda m, gates: None)
        attend((0, 1), None, no_side, lambda m, gates: residual((0, 0), m, gates))
        assert not fillers
        derived_vectors()

    def attend_tiles():
        def body(i, carry):
            start = attend((i, 0), None, finishing((i - 1, 0)),
                           lambda m, gates: residual((i - 1, 1), m, gates))
            attend((i, 1), start, finishing((i - 1, 1)),
                   lambda m, gates: residual((i, 0), m, gates))
            out_copy(i - 1).start()
            return carry
        lax.fori_loop(1, last + 1, body, 0)

    def last_tile():
        gates, start = [], None
        for m in range(n_chunks):
            gates = spill_over(gates) + finishing((last, 0))(m, start)
            start = residual((last, 1), m, gates)
        for g in range(TILE // 16):
            finish((last, 1), g)
        out_copy(last).start()

    def route():
        scores = r_v[...]
        row = lax.broadcasted_iota(I32, scores.shape, 0)
        lane = lax.broadcasted_iota(I32, scores.shape, 1)
        index = jnp.where(lane < TILE // 8, (row // 8) * TILE + lane * 8 + row % 8, seq)

        def arg_top(valid):
            best = jnp.max(jnp.where(valid, scores, -jnp.inf))
            first = jnp.min(jnp.where(valid & (scores == best), index, seq).astype(F32))
            return jnp.minimum(first.astype(I32), seq - 1)

        i0 = arg_top(index < seq)
        i1 = arg_top((index < seq) & (index != i0))

        sub = lax.broadcasted_iota(I32, (16, d), 0)
        def residual_row(i):
            local = pl.ds((i // (2 * TILE)) * TILE + i % TILE, 1)
            return jnp.where((i // TILE) % 2 == 0, x1_v[0][local, :], x1_v[1][local, :])

        x1 = jnp.where(sub == 0, residual_row(i0), residual_row(i1))
        xc, rstd = _centered(x1)
        h2 = xc * rstd * _rows(vec(SCALE_B), 16) + _rows(vec(SHIFT_B), 16)
        gate = _sigmoid(jnp.sum(h2 * _rows(vec(ROUTER), 16), axis=-1, keepdims=True))
        xs = h2.astype(BF16)
        for cp in (wg_cp, wu_cp, wd_cp):
            cp.wait()
        spans = [slice(f, f + FFN_CHUNK) for f in range(0, wd_v.shape[0], FFN_CHUNK)]
        y, hidden = 0.0, None
        for k in range(len(spans) + 1):
            if k < len(spans):
                g = _dot(xs, wg_v[:, spans[k]])
                u = _dot(xs, wu_v[:, spans[k]])
            if k > 0:
                y = y + _dot(hidden, wd_v[spans[k - 1], :])
            hidden = (g * _sigmoid(g) * u).astype(BF16)
        routed = x1 + _rows(vec(GATE_B), 16) * (h2 + y * gate)

        for i in range(last + 1):
            out_copy(i).wait()

        def patch(k, i):
            base = pl.multiple_of((i // 16) * 16, 16)
            old = out_v[pl.ds(base, 16), :].astype(F32)
            out_v[pl.ds(base, 16), :] = jnp.where(
                sub == i - base, routed[k:k + 1], old).astype(BF16)
            return base, copy(out_v.at[pl.ds(base, 16)], out_hbm.at[pl.ds(base, 16)],
                              sem.at[16 + k])

        base0, patch0 = patch(0, i0)
        base1, patch1 = patch(1, i1)
        patch0.start()

        @pl.when(base1 != base0)
        def _():
            patch1.start()
            patch1.wait()

        patch0.wait()

    for cp in (c_cp, wphi_cp, x0_cp, wk_cp):
        cp.start()
    kv_v[...] = jnp.zeros(kv_v.shape, F32)
    z_v[...] = jnp.zeros(z_v.shape, F32)
    r_v[...] = jnp.full(r_v.shape, -jnp.inf, F32)
    c_cp.wait()
    words = pltpu.bitcast(jnp.broadcast_to(c_v[:, :128].astype(F32), (8, 128)), I32)
    zero_v[...] = jnp.minimum(lax.shift_right_logical(words, 1), 0)
    steps = (prologue, first_tile, summarize_tiles, last_summary, first_read_outs, attend_tiles,
             last_tile, route)
    for k, step in enumerate(steps):
        if ONLY is None or ONLY == k:
            with _scope(step.__name__):
                step()


@jax.jit
def pallas_adaLN_cond__linear_kernel_hedgehog__moe_arch_mod__prompt_kernel(
    A_x: jax.Array,
    A_wqkv: jax.Array,
    A_w_phi: jax.Array,
    A_wo: jax.Array,
    B_x: jax.Array,
    B_w_r: jax.Array,
    B_w_gate: jax.Array,
    B_w_up: jax.Array,
    B_w_down: jax.Array,
    c: jax.Array,
    w_mod: jax.Array,
):
    del B_x
    batch, seq, d = A_x.shape
    assert batch == 1 and d == HEADS * HEAD_DIM and seq == 8 * TILE
    n_tiles = seq // TILE
    operands = (A_x.reshape(seq, d), A_wqkv, A_w_phi, A_wo, B_w_r, B_w_gate, B_w_up, B_w_down,
                c, w_mod)
    weight_terms = pltpu.VMEM((TERMS * d // 4, d // 2), I32)
    scratch = [pltpu.VMEM(a.shape, a.dtype) for a in operands] + [
        weight_terms, weight_terms, weight_terms, weight_terms,
        pltpu.VMEM((TERMS * HALF // 2, d // 2), I32),
        [pltpu.VMEM((n_tiles // 2 * TERMS * d // 4, HALF), I32)] * 2,
        [pltpu.VMEM((TERMS * HALF // 2, d // 2), I32)] * 2,
        [pltpu.VMEM((seq // 2, d), F32)] * 2,
        pltpu.VMEM((8, 10 * d), F32),
        pltpu.VMEM((HEADS // 2 * PAIR, 128), F32),
        pltpu.VMEM((HEADS // 2 * HEAD_DIM, 128), I32),
        pltpu.VMEM((HEADS // 2 * 128, 128), F32),
        pltpu.VMEM((seq, d), BF16),
        pltpu.VMEM((n_tiles * 8, 128), F32),
        pltpu.VMEM((8, 128), I32),
        pltpu.VMEM((8, d), I32),
        pltpu.VMEM((d // 2, 128), I32),
        pltpu.SemaphoreType.DMA((22,)),
        pltpu.SemaphoreType.DMA((n_tiles // 2,)),
    ]
    out = pl.pallas_call(
        _kernel,
        out_shape=jax.ShapeDtypeStruct((seq, d), A_x.dtype),
        in_specs=[pl.BlockSpec(memory_space=pl.ANY)] * len(operands),
        out_specs=pl.BlockSpec(memory_space=pl.ANY),
        scratch_shapes=scratch,
        compiler_params=pltpu.CompilerParams(vmem_limit_bytes=110 * 2**20, flags=FLAGS or None),
        name="adaln_hedgehog_mod",
    )(*operands)
    return out.reshape(batch, seq, d)
```

```python
import collections
import contextlib
import functools
import math

import jax
import jax.numpy as jnp
from jax import lax
import jax.experimental.pallas as pl
import jax.experimental.pallas.tpu as pltpu

F32 = jnp.float32
BF16 = jnp.bfloat16
I32 = jnp.int32

HEADS = 32
HEAD_DIM = 32
PAIR = 2 * HEAD_DIM
TERMS = 7
LN_EPS = 1e-5
DEN_EPS = 1e-6
LOG2E = math.log2(math.e)

TILE = 256
HALF = TILE // 2
CHUNK = 128
SCOPES = True
FOLD_GAP = 6
OUT_WIN = tuple((55 + 14 * m, 55 + 14 * m + 14) for m in range(4))
WAIT_AT = (2, 5)
SPLIT = (1, 3)
EARLY_WIN = tuple((7 * n - 1, 7 * n + 13) for n in (0, 2, 4, 6, 8, 10, 12, 13))
ONLY = None
LN_WIN = (None,) * 8
TR_WIN = (None,) * 7
KF_WIN = None
QF_WIN = None
FIN_WIN = ((-1, 7),) * 6 + ((20, 28),) * 5 + ((34, 42),) * 5
FFN_CHUNK = 512
FLAGS = {"XLA_TPU_EVENLY_DISTRIBUTE_CRITICAL_NODES": True}

NT_DIMS = (((1,), (1,)), ((), ()))


def _scope(name):
    return jax.named_scope(name) if SCOPES else contextlib.nullcontext()


def _dot(a, b):
    return jnp.dot(a, b, preferred_element_type=F32)


def _dot_nt(a, b):
    return lax.dot_general(a, b, NT_DIMS, preferred_element_type=F32)


def _pack(v):
    return pltpu.bitcast(v.astype(BF16), I32)


def _pack_heads(v):
    starts = range(0, v.shape[0], PAIR)
    first = jnp.concatenate([v[s:s + HEAD_DIM] for s in starts], axis=0)
    second = jnp.concatenate([v[s + HEAD_DIM:s + PAIR] for s in starts], axis=0)
    return pltpu.pack_elementwise([first, second], packed_dtype=BF16).astype(I32)


def _unpack(v):
    return pltpu.bitcast(v, BF16)


def _recip(d):
    r = pltpu.reciprocal(d, approx=True)
    return r * (2.0 - d * r)


def _sigmoid(v):
    return 1.0 / (1.0 + jnp.exp(-v))


def _rows(v, n):
    return jnp.concatenate([v] * (n // 8), axis=0) if n > 8 else v


def _centered(x, after=None):
    inv_d = 1.0 / x.shape[-1]
    if after is not None:
        head = x[:, :128] + _rows(pltpu.bitcast(after, F32), x.shape[0])
        x = jnp.concatenate([head, x[:, 128:]], axis=1)
    xc = x - jnp.sum(x, axis=-1, keepdims=True) * inv_d
    var = jnp.sum(xc * xc, axis=-1, keepdims=True) * inv_d
    return xc, lax.rsqrt(var + LN_EPS)


def _lhs_terms(a11, a12, a21, a22):
    return [a11 + a22, a21 + a22, a11, a22, a11 + a12, a21 - a11, a12 - a22]


def _rhs_terms(b11, b12, b21, b22):
    return [b11 + b22, b11, b12 - b22, b21 - b11, b22, b11 + b12, b21 + b22]


def _block_matmul(product):
    m1 = product(0)
    m4 = product(3)
    c11 = m1 + m4
    c11 = c11 + product(6)
    m5 = product(4)
    c11 = c11 - m5
    m3 = product(2)
    c12 = m3 + m5
    c22 = m1 + m3
    m2 = product(1)
    c21 = m2 + m4
    c22 = c22 - m2
    c22 = c22 + product(5)
    return c11, c12, c21, c22


def _head_reduce(op, tiles):
    while len(tiles) > 1:
        tiles = [op(tiles[i], tiles[i + 1]) for i in range(0, len(tiles), 2)]
    m = tiles[0]
    m = op(m, pltpu.roll(m, 4, 0))
    return op(m, pltpu.roll(m, 2, 0))


def _feature_map(p):
    tiles = [p[8 * j:8 * j + 8] for j in range(PAIR // 8)]
    hi = _head_reduce(jnp.maximum, tiles)
    lo = _head_reduce(jnp.minimum, tiles)
    e_pos = [jnp.exp2(t - hi) for t in tiles]
    e_neg = [jnp.exp2(lo - t) for t in tiles]
    r_pos = _recip(_head_reduce(jnp.add, e_pos))
    r_neg = _recip(_head_reduce(jnp.add, e_neg))
    return [e * r_pos for e in e_pos] + [e * r_neg for e in e_neg]


Tile = collections.namedtuple("Tile", "x h h_all o x1 x1_all out r")
SHIFT_A, SCALE_A, GATE_A, SHIFT_B, SCALE_B, GATE_B, ROUTER, OUT_SCALE, OUT_SHIFT, SCORE = range(10)


def _kernel(x_hbm, wqkv_hbm, wphi_hbm, wo_hbm, wr_hbm, wg_hbm, wu_hbm, wd_hbm, c_hbm, wmod_hbm,
            out_hbm,
            x_v, wqkv_v, wphi_v, wo_v, wr_v, wg_v, wu_v, wd_v, c_v, wmod_v,
            wq_s, wk_s, wv_s, wo_s, n_s, h_s, h_all, o_s, x1_v, x1_all, mod_v, kv_v, kvm_v, z_v, out_v, r_v, zero_v, act_v, phi_s,
            sem, out_sem):
    seq, d = x_v.shape
    hd = d // 2
    n_tiles = seq // TILE
    n_pairs = HEADS // 2
    n_chunks = hd // CHUNK
    chunk_pairs = CHUNK // PAIR
    h_rows = HALF // 2
    w_rows = hd // 2

    def copy(src, dst, s):
        return pltpu.make_async_copy(src, dst, s)

    def token_copy(src, dst, first, count, s):
        return copy(src.at[pl.ds(first, count)], dst.at[pl.ds(first, count)], s)

    def cols(ref, i, n=1):
        return ref.at[:, pl.ds(i * d, n * d)]

    c_cp = copy(c_hbm, c_v, sem.at[0])
    wphi_cp = copy(wphi_hbm, wphi_v, sem.at[1])
    wr_cp = copy(wr_hbm, wr_v, sem.at[2])
    mod_b_cp = copy(cols(wmod_hbm, 2, 4), cols(wmod_v, 2, 4), sem.at[5])
    wq_cp = copy(cols(wqkv_hbm, 0), cols(wqkv_v, 0), sem.at[6])
    wo_cp = copy(wo_hbm, wo_v, sem.at[9])
    wg_cp = copy(wg_hbm, wg_v, sem.at[10])
    wu_cp = copy(wu_hbm, wu_v, sem.at[11])
    wd_cp = copy(wd_hbm, wd_v, sem.at[12])
    x_first_cp = token_copy(x_hbm, x_v, 0, 2 * TILE, sem.at[13])
    x_next_cp = token_copy(x_hbm, x_v, 2 * TILE, TILE, sem.at[14])
    x_rest_cp = token_copy(x_hbm, x_v, 3 * TILE, seq - 3 * TILE, sem.at[15])

    def kv_weight_copies(j):
        spans = [(pl.ds(half * hd + j * 128, 128), pl.ds(d, 2 * d)) for half in range(2)]
        return [copy(wqkv_hbm.at[span], wqkv_v.at[span], sem.at[18 + j]) for span in spans]

    def mod_a_copies(j):
        spans = [pl.ds(part * hd + j * 128, 128) for part in range(4)]
        return [copy(wmod_hbm.at[:, span], wmod_v.at[:, span], sem.at[22 + j]) for span in spans]

    def view(ref, index, size):
        start = index * size
        return ref.at[pl.ds(start if isinstance(start, int) else pl.multiple_of(start, size), size)]

    def tile(i, parity):
        t = 2 * i + parity
        return Tile(x=view(x_v, t, TILE), h=h_s[parity], h_all=view(h_all, t, TERMS * w_rows),
                    o=o_s[parity],
                    x1=x1_v[parity], x1_all=view(x1_all, t, TILE), out=view(out_v, t, TILE), r=view(r_v, t, 8))

    def out_copy(i):
        return copy(view(out_v, i, 2 * TILE), view(out_hbm, i, 2 * TILE), out_sem.at[i])

    def token(values):
        tiles = [pltpu.bitcast(v[r:r + 8, c:c + 128], I32) for v in values
                 for r in range(0, v.shape[0], 8) for c in range(0, v.shape[1], 128)]
        while len(tiles) > 1:
            tiles = [tiles[j] | tiles[j + 1] if j + 1 < len(tiles) else tiles[j]
                     for j in range(0, len(tiles), 2)]
        return tiles[0] & zero_v[...]

    clock = {"now": 0, "last": None, "jobs": {}, "gates": {}}

    def reset_clock():
        assert not clock["jobs"]
        clock.update(last=None, gates={})

    def run_job(job, after, end):
        zero = job(after)
        clock["gates"].setdefault(end, []).append(zero)

    def plan(job, window):
        if window is None:
            job(None)
            return
        start, end = (clock["now"] + w for w in window)
        if start < clock["now"]:
            run_job(job, clock["last"], end)
        else:
            clock["jobs"].setdefault(start, []).append((job, end))

    def timed_dot(lhs, rhs):
        for zero in clock["gates"].pop(clock["now"], []):
            top = jnp.concatenate([lhs[:8, :128] | zero, lhs[:8, 128:]], axis=1)
            lhs = jnp.concatenate([top, lhs[8:]], axis=0)
        out = _dot(_unpack(lhs), _unpack(rhs))
        clock["last"] = token([out[-8:]])
        for job, end in clock["jobs"].pop(clock["now"], []):
            run_job(job, clock["last"], end)
        clock["now"] += 1
        return out

    def store_terms(dst, g, c0, terms):
        packed = [_pack_heads(term) for term in terms]
        for i, term in enumerate(packed):
            dst[i * w_rows + g * 64:i * w_rows + (g + 1) * 64, c0:c0 + term.shape[1]] = term
        return packed

    def store_lhs_terms(dst, g, c0, group):
        top, bottom = group(g), group(g + hd // 128)
        n = top.shape[1] // 2
        return store_terms(
            dst, g, c0, _lhs_terms(top[:, :n], top[:, n:], bottom[:, :n], bottom[:, n:]))

    def feature_blocks():
        row = lax.broadcasted_iota(I32, (128, 128), 0)
        lane = lax.broadcasted_iota(I32, (128, 128), 1)
        same_head = row // HEAD_DIM == lane // HEAD_DIM
        row_f = lax.broadcasted_iota(I32, (128, HEAD_DIM), 0)
        lane_f = lax.broadcasted_iota(I32, (128, HEAD_DIM), 1)
        pick = jnp.where(row_f % HEAD_DIM == lane_f, 1.0, 0.0).astype(BF16)
        for g in range(d // 128):
            wphi = wphi_v[4 * g:4 * g + 4].reshape(128, HEAD_DIM)
            phi_s[g * 64:(g + 1) * 64, :] = _pack(jnp.where(same_head, _dot_nt(pick, wphi), 0.0))

    def folded(w, g):
        return _dot_nt(_unpack(phi_s[g * 64:(g + 1) * 64, :]), w) * LOG2E

    def weight_slice(col, j, g):
        span = slice(col * d + g * 128, col * d + (g + 1) * 128)
        return jnp.concatenate(
            [wqkv_v[half * hd + j * 128:half * hd + (j + 1) * 128, span] for half in range(2)],
            axis=0)

    def folded_terms(col, dst, j, g):
        store_lhs_terms(dst, g, j * 128, lambda g: folded(weight_slice(col, j, g), g))

    def output_terms(g, after):
        def rows(r0):
            words = pltpu.bitcast(wo_v[r0:r0 + 128, :], I32)
            words = words | jnp.concatenate([_rows(after, 64)] * (d // 128), axis=1)
            return _unpack(words).astype(F32)

        top, bottom = rows(g * 128), rows(hd + g * 128)
        packed = store_terms(
            wo_s, g, 0, _rhs_terms(top[:, :hd], top[:, hd:], bottom[:, :hd], bottom[:, hd:]))
        return token([term[-8:] for term in packed])

    def vec(i):
        return mod_v[:, i * d:(i + 1) * d]

    def modulation_rounds(i):
        partial = {}

        def one(c0, half):
            span = slice(half * hd, (half + 1) * hd)
            m = _dot(_unpack(act_v[:, span]), wmod_v[span, c0:c0 + 128])[0:8]
            if half == 0:
                partial[c0] = 1.0 + m if i in (SCALE_A, SCALE_B) else m
            else:
                mod_v[:, c0:c0 + 128] = partial[c0] + m

        return [functools.partial(one, c0, half)
                for c0 in range(i * d, (i + 1) * d, 128) for half in range(2)]

    def derived_vectors():
        router = jnp.broadcast_to(wr_v[...].astype(F32).reshape(1, d), (8, d))
        for i, v in ((ROUTER, router), (OUT_SCALE, vec(GATE_B) * vec(SCALE_B)),
                     (OUT_SHIFT, vec(GATE_B) * vec(SHIFT_B)), (SCORE, router * vec(SCALE_B))):
            mod_v[:, i * d:(i + 1) * d] = v

    def normed_rows(t, r0, after=None):
        xc, rstd = _centered(t.x[r0:r0 + 16, :].astype(F32), after)
        return xc * rstd

    def normed_piece(t, k, after=None):
        def normed(start):
            xn = normed_rows(t, start + 16 * k, after)
            return xn * _rows(vec(SCALE_A), 16) + _rows(vec(SHIFT_A), 16)

        ha, hb = normed(0), normed(HALF)
        packed = [_pack(term)
                  for term in _rhs_terms(ha[:, :hd], hb[:, :hd], ha[:, hd:], hb[:, hd:])]
        for j, term in enumerate(packed):
            n_s[j * h_rows + 8 * k:j * h_rows + 8 * k + 8, :] = term
        return token(packed)

    def transposed_term(t, j):
        term = pltpu.bitcast(_unpack(n_s[j * h_rows:(j + 1) * h_rows, :]).T, I32)
        t.h[j * w_rows:(j + 1) * w_rows, :] = term
        t.h_all[j * w_rows:(j + 1) * w_rows, :] = term
        return token([term[r:r + 8] for r in range(56, w_rows, 64)])

    def fetch_term(t, j):
        term = t.h_all[j * w_rows:(j + 1) * w_rows, :]
        t.h[j * w_rows:(j + 1) * w_rows, :] = term

    fillers = []

    def fill():
        if fillers:
            fillers.pop(0)()

    def project(w_s, t, m):
        def product(j):
            w = w_s[j * w_rows + m * CHUNK // 2:j * w_rows + (m + 1) * CHUNK // 2, :]
            h = t.h[j * w_rows:(j + 1) * w_rows, :]
            out = timed_dot(w, h)
            fill()
            return out

        c11, c12, c21, c22 = _block_matmul(product)
        halves = (jnp.concatenate([c11, c12], axis=1), jnp.concatenate([c21, c22], axis=1))
        return [(side * (n_pairs // 2) + m * chunk_pairs + j, block[j * PAIR:(j + 1) * PAIR])
                for side, block in enumerate(halves) for j in range(chunk_pairs)]

    def key_features(p, pk):
        phi = jnp.concatenate(_feature_map(pk), axis=0)
        z_v[p * 128:(p + 1) * 128, :] += phi[:, :HALF] + phi[:, HALF:]
        return p, phi.astype(BF16)

    def accumulate_kv(phi, v):
        for (_, phi_p), (p, v_p) in zip(phi, v, strict=True):
            kv_v[p * PAIR:(p + 1) * PAIR, :] += _dot_nt(v_p.astype(BF16), phi_p)

    def features(fn, pairs, windows):
        if windows is None:
            return [fn(*pair) for pair in pairs]
        out = []

        def job(p, block, after):
            if after is not None:
                block = block + _rows(jnp.concatenate([pltpu.bitcast(after, F32)] * 2, axis=1), PAIR)
            out.append(fn(p, block))
            return token([pltpu.bitcast(out[-1][1][-16:], I32)])

        for pair, window in zip(pairs, windows):
            plan(functools.partial(job, *pair), window)
        return out

    def summarize(t, pending, between=lambda m: None):
        for m in range(n_chunks):
            pk = project(wk_s, t, m)
            if pending is not None:
                accumulate_kv(*pending)
            between(m)
            phi = features(key_features, pk, KF_WIN)
            pending = (phi, project(wv_s, t, m))
        return pending

    def normalize(t, ln_windows, tr_windows):
        for k, window in enumerate(ln_windows):
            plan(functools.partial(normed_piece, t, k), window)
        for j, window in enumerate(tr_windows):
            plan(lambda after, j=j: transposed_term(t, j), window)

    def query_features(p, pq):
        phi = _feature_map(pq)
        z = [z_v[p * 128 + 8 * j:p * 128 + 8 * j + 8, :] for j in range(len(phi))]
        den = _head_reduce(
            jnp.add, [f * jnp.concatenate([zj, zj], axis=1) for f, zj in zip(phi, z)])
        return p, jnp.concatenate(phi, axis=0).astype(BF16), _recip(den + DEN_EPS)

    def read_out(t, m, features):
        o_t = [_dot(_unpack(kvm_v[p * HEAD_DIM:(p + 1) * HEAD_DIM, :]), phi) * _rows(inv, PAIR)
               for p, phi, inv in features]
        top = jnp.concatenate(o_t[:chunk_pairs], axis=0)
        bottom = jnp.concatenate(o_t[chunk_pairs:], axis=0)
        terms = _lhs_terms(top[:, :HALF], bottom[:, :HALF], top[:, HALF:], bottom[:, HALF:])
        for j, term in enumerate(terms):
            t.o[j * h_rows:(j + 1) * h_rows, m * CHUNK:(m + 1) * CHUNK] = pltpu.bitcast(
                term.astype(BF16).T, I32)

    def residual(t, g):
        def product(j):
            o = t.o[j * h_rows:(j + 1) * h_rows, :]
            w = wo_s[j * w_rows:(j + 1) * w_rows, g * 128:(g + 1) * 128]
            out = timed_dot(o, w)
            fill()
            return out

        for b, attn in enumerate(_block_matmul(product)):
            r0 = (b // 2) * HALF
            c0 = (b % 2) * hd + g * 128
            gate = _rows(mod_v[:, GATE_A * d + c0:GATE_A * d + c0 + 128], HALF)
            x = t.x[r0:r0 + HALF, c0:c0 + 128].astype(F32)
            x1 = x + gate * attn
            t.x1[r0:r0 + HALF, c0:c0 + 128] = x1
            t.x1_all[r0:r0 + HALF, c0:c0 + 128] = x1

    def finish(t, g, after=None):
        x1 = t.x1[16 * g:16 * g + 16, :]
        xc, rstd = _centered(x1, after)
        out = x1 + (xc * rstd * _rows(vec(OUT_SCALE), 16) + _rows(vec(OUT_SHIFT), 16))
        t.out[16 * g:16 * g + 16, :] = out.astype(BF16)
        score = jnp.sum(xc * _rows(vec(SCORE), 16), axis=-1, keepdims=True) * rstd
        lane = lax.broadcasted_iota(I32, (8, 128), 1)
        packed = t.r[...]
        for s in range(2):
            packed = jnp.where(lane == 2 * g + s, score[8 * s:8 * s + 8], packed)
        t.r[...] = packed
        return token([packed, out[:, -128:]])

    def fetch(t):
        for j in range(TERMS):
            fetch_term(t, j)

    def finishing(t, windows):
        for g, window in enumerate(windows):
            plan(functools.partial(finish, t, g), window)

    def attend(t, middle):
        ready = features(query_features, project(wq_s, t, 0), QF_WIN)
        for m in range(n_chunks):
            if m + 1 < n_chunks:
                ahead = features(query_features, project(wq_s, t, m + 1),
                                 QF_WIN if middle else None)
                if middle:
                    middle(m)
                read_out(t, m, ready)
                ready = ahead
            else:
                read_out(t, m, ready)
                if middle:
                    middle(m)

    def partial_product(i):
        return x1_all.at[pl.ds(i // 4 * hd, hd), pl.ds(i % 4 * TILE, TILE)]

    def start_up():
        early = (tile(0, 0), tile(0, 1))
        cf = c_v[...].astype(F32)
        act_v[...] = _pack(jnp.broadcast_to(cf * _sigmoid(cf), (16, d)))
        wphi_cp.wait()
        feature_blocks()
        def slices(j):
            return slice(j * 128, (j + 1) * 128), slice(hd + j * 128, hd + (j + 1) * 128)

        def activation_terms(j):
            for cp in mod_a_copies(j):
                cp.wait()
            lo, hi = slices(j)
            parts = [slice(part * hd + j * 128, part * hd + (j + 1) * 128) for part in range(4)]
            m = _dot(_unpack(act_v[...]),
                     jnp.concatenate([wmod_v[:, part] for part in parts], axis=1))[0:8]
            vectors = [m[:, :128], m[:, 128:256], 1.0 + m[:, 256:384], 1.0 + m[:, 384:]]
            for part, v in zip(parts, vectors):
                mod_v[:, part] = v
            shift_lo, shift_hi, scale_lo, scale_hi = (_rows(v, HALF) for v in vectors)
            for t in early:
                terms = _rhs_terms(t.x1[:HALF, lo] * scale_lo + shift_lo,
                                   t.x1[HALF:, lo] * scale_lo + shift_lo,
                                   t.x1[:HALF, hi] * scale_hi + shift_hi,
                                   t.x1[HALF:, hi] * scale_hi + shift_hi)
                for i, term in enumerate(terms):
                    t.h_all[i * w_rows + j * 64:i * w_rows + (j + 1) * 64, :] = pltpu.bitcast(
                        term.astype(BF16).T, I32)

        def weight_terms(j):
            for cp in kv_weight_copies(j):
                cp.wait()

            for g in range(n_chunks):
                folded_terms(1, wk_s, j, g)
                store_lhs_terms(wv_s, g, j * 128, lambda g: weight_slice(2, j, g).astype(F32).T)

        x_first_cp.wait()
        for t in early:
            for r0 in range(0, TILE, 16):
                t.x1[r0:r0 + 16, :] = normed_rows(t, r0)
        weight_terms(0)
        activation_terms(0)
        for j in range(n_chunks):
            for i in range(TERMS):
                if i == WAIT_AT[0] and j + 1 < n_chunks:
                    weight_terms(j + 1)
                if i == WAIT_AT[1] and j + 1 < n_chunks:
                    activation_terms(j + 1)
                if i == 0 and j + 1 == n_chunks:
                    x_next_cp.wait()
                    normalize(tile(1, 0), LN_WIN, TR_WIN)
                h = jnp.concatenate(
                    [t.h_all[i * w_rows + j * 64:i * w_rows + (j + 1) * 64, :] for t in early],
                    axis=1)
                for k, w_s in enumerate((wk_s, wv_s)):
                    acc = partial_product(k * TERMS + i)
                    w = w_s[i * w_rows:(i + 1) * w_rows, j * 128:(j + 1) * 128]
                    product = _dot(_unpack(w), _unpack(h))
                    acc[...] = product + acc[...] if j else product
        for cp in (wq_cp, wo_cp, wr_cp):
            cp.start()

    def early_features(m, side, after):
        def blocks(k):
            return _block_matmul(
                lambda i: partial_product(k * TERMS + i)[m * CHUNK:(m + 1) * CHUNK, :]
            )[2 * side:2 * side + 2]

        phi, v = [], []
        for pk_block, v_block in zip(blocks(0), blocks(1)):
            if after is not None:
                pk_block = pk_block + _rows(
                    jnp.concatenate([pltpu.bitcast(after, F32)] * 2, axis=1), CHUNK)
            for j in range(chunk_pairs):
                p = side * (n_pairs // 2) + m * chunk_pairs + j
                phi.append(key_features(p, pk_block[j * PAIR:(j + 1) * PAIR]))
                v.append((p, v_block[j * PAIR:(j + 1) * PAIR]))
        return phi, v

    def second_tiles():
        ready = []

        def job(n, after):
            ready.append(early_features(n // 2, n % 2, after))
            return token([pltpu.bitcast(ready[-1][0][-1][1][-16:], I32)])

        def drain(m):
            while len(ready) > 1:
                accumulate_kv(*ready.pop(0))

        for n, window in enumerate(EARLY_WIN):
            plan(functools.partial(job, n), window)
        x_rest_cp.wait()
        mod_b_cp.start()
        normalize(tile(1, 1), LN_WIN, TR_WIN)
        pending = summarize(tile(1, 0), None, drain)
        wg_cp.start()
        normalize(tile(2, 0), LN_WIN, TR_WIN)
        pending = summarize(tile(1, 1), pending, drain)
        for features in ready + [pending]:
            accumulate_kv(*features)

    def third_tiles():
        wu_cp.start()
        normalize(tile(2, 1), LN_WIN, TR_WIN)
        pending = summarize(tile(2, 0), None)
        wd_cp.start()
        normalize(tile(3, 0), LN_WIN, TR_WIN)
        accumulate_kv(*summarize(tile(2, 1), pending))

    last = n_tiles // 2 - 1

    def last_tiles():
        for cp in (wq_cp, wo_cp, wr_cp, mod_b_cp):
            cp.wait()
        normalize(tile(last, 1), LN_WIN, TR_WIN)
        for m, window in enumerate(OUT_WIN):
            plan(functools.partial(output_terms, m), window)
        for j in range(n_chunks):
            for g in range(n_chunks):
                fillers.append(functools.partial(folded_terms, 0, wq_s, j, g))
                fillers.extend([lambda: None] * FOLD_GAP)
        pending = summarize(tile(last, 0), None)
        accumulate_kv(*summarize(tile(last, 1), pending))
        assert not fillers

    def first_read_outs():
        row = lax.broadcasted_iota(I32, (PAIR, 128), 0)
        lane = lax.broadcasted_iota(I32, (PAIR, 128), 1)
        for p in range(n_pairs):
            kv = jnp.where(row % 2 == lane % 2, kv_v[p * PAIR:(p + 1) * PAIR, :], 0.0)
            kvm_v[p * HEAD_DIM:(p + 1) * HEAD_DIM, :] = _pack(kv)
            z = jnp.sum(z_v[p * 128:(p + 1) * 128, :], axis=1, keepdims=True)
            z_v[p * 128:(p + 1) * 128, :] = jnp.broadcast_to(z, (128, 128))
        for i in (GATE_A, SHIFT_B, SCALE_B, GATE_B):
            fillers.extend(modulation_rounds(i))
        fetch(tile(0, 0))
        fetch(tile(0, 1))
        attend(tile(0, 0), None)
        fetch(tile(1, 0))
        attend(tile(0, 1), functools.partial(residual, tile(0, 0)))
        assert not fillers
        derived_vectors()

    def attend_tiles():
        def body(i, carry):
            reset_clock()
            tiles = [tile(i - 1, 0), tile(i - 1, 1), tile(i, 0), tile(i, 1)]
            tiles.append(tile(jnp.minimum(i + 1, last), 0))
            for k in range(2):
                fetch(tiles[k + 3])
                finishing(tiles[k], FIN_WIN)
                attend(tiles[k + 2], functools.partial(residual, tiles[k + 1]))
            out_copy(i - 1).start()
            return carry
        lax.fori_loop(1, last + 1, body, 0)

    def last_tile():
        finishing(tile(last, 0), [(7 * (g // 5) - 1, 7 * (g // 5) + 7) for g in range(TILE // 16)])
        for m in range(n_chunks):
            residual(tile(last, 1), m)
        for g in range(TILE // 16):
            finish(tile(last, 1), g)
        out_copy(last).start()

    def route():
        scores = r_v[...]
        row = lax.broadcasted_iota(I32, scores.shape, 0)
        lane = lax.broadcasted_iota(I32, scores.shape, 1)
        index = jnp.where(lane < TILE // 8, (row // 8) * TILE + lane * 8 + row % 8, seq)

        def arg_top(valid):
            best = jnp.max(jnp.where(valid, scores, -jnp.inf))
            first = jnp.min(jnp.where(valid & (scores == best), index, seq).astype(F32))
            return jnp.minimum(first.astype(I32), seq - 1)

        i0 = arg_top(index < seq)
        i1 = arg_top((index < seq) & (index != i0))

        sub = lax.broadcasted_iota(I32, (16, d), 0)
        x1 = jnp.where(sub == 0, x1_all[pl.ds(i0, 1), :], x1_all[pl.ds(i1, 1), :])
        xc, rstd = _centered(x1)
        h2 = xc * rstd * _rows(vec(SCALE_B), 16) + _rows(vec(SHIFT_B), 16)
        gate = _sigmoid(jnp.sum(h2 * _rows(vec(ROUTER), 16), axis=-1, keepdims=True))
        xs = h2.astype(BF16)
        for cp in (wg_cp, wu_cp, wd_cp):
            cp.wait()
        spans = [slice(f, f + FFN_CHUNK) for f in range(0, wd_v.shape[0], FFN_CHUNK)]
        y, hidden = 0.0, None
        for k in range(len(spans) + 1):
            if k < len(spans):
                g = _dot(xs, wg_v[:, spans[k]])
                u = _dot(xs, wu_v[:, spans[k]])
            if k > 0:
                y = y + _dot(hidden, wd_v[spans[k - 1], :])
            hidden = (g * _sigmoid(g) * u).astype(BF16)
        routed = x1 + _rows(vec(GATE_B), 16) * (h2 + y * gate)

        for i in range(last + 1):
            out_copy(i).wait()

        def patch(k, i):
            base = pl.multiple_of((i // 16) * 16, 16)
            old = out_v[pl.ds(base, 16), :].astype(F32)
            out_v[pl.ds(base, 16), :] = jnp.where(
                sub == i - base, routed[k:k + 1], old).astype(BF16)
            return base, copy(out_v.at[pl.ds(base, 16)], out_hbm.at[pl.ds(base, 16)],
                              sem.at[16 + k])

        base0, patch0 = patch(0, i0)
        base1, patch1 = patch(1, i1)
        patch0.start()

        @pl.when(base1 != base0)
        def _():
            patch1.start()
            patch1.wait()

        patch0.wait()

    for cp in (c_cp, wphi_cp, x_first_cp):
        cp.start()
    for j in range(n_chunks):
        for cp in kv_weight_copies(j) + mod_a_copies(j):
            cp.start()
    x_next_cp.start()
    x_rest_cp.start()
    kv_v[...] = jnp.zeros(kv_v.shape, F32)
    z_v[...] = jnp.zeros(z_v.shape, F32)
    r_v[...] = jnp.full(r_v.shape, -jnp.inf, F32)
    c_cp.wait()
    words = pltpu.bitcast(jnp.broadcast_to(c_v[:, :128].astype(F32), (8, 128)), I32)
    zero = jnp.minimum(lax.shift_right_logical(words, 1), 0)
    zero_v[...] = zero
    origin = jnp.max(zero)
    steps = (start_up, second_tiles, third_tiles, last_tiles, first_read_outs, attend_tiles,
             last_tile, route)
    for k, step in enumerate(steps):
        if ONLY is None or ONLY == k:
            with _scope(step.__name__):
                reset_clock()
                if k in SPLIT:
                    pl.when(origin <= k)(step)
                else:
                    step()


@jax.jit
def pallas_adaLN_cond__linear_kernel_hedgehog__moe_arch_mod__prompt_kernel(
    A_x: jax.Array,
    A_wqkv: jax.Array,
    A_w_phi: jax.Array,
    A_wo: jax.Array,
    B_x: jax.Array,
    B_w_r: jax.Array,
    B_w_gate: jax.Array,
    B_w_up: jax.Array,
    B_w_down: jax.Array,
    c: jax.Array,
    w_mod: jax.Array,
):
    del B_x
    batch, seq, d = A_x.shape
    assert batch == 1 and d == HEADS * HEAD_DIM and seq == 8 * TILE
    n_tiles = seq // TILE
    operands = (A_x.reshape(seq, d), A_wqkv, A_w_phi, A_wo, B_w_r, B_w_gate, B_w_up, B_w_down,
                c, w_mod)
    weight_terms = pltpu.VMEM((TERMS * d // 4, d // 2), I32)
    scratch = [pltpu.VMEM(a.shape, a.dtype) for a in operands] + [
        weight_terms, weight_terms, weight_terms, weight_terms,
        pltpu.VMEM((TERMS * HALF // 2, d // 2), I32),
        [pltpu.VMEM((TERMS * d // 4, HALF), I32)] * 2,
        pltpu.VMEM((n_tiles * TERMS * d // 4, HALF), I32),
        [pltpu.VMEM((TERMS * HALF // 2, d // 2), I32)] * 2,
        [pltpu.VMEM((TILE, d), F32)] * 2,
        pltpu.VMEM((seq, d), F32),
        pltpu.VMEM((8, 10 * d), F32),
        pltpu.VMEM((HEADS // 2 * PAIR, 128), F32),
        pltpu.VMEM((HEADS // 2 * HEAD_DIM, 128), I32),
        pltpu.VMEM((HEADS // 2 * 128, 128), F32),
        pltpu.VMEM((seq, d), BF16),
        pltpu.VMEM((n_tiles * 8, 128), F32),
        pltpu.VMEM((8, 128), I32),
        pltpu.VMEM((8, d), I32),
        pltpu.VMEM((d // 2, 128), I32),
        pltpu.SemaphoreType.DMA((26,)),
        pltpu.SemaphoreType.DMA((n_tiles // 2,)),
    ]
    out = pl.pallas_call(
        _kernel,
        out_shape=jax.ShapeDtypeStruct((seq, d), A_x.dtype),
        in_specs=[pl.BlockSpec(memory_space=pl.ANY)] * len(operands),
        out_specs=pl.BlockSpec(memory_space=pl.ANY),
        scratch_shapes=scratch,
        compiler_params=pltpu.CompilerParams(vmem_limit_bytes=110 * 2**20, flags=FLAGS or None),
        name="adaln_hedgehog_mod",
    )(*operands)
    return out.reshape(batch, seq, d)
```

```python
import collections
import contextlib
import functools
import math

import jax
import jax.numpy as jnp
from jax import lax
import jax.experimental.pallas as pl
import jax.experimental.pallas.tpu as pltpu

F32 = jnp.float32
BF16 = jnp.bfloat16
I32 = jnp.int32

HEADS = 32
HEAD_DIM = 32
PAIR = 2 * HEAD_DIM
TERMS = 7
LN_EPS = 1e-5
DEN_EPS = 1e-6
LOG2E = math.log2(math.e)

TILE = 256
HALF = TILE // 2
CHUNK = 128
SCOPES = True
LAST_WIN = tuple((7 * (g // 5), 7 * (g // 5) + 9) for g in range(16))
FOLD_GAP = 2
OUT_WIN = tuple((55 + 7 * p, 64 + 7 * p) for p in range(7)) + ((97, 111),)
WAIT_AT = (2, 5)
SPLIT = (1, 3)
EARLY_WIN = (None,) * 4
ONLY = None
LN_WIN = (None,) * 8
TR_WIN = (None,) * 7
KF_WIN = None
QF_WIN = None
FIN_WIN = ((-1, 9),) * 4 + ((20, 30),) * 4 + ((34, 44),) * 4 + ((41, 51),) * 4
FFN_CHUNK = 512
FLAGS = {"XLA_TPU_EVENLY_DISTRIBUTE_CRITICAL_NODES": True}

NT_DIMS = (((1,), (1,)), ((), ()))


def _scope(name):
    return jax.named_scope(name) if SCOPES else contextlib.nullcontext()


def _dot(a, b):
    return jnp.dot(a, b, preferred_element_type=F32)


def _dot_nt(a, b):
    return lax.dot_general(a, b, NT_DIMS, preferred_element_type=F32)


def _pack(v):
    return pltpu.bitcast(v.astype(BF16), I32)


def _pack_heads(v):
    starts = range(0, v.shape[0], PAIR)
    first = jnp.concatenate([v[s:s + HEAD_DIM] for s in starts], axis=0)
    second = jnp.concatenate([v[s + HEAD_DIM:s + PAIR] for s in starts], axis=0)
    return pltpu.pack_elementwise([first, second], packed_dtype=BF16).astype(I32)


def _unpack(v):
    return pltpu.bitcast(v, BF16)


def _recip(d):
    r = pltpu.reciprocal(d, approx=True)
    return r * (2.0 - d * r)


def _sigmoid(v):
    return 1.0 / (1.0 + jnp.exp(-v))


def _rows(v, n):
    return jnp.concatenate([v] * (n // 8), axis=0) if n > 8 else v


def _centered(x, after=None):
    inv_d = 1.0 / x.shape[-1]
    if after is not None:
        head = x[:, :128] + _rows(pltpu.bitcast(after, F32), x.shape[0])
        x = jnp.concatenate([head, x[:, 128:]], axis=1)
    xc = x - jnp.sum(x, axis=-1, keepdims=True) * inv_d
    var = jnp.sum(xc * xc, axis=-1, keepdims=True) * inv_d
    return xc, lax.rsqrt(var + LN_EPS)


def _lhs_terms(a11, a12, a21, a22):
    return [a11 + a22, a21 + a22, a11, a22, a11 + a12, a21 - a11, a12 - a22]


def _rhs_terms(b11, b12, b21, b22):
    return [b11 + b22, b11, b12 - b22, b21 - b11, b22, b11 + b12, b21 + b22]


def _block_matmul(product):
    m1 = product(0)
    m4 = product(3)
    c11 = m1 + m4
    c11 = c11 + product(6)
    m5 = product(4)
    c11 = c11 - m5
    m3 = product(2)
    c12 = m3 + m5
    c22 = m1 + m3
    m2 = product(1)
    c21 = m2 + m4
    c22 = c22 - m2
    c22 = c22 + product(5)
    return c11, c12, c21, c22


def _head_reduce(op, tiles):
    while len(tiles) > 1:
        tiles = [op(tiles[i], tiles[i + 1]) for i in range(0, len(tiles), 2)]
    m = tiles[0]
    m = op(m, pltpu.roll(m, 4, 0))
    return op(m, pltpu.roll(m, 2, 0))


def _feature_map(p):
    tiles = [p[8 * j:8 * j + 8] for j in range(PAIR // 8)]
    hi = _head_reduce(jnp.maximum, tiles)
    lo = _head_reduce(jnp.minimum, tiles)
    e_pos = [jnp.exp2(t - hi) for t in tiles]
    e_neg = [jnp.exp2(lo - t) for t in tiles]
    r_pos = _recip(_head_reduce(jnp.add, e_pos))
    r_neg = _recip(_head_reduce(jnp.add, e_neg))
    return [e * r_pos for e in e_pos] + [e * r_neg for e in e_neg]


Tile = collections.namedtuple("Tile", "x h h_all o x1 x1_all out r")
SHIFT_A, SCALE_A, GATE_A, SHIFT_B, SCALE_B, GATE_B, ROUTER, OUT_SCALE, OUT_SHIFT, SCORE = range(10)


def _kernel(x_hbm, wqkv_hbm, wphi_hbm, wo_hbm, wr_hbm, wg_hbm, wu_hbm, wd_hbm, c_hbm, wmod_hbm,
            out_hbm,
            x_v, wqkv_v, wphi_v, wo_v, wr_v, wg_v, wu_v, wd_v, c_v, wmod_v,
            wq_s, wk_s, wv_s, wo_s, n_s, h_s, h_all, o_s, x1_v, x1_all, mod_v, kv_v, kvm_v, z_v, out_v, r_v, zero_v, act_v, phi_s,
            sem, out_sem):
    seq, d = x_v.shape
    hd = d // 2
    n_tiles = seq // TILE
    n_pairs = HEADS // 2
    n_chunks = hd // CHUNK
    chunk_pairs = CHUNK // PAIR
    h_rows = HALF // 2
    w_rows = hd // 2

    def copy(src, dst, s):
        return pltpu.make_async_copy(src, dst, s)

    def token_copy(src, dst, first, count, s):
        return copy(src.at[pl.ds(first, count)], dst.at[pl.ds(first, count)], s)

    def cols(ref, i, n=1):
        return ref.at[:, pl.ds(i * d, n * d)]

    c_cp = copy(c_hbm, c_v, sem.at[0])
    wphi_cp = copy(wphi_hbm, wphi_v, sem.at[1])
    wr_cp = copy(wr_hbm, wr_v, sem.at[2])
    mod_b_cp = copy(cols(wmod_hbm, 2, 4), cols(wmod_v, 2, 4), sem.at[5])
    wq_cp = copy(cols(wqkv_hbm, 0), cols(wqkv_v, 0), sem.at[6])
    wo_cp = copy(wo_hbm, wo_v, sem.at[9])
    wg_cp = copy(wg_hbm, wg_v, sem.at[10])
    wu_cp = copy(wu_hbm, wu_v, sem.at[11])
    wd_cp = copy(wd_hbm, wd_v, sem.at[12])
    x_first_cp = token_copy(x_hbm, x_v, 0, 2 * TILE, sem.at[13])
    x_next_cp = token_copy(x_hbm, x_v, 2 * TILE, TILE, sem.at[14])
    x_rest_cp = token_copy(x_hbm, x_v, 3 * TILE, seq - 3 * TILE, sem.at[15])

    def kv_weight_copies(j):
        spans = [(pl.ds(half * hd + j * 128, 128), pl.ds(d, 2 * d)) for half in range(2)]
        return [copy(wqkv_hbm.at[span], wqkv_v.at[span], sem.at[18 + j]) for span in spans]

    def mod_a_copies(j):
        spans = [pl.ds(part * hd + j * 128, 128) for part in range(4)]
        return [copy(wmod_hbm.at[:, span], wmod_v.at[:, span], sem.at[22 + j]) for span in spans]

    def view(ref, index, size):
        start = index * size
        return ref.at[pl.ds(start if isinstance(start, int) else pl.multiple_of(start, size), size)]

    def tile(i, parity):
        t = 2 * i + parity
        return Tile(x=view(x_v, t, TILE), h=h_s[parity], h_all=view(h_all, t, TERMS * w_rows),
                    o=o_s[parity],
                    x1=x1_v[parity], x1_all=view(x1_all, t, TILE), out=view(out_v, t, TILE), r=view(r_v, t, 8))

    def out_copy(i):
        return copy(view(out_v, i, 2 * TILE), view(out_hbm, i, 2 * TILE), out_sem.at[i])

    def token(values):
        tiles = [pltpu.bitcast(v[r:r + 8, c:c + 128], I32) for v in values
                 for r in range(0, v.shape[0], 8) for c in range(0, v.shape[1], 128)]
        while len(tiles) > 1:
            tiles = [tiles[j] | tiles[j + 1] if j + 1 < len(tiles) else tiles[j]
                     for j in range(0, len(tiles), 2)]
        return tiles[0] & zero_v[...]

    clock = {"now": 0, "last": None, "jobs": {}, "gates": {}}

    def reset_clock():
        assert not clock["jobs"]
        clock.update(last=None, gates={})

    def run_job(job, after, end):
        zero = job(after)
        clock["gates"].setdefault(end, []).append(zero)

    def plan(job, window):
        if window is None:
            job(None)
            return
        start, end = (clock["now"] + w for w in window)
        if start < clock["now"]:
            run_job(job, clock["last"], end)
        else:
            clock["jobs"].setdefault(start, []).append((job, end))

    def timed_dot(lhs, rhs):
        for zero in clock["gates"].pop(clock["now"], []):
            top = jnp.concatenate([lhs[:8, :128] | zero, lhs[:8, 128:]], axis=1)
            lhs = jnp.concatenate([top, lhs[8:]], axis=0)
        out = _dot(_unpack(lhs), _unpack(rhs))
        clock["last"] = token([out[-8:]])
        for job, end in clock["jobs"].pop(clock["now"], []):
            run_job(job, clock["last"], end)
        clock["now"] += 1
        return out

    def store_terms(dst, g, c0, terms):
        packed = [_pack_heads(term) for term in terms]
        for i, term in enumerate(packed):
            dst[i * w_rows + g * 64:i * w_rows + (g + 1) * 64, c0:c0 + term.shape[1]] = term
        return packed

    def store_lhs_terms(dst, g, c0, group):
        top, bottom = group(g), group(g + hd // 128)
        n = top.shape[1] // 2
        return store_terms(
            dst, g, c0, _lhs_terms(top[:, :n], top[:, n:], bottom[:, :n], bottom[:, n:]))

    def feature_blocks():
        row = lax.broadcasted_iota(I32, (128, 128), 0)
        lane = lax.broadcasted_iota(I32, (128, 128), 1)
        same_head = row // HEAD_DIM == lane // HEAD_DIM
        row_f = lax.broadcasted_iota(I32, (128, HEAD_DIM), 0)
        lane_f = lax.broadcasted_iota(I32, (128, HEAD_DIM), 1)
        pick = jnp.where(row_f % HEAD_DIM == lane_f, 1.0, 0.0).astype(BF16)
        for g in range(d // 128):
            wphi = wphi_v[4 * g:4 * g + 4].reshape(128, HEAD_DIM)
            phi_s[g * 64:(g + 1) * 64, :] = _pack(jnp.where(same_head, _dot_nt(pick, wphi), 0.0))

    def folded(w, g):
        return _dot_nt(_unpack(phi_s[g * 64:(g + 1) * 64, :]), w) * LOG2E

    def weight_slice(col, j, g):
        span = slice(col * d + g * 128, col * d + (g + 1) * 128)
        return jnp.concatenate(
            [wqkv_v[half * hd + j * 128:half * hd + (j + 1) * 128, span] for half in range(2)],
            axis=0)

    def folded_terms(col, dst, j, g):
        store_lhs_terms(dst, g, j * 128, lambda g: folded(weight_slice(col, j, g), g))

    def output_terms(p, c, after):
        def block(r0, c0):
            words = pltpu.bitcast(wo_v[r0:r0 + PAIR, c0:c0 + 128], I32) | _rows(after, HEAD_DIM)
            return _unpack(words).astype(F32)

        terms = _rhs_terms(*(block(r + p * PAIR, k + c * 128) for r in (0, hd) for k in (0, hd)))
        packed = [_pack_heads(term) for term in terms]
        for i, term in enumerate(packed):
            r0 = i * w_rows + p * HEAD_DIM
            wo_s[r0:r0 + HEAD_DIM, c * 128:(c + 1) * 128] = term
        return token([term[-8:] for term in packed])

    def vec(i):
        return mod_v[:, i * d:(i + 1) * d]

    def modulation_rounds(i):
        partial = {}

        def one(c0, half):
            span = slice(half * hd, (half + 1) * hd)
            m = _dot(_unpack(act_v[:, span]), wmod_v[span, c0:c0 + 128])[0:8]
            if half == 0:
                partial[c0] = 1.0 + m if i in (SCALE_A, SCALE_B) else m
            else:
                mod_v[:, c0:c0 + 128] = partial[c0] + m

        return [functools.partial(one, c0, half)
                for c0 in range(i * d, (i + 1) * d, 128) for half in range(2)]

    def derived_vectors():
        router = jnp.broadcast_to(wr_v[...].astype(F32).reshape(1, d), (8, d))
        for i, v in ((ROUTER, router), (OUT_SCALE, vec(GATE_B) * vec(SCALE_B)),
                     (OUT_SHIFT, vec(GATE_B) * vec(SHIFT_B)), (SCORE, router * vec(SCALE_B))):
            mod_v[:, i * d:(i + 1) * d] = v

    def normed_rows(t, r0, after=None):
        xc, rstd = _centered(t.x[r0:r0 + 16, :].astype(F32), after)
        return xc * rstd

    def normed_piece(t, k, after=None):
        def normed(start):
            xn = normed_rows(t, start + 16 * k, after)
            return xn * _rows(vec(SCALE_A), 16) + _rows(vec(SHIFT_A), 16)

        ha, hb = normed(0), normed(HALF)
        packed = [_pack(term)
                  for term in _rhs_terms(ha[:, :hd], hb[:, :hd], ha[:, hd:], hb[:, hd:])]
        for j, term in enumerate(packed):
            n_s[j * h_rows + 8 * k:j * h_rows + 8 * k + 8, :] = term
        return token(packed)

    def transposed_term(t, j):
        term = pltpu.bitcast(_unpack(n_s[j * h_rows:(j + 1) * h_rows, :]).T, I32)
        t.h[j * w_rows:(j + 1) * w_rows, :] = term
        t.h_all[j * w_rows:(j + 1) * w_rows, :] = term
        return token([term[r:r + 8] for r in range(56, w_rows, 64)])

    def fetch_term(t, j):
        term = t.h_all[j * w_rows:(j + 1) * w_rows, :]
        t.h[j * w_rows:(j + 1) * w_rows, :] = term

    fillers = []

    def fill():
        if fillers:
            fillers.pop(0)()

    def project(w_s, t, m):
        def product(j):
            w = w_s[j * w_rows + m * CHUNK // 2:j * w_rows + (m + 1) * CHUNK // 2, :]
            h = t.h[j * w_rows:(j + 1) * w_rows, :]
            out = timed_dot(w, h)
            fill()
            return out

        c11, c12, c21, c22 = _block_matmul(product)
        halves = (jnp.concatenate([c11, c12], axis=1), jnp.concatenate([c21, c22], axis=1))
        return [(side * (n_pairs // 2) + m * chunk_pairs + j, block[j * PAIR:(j + 1) * PAIR])
                for side, block in enumerate(halves) for j in range(chunk_pairs)]

    def key_features(p, pk):
        phi = jnp.concatenate(_feature_map(pk), axis=0)
        z_v[p * 128:(p + 1) * 128, :] += phi[:, :HALF] + phi[:, HALF:]
        return p, phi.astype(BF16)

    def accumulate_kv(phi, v):
        for (_, phi_p), (p, v_p) in zip(phi, v, strict=True):
            kv_v[p * PAIR:(p + 1) * PAIR, :] += _dot_nt(v_p.astype(BF16), phi_p)

    def features(fn, pairs, windows):
        if windows is None:
            return [fn(*pair) for pair in pairs]
        out = []

        def job(p, block, after):
            if after is not None:
                block = block + _rows(jnp.concatenate([pltpu.bitcast(after, F32)] * 2, axis=1), PAIR)
            out.append(fn(p, block))
            return token([pltpu.bitcast(out[-1][1][-16:], I32)])

        for pair, window in zip(pairs, windows):
            plan(functools.partial(job, *pair), window)
        return out

    def summarize(t, pending, between=lambda m: None):
        for m in range(n_chunks):
            pk = project(wk_s, t, m)
            if pending is not None:
                accumulate_kv(*pending)
            between(m)
            phi = features(key_features, pk, KF_WIN)
            pending = (phi, project(wv_s, t, m))
        return pending

    def normalize(t, ln_windows, tr_windows):
        for k, window in enumerate(ln_windows):
            plan(functools.partial(normed_piece, t, k), window)
        for j, window in enumerate(tr_windows):
            plan(lambda after, j=j: transposed_term(t, j), window)

    def query_features(p, pq):
        phi = _feature_map(pq)
        z = [z_v[p * 128 + 8 * j:p * 128 + 8 * j + 8, :] for j in range(len(phi))]
        den = _head_reduce(
            jnp.add, [f * jnp.concatenate([zj, zj], axis=1) for f, zj in zip(phi, z)])
        return p, jnp.concatenate(phi, axis=0).astype(BF16), _recip(den + DEN_EPS)

    def read_out(t, m, features):
        o_t = [_dot(_unpack(kvm_v[p * HEAD_DIM:(p + 1) * HEAD_DIM, :]), phi) * _rows(inv, PAIR)
               for p, phi, inv in features]
        top = jnp.concatenate(o_t[:chunk_pairs], axis=0)
        bottom = jnp.concatenate(o_t[chunk_pairs:], axis=0)
        terms = _lhs_terms(top[:, :HALF], bottom[:, :HALF], top[:, HALF:], bottom[:, HALF:])
        for j, term in enumerate(terms):
            t.o[j * h_rows:(j + 1) * h_rows, m * CHUNK:(m + 1) * CHUNK] = pltpu.bitcast(
                term.astype(BF16).T, I32)

    def residual(t, g, first=0, count=HALF):
        def product(j):
            o = t.o[j * h_rows + first // 2:j * h_rows + (first + count) // 2, :]
            w = wo_s[j * w_rows:(j + 1) * w_rows, g * 128:(g + 1) * 128]
            out = timed_dot(o, w)
            fill()
            return out

        for b, attn in enumerate(_block_matmul(product)):
            r0 = (b // 2) * HALF + first
            c0 = (b % 2) * hd + g * 128
            gate = _rows(mod_v[:, GATE_A * d + c0:GATE_A * d + c0 + 128], count)
            x1 = t.x[r0:r0 + count, c0:c0 + 128].astype(F32) + gate * attn
            t.x1[r0:r0 + count, c0:c0 + 128] = x1
            t.x1_all[r0:r0 + count, c0:c0 + 128] = x1

    def finish(t, g, after=None):
        x1 = t.x1[16 * g:16 * g + 16, :]
        xc, rstd = _centered(x1, after)
        out = x1 + (xc * rstd * _rows(vec(OUT_SCALE), 16) + _rows(vec(OUT_SHIFT), 16))
        t.out[16 * g:16 * g + 16, :] = out.astype(BF16)
        score = jnp.sum(xc * _rows(vec(SCORE), 16), axis=-1, keepdims=True) * rstd
        lane = lax.broadcasted_iota(I32, (8, 128), 1)
        packed = t.r[...]
        for s in range(2):
            packed = jnp.where(lane == 2 * g + s, score[8 * s:8 * s + 8], packed)
        t.r[...] = packed
        return token([packed, out[:, -128:]])

    def fetch(t):
        for j in range(TERMS):
            fetch_term(t, j)

    def finishing(t, windows):
        for g, window in enumerate(windows):
            plan(functools.partial(finish, t, g), window)

    def attend(t, middle):
        ready = features(query_features, project(wq_s, t, 0), QF_WIN)
        for m in range(n_chunks):
            if m + 1 < n_chunks:
                ahead = features(query_features, project(wq_s, t, m + 1),
                                 QF_WIN if middle else None)
                if middle:
                    middle(m)
                read_out(t, m, ready)
                ready = ahead
            else:
                read_out(t, m, ready)
                if middle:
                    middle(m)

    def partial_product(i):
        return x1_all.at[pl.ds(i // 4 * hd, hd), pl.ds(i % 4 * TILE, TILE)]

    def start_up():
        early = (tile(0, 0), tile(0, 1))
        cf = c_v[...].astype(F32)
        act_v[...] = _pack(jnp.broadcast_to(cf * _sigmoid(cf), (16, d)))
        wphi_cp.wait()
        feature_blocks()
        def slices(j):
            return slice(j * 128, (j + 1) * 128), slice(hd + j * 128, hd + (j + 1) * 128)

        def activation_terms(j):
            for cp in mod_a_copies(j):
                cp.wait()
            lo, hi = slices(j)
            parts = [slice(part * hd + j * 128, part * hd + (j + 1) * 128) for part in range(4)]
            m = _dot(_unpack(act_v[...]),
                     jnp.concatenate([wmod_v[:, part] for part in parts], axis=1))[0:8]
            vectors = [m[:, :128], m[:, 128:256], 1.0 + m[:, 256:384], 1.0 + m[:, 384:]]
            for part, v in zip(parts, vectors):
                mod_v[:, part] = v
            shift_lo, shift_hi, scale_lo, scale_hi = (_rows(v, HALF) for v in vectors)
            for t in early:
                terms = _rhs_terms(t.x1[:HALF, lo] * scale_lo + shift_lo,
                                   t.x1[HALF:, lo] * scale_lo + shift_lo,
                                   t.x1[:HALF, hi] * scale_hi + shift_hi,
                                   t.x1[HALF:, hi] * scale_hi + shift_hi)
                for i, term in enumerate(terms):
                    t.h_all[i * w_rows + j * 64:i * w_rows + (j + 1) * 64, :] = pltpu.bitcast(
                        term.astype(BF16).T, I32)

        def weight_terms(j):
            for cp in kv_weight_copies(j):
                cp.wait()

            for g in range(n_chunks):
                folded_terms(1, wk_s, j, g)
                store_lhs_terms(wv_s, g, j * 128, lambda g: weight_slice(2, j, g).astype(F32).T)

        x_first_cp.wait()
        for t in early:
            for r0 in range(0, TILE, 16):
                t.x1[r0:r0 + 16, :] = normed_rows(t, r0)
        weight_terms(0)
        activation_terms(0)
        for j in range(n_chunks):
            for i in range(TERMS):
                if i == WAIT_AT[0] and j + 1 < n_chunks:
                    weight_terms(j + 1)
                if i == WAIT_AT[1] and j + 1 < n_chunks:
                    activation_terms(j + 1)
                if i == 0 and j + 1 == n_chunks:
                    x_next_cp.wait()
                    normalize(tile(1, 0), LN_WIN, TR_WIN)
                h = jnp.concatenate(
                    [t.h_all[i * w_rows + j * 64:i * w_rows + (j + 1) * 64, :] for t in early],
                    axis=1)
                for k, w_s in enumerate((wk_s, wv_s)):
                    acc = partial_product(k * TERMS + i)
                    w = w_s[i * w_rows:(i + 1) * w_rows, j * 128:(j + 1) * 128]
                    product = _dot(_unpack(w), _unpack(h))
                    acc[...] = product + acc[...] if j else product
        for cp in (wq_cp, wo_cp, wr_cp):
            cp.start()

    def early_features(m, side, after):
        def blocks(k):
            return _block_matmul(
                lambda i: partial_product(k * TERMS + i)[m * CHUNK:(m + 1) * CHUNK, :]
            )[2 * side:2 * side + 2]

        phi, v = [], []
        for pk_block, v_block in zip(blocks(0), blocks(1)):
            if after is not None:
                pk_block = pk_block + _rows(
                    jnp.concatenate([pltpu.bitcast(after, F32)] * 2, axis=1), CHUNK)
            for j in range(chunk_pairs):
                p = side * (n_pairs // 2) + m * chunk_pairs + j
                phi.append(key_features(p, pk_block[j * PAIR:(j + 1) * PAIR]))
                v.append((p, v_block[j * PAIR:(j + 1) * PAIR]))
        return phi, v

    def summarize_pair(i, copies):
        ready = []

        def job(n, after):
            ready.append(early_features(n // 2, n % 2, after))
            return token([pltpu.bitcast(ready[-1][0][-1][1][-16:], I32)])

        def drain(m):
            if m % 2:
                accumulate_kv(*ready.pop(0))

        for n, window in enumerate(EARLY_WIN):
            plan(functools.partial(job, (i - 1) * len(EARLY_WIN) + n), window)
        copies[0].start()
        normalize(tile(i, 1), LN_WIN, TR_WIN)
        pending = summarize(tile(i, 0), None, drain)
        copies[1].start()
        normalize(tile(i + 1, 0), LN_WIN, TR_WIN)
        accumulate_kv(*summarize(tile(i, 1), pending, drain))
        assert not ready

    def second_tiles():
        x_rest_cp.wait()
        summarize_pair(1, (mod_b_cp, wg_cp))

    def third_tiles():
        summarize_pair(2, (wu_cp, wd_cp))

    last = n_tiles // 2 - 1

    def last_tiles():
        for cp in (wq_cp, wo_cp, wr_cp, mod_b_cp):
            cp.wait()
        normalize(tile(last, 1), LN_WIN, TR_WIN)
        for p, window in enumerate(OUT_WIN):
            for c in range(n_chunks):
                plan(functools.partial(output_terms, p, c), window)
        for j in range(n_chunks):
            for g in range(n_chunks):
                fillers.append(functools.partial(folded_terms, 0, wq_s, j, g))
                fillers.extend([lambda: None] * FOLD_GAP)
        pending = summarize(tile(last, 0), None)
        accumulate_kv(*summarize(tile(last, 1), pending))
        assert not fillers

    def first_read_outs():
        row = lax.broadcasted_iota(I32, (PAIR, 128), 0)
        lane = lax.broadcasted_iota(I32, (PAIR, 128), 1)
        for p in range(n_pairs):
            kv = jnp.where(row % 2 == lane % 2, kv_v[p * PAIR:(p + 1) * PAIR, :], 0.0)
            kvm_v[p * HEAD_DIM:(p + 1) * HEAD_DIM, :] = _pack(kv)
            z = jnp.sum(z_v[p * 128:(p + 1) * 128, :], axis=1, keepdims=True)
            z_v[p * 128:(p + 1) * 128, :] = jnp.broadcast_to(z, (128, 128))
        for i in (GATE_A, SHIFT_B, SCALE_B, GATE_B):
            fillers.extend(modulation_rounds(i))
        fetch(tile(0, 0))
        fetch(tile(0, 1))
        attend(tile(0, 0), None)
        fetch(tile(1, 0))
        attend(tile(0, 1), functools.partial(residual, tile(0, 0)))
        assert not fillers
        derived_vectors()

    def attend_tiles():
        def body(i, carry):
            reset_clock()
            tiles = [tile(i - 1, 0), tile(i - 1, 1), tile(i, 0), tile(i, 1)]
            tiles.append(tile(jnp.minimum(i + 1, last), 0))
            for k in range(2):
                fetch(tiles[k + 3])
                finishing(tiles[k], FIN_WIN)
                attend(tiles[k + 2], functools.partial(residual, tiles[k + 1]))
            out_copy(i - 1).start()
            return carry
        lax.fori_loop(1, last + 1, body, 0)

    def last_tile():
        final = tile(last, 1)
        finishing(tile(last, 0), LAST_WIN)
        for g in range(n_chunks):
            residual(final, g, 0, HALF // 2)
        groups = HALF // 32
        for n, g in enumerate(side * 2 * groups + g for side in range(2) for g in range(groups)):
            plan(functools.partial(finish, final, g), (7 * (n // 3) - 1, 7 * (n // 3) + 9))
        for g in range(n_chunks):
            residual(final, g, HALF // 2, HALF // 2)
        for side in range(2):
            for g in range(groups):
                finish(final, (2 * side + 1) * groups + g)
        out_copy(last).start()

    def route():
        scores = r_v[...]
        row = lax.broadcasted_iota(I32, scores.shape, 0)
        lane = lax.broadcasted_iota(I32, scores.shape, 1)
        index = jnp.where(lane < TILE // 8, (row // 8) * TILE + lane * 8 + row % 8, seq)

        def arg_top(valid):
            best = jnp.max(jnp.where(valid, scores, -jnp.inf))
            first = jnp.min(jnp.where(valid & (scores == best), index, seq).astype(F32))
            return jnp.minimum(first.astype(I32), seq - 1)

        i0 = arg_top(index < seq)
        i1 = arg_top((index < seq) & (index != i0))

        sub = lax.broadcasted_iota(I32, (16, d), 0)
        x1 = jnp.where(sub == 0, x1_all[pl.ds(i0, 1), :], x1_all[pl.ds(i1, 1), :])
        xc, rstd = _centered(x1)
        h2 = xc * rstd * _rows(vec(SCALE_B), 16) + _rows(vec(SHIFT_B), 16)
        gate = _sigmoid(jnp.sum(h2 * _rows(vec(ROUTER), 16), axis=-1, keepdims=True))
        xs = h2.astype(BF16)
        for cp in (wg_cp, wu_cp, wd_cp):
            cp.wait()
        spans = [slice(f, f + FFN_CHUNK) for f in range(0, wd_v.shape[0], FFN_CHUNK)]
        y, hidden = 0.0, None
        for k in range(len(spans) + 1):
            if k < len(spans):
                g = _dot(xs, wg_v[:, spans[k]])
                u = _dot(xs, wu_v[:, spans[k]])
            if k > 0:
                y = y + _dot(hidden, wd_v[spans[k - 1], :])
            hidden = (g * _sigmoid(g) * u).astype(BF16)
        routed = x1 + _rows(vec(GATE_B), 16) * (h2 + y * gate)

        for i in range(last + 1):
            out_copy(i).wait()

        def patch(k, i):
            base = pl.multiple_of((i // 16) * 16, 16)
            old = out_v[pl.ds(base, 16), :].astype(F32)
            out_v[pl.ds(base, 16), :] = jnp.where(
                sub == i - base, routed[k:k + 1], old).astype(BF16)
            return base, copy(out_v.at[pl.ds(base, 16)], out_hbm.at[pl.ds(base, 16)],
                              sem.at[16 + k])

        base0, patch0 = patch(0, i0)
        base1, patch1 = patch(1, i1)
        patch0.start()

        @pl.when(base1 != base0)
        def _():
            patch1.start()
            patch1.wait()

        patch0.wait()

    for cp in (c_cp, wphi_cp, x_first_cp):
        cp.start()
    for j in range(n_chunks):
        for cp in kv_weight_copies(j) + mod_a_copies(j):
            cp.start()
    x_next_cp.start()
    x_rest_cp.start()
    kv_v[...] = jnp.zeros(kv_v.shape, F32)
    z_v[...] = jnp.zeros(z_v.shape, F32)
    r_v[...] = jnp.full(r_v.shape, -jnp.inf, F32)
    c_cp.wait()
    words = pltpu.bitcast(jnp.broadcast_to(c_v[:, :128].astype(F32), (8, 128)), I32)
    zero = jnp.minimum(lax.shift_right_logical(words, 1), 0)
    zero_v[...] = zero
    origin = jnp.max(zero)
    steps = (start_up, second_tiles, third_tiles, last_tiles, first_read_outs, attend_tiles,
             last_tile, route)
    for k, step in enumerate(steps):
        if ONLY is None or ONLY == k:
            with _scope(step.__name__):
                reset_clock()
                if k in SPLIT:
                    pl.when(origin <= k)(step)
                else:
                    step()


@jax.jit
def pallas_adaLN_cond__linear_kernel_hedgehog__moe_arch_mod__prompt_kernel(
    A_x: jax.Array,
    A_wqkv: jax.Array,
    A_w_phi: jax.Array,
    A_wo: jax.Array,
    B_x: jax.Array,
    B_w_r: jax.Array,
    B_w_gate: jax.Array,
    B_w_up: jax.Array,
    B_w_down: jax.Array,
    c: jax.Array,
    w_mod: jax.Array,
):
    del B_x
    batch, seq, d = A_x.shape
    assert batch == 1 and d == HEADS * HEAD_DIM and seq == 8 * TILE
    n_tiles = seq // TILE
    operands = (A_x.reshape(seq, d), A_wqkv, A_w_phi, A_wo, B_w_r, B_w_gate, B_w_up, B_w_down,
                c, w_mod)
    weight_terms = pltpu.VMEM((TERMS * d // 4, d // 2), I32)
    scratch = [pltpu.VMEM(a.shape, a.dtype) for a in operands] + [
        weight_terms, weight_terms, weight_terms, weight_terms,
        pltpu.VMEM((TERMS * HALF // 2, d // 2), I32),
        [pltpu.VMEM((TERMS * d // 4, HALF), I32)] * 2,
        pltpu.VMEM((n_tiles * TERMS * d // 4, HALF), I32),
        [pltpu.VMEM((TERMS * HALF // 2, d // 2), I32)] * 2,
        [pltpu.VMEM((TILE, d), F32)] * 2,
        pltpu.VMEM((seq, d), F32),
        pltpu.VMEM((8, 10 * d), F32),
        pltpu.VMEM((HEADS // 2 * PAIR, 128), F32),
        pltpu.VMEM((HEADS // 2 * HEAD_DIM, 128), I32),
        pltpu.VMEM((HEADS // 2 * 128, 128), F32),
        pltpu.VMEM((seq, d), BF16),
        pltpu.VMEM((n_tiles * 8, 128), F32),
        pltpu.VMEM((8, 128), I32),
        pltpu.VMEM((8, d), I32),
        pltpu.VMEM((d // 2, 128), I32),
        pltpu.SemaphoreType.DMA((26,)),
        pltpu.SemaphoreType.DMA((n_tiles // 2,)),
    ]
    out = pl.pallas_call(
        _kernel,
        out_shape=jax.ShapeDtypeStruct((seq, d), A_x.dtype),
        in_specs=[pl.BlockSpec(memory_space=pl.ANY)] * len(operands),
        out_specs=pl.BlockSpec(memory_space=pl.ANY),
        scratch_shapes=scratch,
        compiler_params=pltpu.CompilerParams(vmem_limit_bytes=110 * 2**20, flags=FLAGS or None),
        name="adaln_hedgehog_mod",
    )(*operands)
    return out.reshape(batch, seq, d)
```

```python
import collections
import contextlib
import functools
import math

import jax
import jax.numpy as jnp
from jax import lax
import jax.experimental.pallas as pl
import jax.experimental.pallas.tpu as pltpu

F32 = jnp.float32
BF16 = jnp.bfloat16
I32 = jnp.int32

HEADS = 32
HEAD_DIM = 32
PAIR = 2 * HEAD_DIM
TERMS = 7
LN_EPS = 1e-5
DEN_EPS = 1e-6
LOG2E = math.log2(math.e)

TILE = 256
HALF = TILE // 2
CHUNK = 128
SCOPES = True
LAST_WIN = tuple((7 * (g // 5), 7 * (g // 5) + 9) for g in range(16))
FOLD_GAP = 2
OUT_WIN = tuple((55 + 6 * p, 67 + 6 * p) for p in range(8))
WAIT_AT = (2, 5)
SPLIT = (1, 3)
EARLY_WIN = tuple((6 * n - 1, 6 * n + 16) for n in range(16))
ONLY = None
LN_WIN = (None,) * 8
TR_WIN = (None,) * 7
KF_WIN = None
QF_WIN = None
FIN_WIN = tuple((3 * k - 1, min(3 * k + 11, 55)) for k in range(16))
FFN_CHUNK = 512
FLAGS = {"XLA_TPU_EVENLY_DISTRIBUTE_CRITICAL_NODES": True}

NT_DIMS = (((1,), (1,)), ((), ()))


def _scope(name):
    return jax.named_scope(name) if SCOPES else contextlib.nullcontext()


def _dot(a, b):
    return jnp.dot(a, b, preferred_element_type=F32)


def _dot_nt(a, b):
    return lax.dot_general(a, b, NT_DIMS, preferred_element_type=F32)


def _pack(v):
    return pltpu.bitcast(v.astype(BF16), I32)


def _pack_heads(v):
    starts = range(0, v.shape[0], PAIR)
    first = jnp.concatenate([v[s:s + HEAD_DIM] for s in starts], axis=0)
    second = jnp.concatenate([v[s + HEAD_DIM:s + PAIR] for s in starts], axis=0)
    return pltpu.pack_elementwise([first, second], packed_dtype=BF16).astype(I32)


def _unpack(v):
    return pltpu.bitcast(v, BF16)


def _recip(d):
    r = pltpu.reciprocal(d, approx=True)
    return r * (2.0 - d * r)


def _sigmoid(v):
    return 1.0 / (1.0 + jnp.exp(-v))


def _rows(v, n):
    return jnp.concatenate([v] * (n // 8), axis=0) if n > 8 else v


def _centered(x, after=None):
    inv_d = 1.0 / x.shape[-1]
    if after is not None:
        head = x[:, :128] + _rows(pltpu.bitcast(after, F32), x.shape[0])
        x = jnp.concatenate([head, x[:, 128:]], axis=1)
    xc = x - jnp.sum(x, axis=-1, keepdims=True) * inv_d
    var = jnp.sum(xc * xc, axis=-1, keepdims=True) * inv_d
    return xc, lax.rsqrt(var + LN_EPS)


def _lhs_terms(a11, a12, a21, a22):
    return [a11 + a22, a21 + a22, a11, a22, a11 + a12, a21 - a11, a12 - a22]


def _rhs_terms(b11, b12, b21, b22):
    return [b11 + b22, b11, b12 - b22, b21 - b11, b22, b11 + b12, b21 + b22]


def _block_matmul(product):
    m1 = product(0)
    m4 = product(3)
    c11 = m1 + m4
    c11 = c11 + product(6)
    m5 = product(4)
    c11 = c11 - m5
    m3 = product(2)
    c12 = m3 + m5
    c22 = m1 + m3
    m2 = product(1)
    c21 = m2 + m4
    c22 = c22 - m2
    c22 = c22 + product(5)
    return c11, c12, c21, c22


def _head_reduce(op, tiles):
    while len(tiles) > 1:
        tiles = [op(tiles[i], tiles[i + 1]) for i in range(0, len(tiles), 2)]
    m = tiles[0]
    m = op(m, pltpu.roll(m, 4, 0))
    return op(m, pltpu.roll(m, 2, 0))


def _feature_map(p):
    tiles = [p[8 * j:8 * j + 8] for j in range(PAIR // 8)]
    hi = _head_reduce(jnp.maximum, tiles)
    lo = _head_reduce(jnp.minimum, tiles)
    e_pos = [jnp.exp2(t - hi) for t in tiles]
    e_neg = [jnp.exp2(lo - t) for t in tiles]
    r_pos = _recip(_head_reduce(jnp.add, e_pos))
    r_neg = _recip(_head_reduce(jnp.add, e_neg))
    return [e * r_pos for e in e_pos] + [e * r_neg for e in e_neg]


Tile = collections.namedtuple("Tile", "x h h_all o x1 x1_all out r")
SHIFT_A, SCALE_A, GATE_A, SHIFT_B, SCALE_B, GATE_B, ROUTER, OUT_SCALE, OUT_SHIFT, SCORE = range(10)


def _kernel(x_hbm, wqkv_hbm, wphi_hbm, wo_hbm, wr_hbm, wg_hbm, wu_hbm, wd_hbm, c_hbm, wmod_hbm,
            out_hbm,
            x_v, wqkv_v, wphi_v, wo_v, wr_v, wg_v, wu_v, wd_v, c_v, wmod_v,
            wq_s, wk_s, wv_s, wo_s, n_s, h_s, h_all, o_s, x1_v, x1_all, mod_v, kv_v, kvm_v, z_v, out_v, r_v, zero_v, act_v, phi_s,
            sem, out_sem):
    seq, d = x_v.shape
    hd = d // 2
    n_tiles = seq // TILE
    n_pairs = HEADS // 2
    n_chunks = hd // CHUNK
    chunk_pairs = CHUNK // PAIR
    h_rows = HALF // 2
    w_rows = hd // 2

    def copy(src, dst, s):
        return pltpu.make_async_copy(src, dst, s)

    def token_copy(src, dst, first, count, s):
        return copy(src.at[pl.ds(first, count)], dst.at[pl.ds(first, count)], s)

    def cols(ref, i, n=1):
        return ref.at[:, pl.ds(i * d, n * d)]

    c_cp = copy(c_hbm, c_v, sem.at[0])
    wphi_cp = copy(wphi_hbm, wphi_v, sem.at[1])
    wr_cp = copy(wr_hbm, wr_v, sem.at[2])
    mod_b_cp = copy(cols(wmod_hbm, 2, 4), cols(wmod_v, 2, 4), sem.at[5])
    wq_cp = copy(cols(wqkv_hbm, 0), cols(wqkv_v, 0), sem.at[6])
    wo_cp = copy(wo_hbm, wo_v, sem.at[9])
    wg_cp = copy(wg_hbm, wg_v, sem.at[10])
    wu_cp = copy(wu_hbm, wu_v, sem.at[11])
    wd_cp = copy(wd_hbm, wd_v, sem.at[12])
    x_first_cp = token_copy(x_hbm, x_v, 0, 2 * TILE, sem.at[13])
    x_next_cp = token_copy(x_hbm, x_v, 2 * TILE, TILE, sem.at[14])
    x_rest_cp = token_copy(x_hbm, x_v, 3 * TILE, seq - 3 * TILE, sem.at[15])

    def kv_weight_copies(j):
        spans = [(pl.ds(half * hd + j * 128, 128), pl.ds(d, 2 * d)) for half in range(2)]
        return [copy(wqkv_hbm.at[span], wqkv_v.at[span], sem.at[18 + j]) for span in spans]

    def mod_a_copies(j):
        spans = [pl.ds(part * hd + j * 128, 128) for part in range(4)]
        return [copy(wmod_hbm.at[:, span], wmod_v.at[:, span], sem.at[22 + j]) for span in spans]

    def view(ref, index, size):
        start = index * size
        return ref.at[pl.ds(start if isinstance(start, int) else pl.multiple_of(start, size), size)]

    def tile(i, parity):
        t = 2 * i + parity
        return Tile(x=view(x_v, t, TILE), h=h_s[parity], h_all=view(h_all, t, TERMS * w_rows),
                    o=o_s[parity],
                    x1=x1_v[parity], x1_all=view(x1_all, t, TILE), out=view(out_v, t, TILE), r=view(r_v, t, 8))

    def out_copy(i):
        return copy(view(out_v, i, 2 * TILE), view(out_hbm, i, 2 * TILE), out_sem.at[i])

    def token(values):
        tiles = [pltpu.bitcast(v[r:r + 8, c:c + 128], I32) for v in values
                 for r in range(0, v.shape[0], 8) for c in range(0, v.shape[1], 128)]
        while len(tiles) > 1:
            tiles = [tiles[j] | tiles[j + 1] if j + 1 < len(tiles) else tiles[j]
                     for j in range(0, len(tiles), 2)]
        return tiles[0] & zero_v[...]

    clock = {"now": 0, "last": None, "jobs": {}, "gates": {}}

    def reset_clock():
        assert not clock["jobs"]
        clock.update(last=None, gates={})

    def run_job(job, after, end):
        zero = job(after)
        clock["gates"].setdefault(end, []).append(zero)

    def plan(job, window):
        if window is None:
            job(None)
            return
        start, end = (clock["now"] + w for w in window)
        if start < clock["now"]:
            run_job(job, clock["last"], end)
        else:
            clock["jobs"].setdefault(start, []).append((job, end))

    def timed_dot(lhs, rhs):
        for zero in clock["gates"].pop(clock["now"], []):
            top = jnp.concatenate([lhs[:8, :128] | zero, lhs[:8, 128:]], axis=1)
            lhs = jnp.concatenate([top, lhs[8:]], axis=0)
        out = _dot(_unpack(lhs), _unpack(rhs))
        clock["last"] = token([out[-8:]])
        for job, end in clock["jobs"].pop(clock["now"], []):
            run_job(job, clock["last"], end)
        clock["now"] += 1
        return out

    def store_terms(dst, g, c0, terms):
        packed = [_pack_heads(term) for term in terms]
        for i, term in enumerate(packed):
            dst[i * w_rows + g * 64:i * w_rows + (g + 1) * 64, c0:c0 + term.shape[1]] = term
        return packed

    def store_lhs_terms(dst, g, c0, group):
        top, bottom = group(g), group(g + hd // 128)
        n = top.shape[1] // 2
        return store_terms(
            dst, g, c0, _lhs_terms(top[:, :n], top[:, n:], bottom[:, :n], bottom[:, n:]))

    def feature_blocks():
        row = lax.broadcasted_iota(I32, (128, 128), 0)
        lane = lax.broadcasted_iota(I32, (128, 128), 1)
        same_head = row // HEAD_DIM == lane // HEAD_DIM
        row_f = lax.broadcasted_iota(I32, (128, HEAD_DIM), 0)
        lane_f = lax.broadcasted_iota(I32, (128, HEAD_DIM), 1)
        pick = jnp.where(row_f % HEAD_DIM == lane_f, 1.0, 0.0).astype(BF16)
        for g in range(d // 128):
            wphi = wphi_v[4 * g:4 * g + 4].reshape(128, HEAD_DIM)
            phi_s[g * 64:(g + 1) * 64, :] = _pack(jnp.where(same_head, _dot_nt(pick, wphi), 0.0))

    def folded(w, g):
        return _dot_nt(_unpack(phi_s[g * 64:(g + 1) * 64, :]), w) * LOG2E

    def weight_slice(col, j, g):
        span = slice(col * d + g * 128, col * d + (g + 1) * 128)
        return jnp.concatenate(
            [wqkv_v[half * hd + j * 128:half * hd + (j + 1) * 128, span] for half in range(2)],
            axis=0)

    def folded_terms(col, dst, j, g):
        store_lhs_terms(dst, g, j * 128, lambda g: folded(weight_slice(col, j, g), g))

    def output_terms(p, c, after):
        def block(r0, c0):
            words = pltpu.bitcast(wo_v[r0:r0 + PAIR, c0:c0 + 128], I32) | _rows(after, HEAD_DIM)
            return _unpack(words).astype(F32)

        terms = _rhs_terms(*(block(r + p * PAIR, k + c * 128) for r in (0, hd) for k in (0, hd)))
        packed = [_pack_heads(term) for term in terms]
        for i, term in enumerate(packed):
            r0 = i * w_rows + p * HEAD_DIM
            wo_s[r0:r0 + HEAD_DIM, c * 128:(c + 1) * 128] = term
        return token([term[-8:] for term in packed])

    def vec(i):
        return mod_v[:, i * d:(i + 1) * d]

    def modulation_rounds(i):
        partial = {}

        def one(c0, half):
            span = slice(half * hd, (half + 1) * hd)
            m = _dot(_unpack(act_v[:, span]), wmod_v[span, c0:c0 + 128])[0:8]
            if half == 0:
                partial[c0] = 1.0 + m if i in (SCALE_A, SCALE_B) else m
            else:
                mod_v[:, c0:c0 + 128] = partial[c0] + m

        return [functools.partial(one, c0, half)
                for c0 in range(i * d, (i + 1) * d, 128) for half in range(2)]

    def derived_vectors():
        router = jnp.broadcast_to(wr_v[...].astype(F32).reshape(1, d), (8, d))
        for i, v in ((ROUTER, router), (OUT_SCALE, vec(GATE_B) * vec(SCALE_B)),
                     (OUT_SHIFT, vec(GATE_B) * vec(SHIFT_B)), (SCORE, router * vec(SCALE_B))):
            mod_v[:, i * d:(i + 1) * d] = v

    def normed_rows(t, r0, after=None):
        xc, rstd = _centered(t.x[r0:r0 + 16, :].astype(F32), after)
        return xc * rstd

    def normed_piece(t, k, after=None):
        def normed(start):
            xn = normed_rows(t, start + 16 * k, after)
            return xn * _rows(vec(SCALE_A), 16) + _rows(vec(SHIFT_A), 16)

        ha, hb = normed(0), normed(HALF)
        packed = [_pack(term)
                  for term in _rhs_terms(ha[:, :hd], hb[:, :hd], ha[:, hd:], hb[:, hd:])]
        for j, term in enumerate(packed):
            n_s[j * h_rows + 8 * k:j * h_rows + 8 * k + 8, :] = term
        return token(packed)

    def transposed_term(t, j):
        term = pltpu.bitcast(_unpack(n_s[j * h_rows:(j + 1) * h_rows, :]).T, I32)
        t.h[j * w_rows:(j + 1) * w_rows, :] = term
        t.h_all[j * w_rows:(j + 1) * w_rows, :] = term
        return token([term[r:r + 8] for r in range(56, w_rows, 64)])

    def fetch_term(t, j):
        term = t.h_all[j * w_rows:(j + 1) * w_rows, :]
        t.h[j * w_rows:(j + 1) * w_rows, :] = term

    fillers = []

    def fill():
        if fillers:
            fillers.pop(0)()

    def project(w_s, t, m):
        def product(j):
            w = w_s[j * w_rows + m * CHUNK // 2:j * w_rows + (m + 1) * CHUNK // 2, :]
            h = t.h[j * w_rows:(j + 1) * w_rows, :]
            out = timed_dot(w, h)
            fill()
            return out

        c11, c12, c21, c22 = _block_matmul(product)
        halves = (jnp.concatenate([c11, c12], axis=1), jnp.concatenate([c21, c22], axis=1))
        return [(side * (n_pairs // 2) + m * chunk_pairs + j, block[j * PAIR:(j + 1) * PAIR])
                for side, block in enumerate(halves) for j in range(chunk_pairs)]

    def key_features(p, pk):
        phi = jnp.concatenate(_feature_map(pk), axis=0)
        z_v[p * 128:(p + 1) * 128, :] += phi[:, :HALF] + phi[:, HALF:]
        return p, phi.astype(BF16)

    def accumulate_kv(phi, v):
        for (_, phi_p), (p, v_p) in zip(phi, v, strict=True):
            kv_v[p * PAIR:(p + 1) * PAIR, :] += _dot_nt(v_p.astype(BF16), phi_p)

    def features(fn, pairs, windows):
        if windows is None:
            return [fn(*pair) for pair in pairs]
        out = []

        def job(p, block, after):
            if after is not None:
                block = block + _rows(jnp.concatenate([pltpu.bitcast(after, F32)] * 2, axis=1), PAIR)
            out.append(fn(p, block))
            return token([pltpu.bitcast(out[-1][1][-16:], I32)])

        for pair, window in zip(pairs, windows):
            plan(functools.partial(job, *pair), window)
        return out

    def summarize(t, pending, between=lambda: None):
        for m in range(n_chunks):
            pk = project(wk_s, t, m)
            if pending is not None:
                accumulate_kv(*pending)
            between()
            phi = features(key_features, pk, KF_WIN)
            pending = (phi, project(wv_s, t, m))
            between()
        return pending

    def normalize(t, ln_windows, tr_windows):
        for k, window in enumerate(ln_windows):
            plan(functools.partial(normed_piece, t, k), window)
        for j, window in enumerate(tr_windows):
            plan(lambda after, j=j: transposed_term(t, j), window)

    def query_features(p, pq):
        phi = _feature_map(pq)
        z = [z_v[p * 128 + 8 * j:p * 128 + 8 * j + 8, :] for j in range(len(phi))]
        den = _head_reduce(
            jnp.add, [f * jnp.concatenate([zj, zj], axis=1) for f, zj in zip(phi, z)])
        return p, jnp.concatenate(phi, axis=0).astype(BF16), _recip(den + DEN_EPS)

    def read_out(t, m, features):
        o_t = [_dot(_unpack(kvm_v[p * HEAD_DIM:(p + 1) * HEAD_DIM, :]), phi) * _rows(inv, PAIR)
               for p, phi, inv in features]
        top = jnp.concatenate(o_t[:chunk_pairs], axis=0)
        bottom = jnp.concatenate(o_t[chunk_pairs:], axis=0)
        terms = _lhs_terms(top[:, :HALF], bottom[:, :HALF], top[:, HALF:], bottom[:, HALF:])
        for j, term in enumerate(terms):
            t.o[j * h_rows:(j + 1) * h_rows, m * CHUNK:(m + 1) * CHUNK] = pltpu.bitcast(
                term.astype(BF16).T, I32)

    def residual(t, g, first=0, count=HALF):
        def product(j):
            o = t.o[j * h_rows + first // 2:j * h_rows + (first + count) // 2, :]
            w = wo_s[j * w_rows:(j + 1) * w_rows, g * 128:(g + 1) * 128]
            out = timed_dot(o, w)
            fill()
            return out

        for b, attn in enumerate(_block_matmul(product)):
            r0 = (b // 2) * HALF + first
            c0 = (b % 2) * hd + g * 128
            gate = _rows(mod_v[:, GATE_A * d + c0:GATE_A * d + c0 + 128], count)
            x1 = t.x[r0:r0 + count, c0:c0 + 128].astype(F32) + gate * attn
            t.x1[r0:r0 + count, c0:c0 + 128] = x1
            t.x1_all[r0:r0 + count, c0:c0 + 128] = x1

    def finish(t, g, after=None):
        x1 = t.x1[16 * g:16 * g + 16, :]
        xc, rstd = _centered(x1, after)
        out = x1 + (xc * rstd * _rows(vec(OUT_SCALE), 16) + _rows(vec(OUT_SHIFT), 16))
        t.out[16 * g:16 * g + 16, :] = out.astype(BF16)
        score = jnp.sum(xc * _rows(vec(SCORE), 16), axis=-1, keepdims=True) * rstd
        lane = lax.broadcasted_iota(I32, (8, 128), 1)
        packed = t.r[...]
        for s in range(2):
            packed = jnp.where(lane == 2 * g + s, score[8 * s:8 * s + 8], packed)
        t.r[...] = packed
        return token([packed, out[:, -128:]])

    def fetch(t):
        for j in range(TERMS):
            fetch_term(t, j)

    def finishing(t, windows):
        for g, window in enumerate(windows):
            plan(functools.partial(finish, t, g), window)

    def attend(t, middle):
        ready = features(query_features, project(wq_s, t, 0), QF_WIN)
        for m in range(n_chunks):
            if m + 1 < n_chunks:
                ahead = features(query_features, project(wq_s, t, m + 1),
                                 QF_WIN if middle else None)
                if middle:
                    middle(m)
                read_out(t, m, ready)
                ready = ahead
            else:
                read_out(t, m, ready)
                if middle:
                    middle(m)

    def partial_product(i):
        return x1_all.at[pl.ds(i // 4 * hd, hd), pl.ds(i % 4 * TILE, TILE)]

    def start_up():
        early = (tile(0, 0), tile(0, 1))
        cf = c_v[...].astype(F32)
        act_v[...] = _pack(jnp.broadcast_to(cf * _sigmoid(cf), (16, d)))
        wphi_cp.wait()
        feature_blocks()
        def slices(j):
            return slice(j * 128, (j + 1) * 128), slice(hd + j * 128, hd + (j + 1) * 128)

        def activation_terms(j):
            for cp in mod_a_copies(j):
                cp.wait()
            lo, hi = slices(j)
            parts = [slice(part * hd + j * 128, part * hd + (j + 1) * 128) for part in range(4)]
            m = _dot(_unpack(act_v[...]),
                     jnp.concatenate([wmod_v[:, part] for part in parts], axis=1))[0:8]
            vectors = [m[:, :128], m[:, 128:256], 1.0 + m[:, 256:384], 1.0 + m[:, 384:]]
            for part, v in zip(parts, vectors):
                mod_v[:, part] = v
            shift_lo, shift_hi, scale_lo, scale_hi = (_rows(v, HALF) for v in vectors)
            for t in early:
                terms = _rhs_terms(t.x1[:HALF, lo] * scale_lo + shift_lo,
                                   t.x1[HALF:, lo] * scale_lo + shift_lo,
                                   t.x1[:HALF, hi] * scale_hi + shift_hi,
                                   t.x1[HALF:, hi] * scale_hi + shift_hi)
                for i, term in enumerate(terms):
                    t.h_all[i * w_rows + j * 64:i * w_rows + (j + 1) * 64, :] = pltpu.bitcast(
                        term.astype(BF16).T, I32)

        def weight_terms(j):
            for cp in kv_weight_copies(j):
                cp.wait()

            for g in range(n_chunks):
                folded_terms(1, wk_s, j, g)
                store_lhs_terms(wv_s, g, j * 128, lambda g: weight_slice(2, j, g).astype(F32).T)

        x_first_cp.wait()
        for t in early:
            for r0 in range(0, TILE, 16):
                t.x1[r0:r0 + 16, :] = normed_rows(t, r0)
        weight_terms(0)
        activation_terms(0)
        for j in range(n_chunks):
            for i in range(TERMS):
                if i == WAIT_AT[0] and j + 1 < n_chunks:
                    weight_terms(j + 1)
                if i == WAIT_AT[1] and j + 1 < n_chunks:
                    activation_terms(j + 1)
                if i == 0 and j + 1 == n_chunks:
                    x_next_cp.wait()
                    normalize(tile(1, 0), LN_WIN, TR_WIN)
                h = jnp.concatenate(
                    [t.h_all[i * w_rows + j * 64:i * w_rows + (j + 1) * 64, :] for t in early],
                    axis=1)
                for k, w_s in enumerate((wk_s, wv_s)):
                    acc = partial_product(k * TERMS + i)
                    w = w_s[i * w_rows:(i + 1) * w_rows, j * 128:(j + 1) * 128]
                    product = _dot(_unpack(w), _unpack(h))
                    acc[...] = product + acc[...] if j else product
        for cp in (wq_cp, wo_cp, wr_cp):
            cp.start()

    def early_features(q, b, after):
        def block(k):
            return _block_matmul(
                lambda i: partial_product(k * TERMS + i)[q * PAIR:(q + 1) * PAIR, :])[b]

        pk = block(0)
        if after is not None:
            pk = pk + _rows(jnp.concatenate([pltpu.bitcast(after, F32)] * 2, axis=1), PAIR)
        p = b // 2 * (n_pairs // 2) + q
        return [key_features(p, pk)], [(p, block(1))]

    def summarize_pair(i, copies):
        ready = []

        def job(n, end, after):
            ready.append((end, early_features(n // 4, n % 4, after)))
            return token([pltpu.bitcast(ready[-1][1][0][0][1][-16:], I32)])

        def drain():
            while ready and ready[0][0] <= clock["now"]:
                accumulate_kv(*ready.pop(0)[1])

        for n, window in enumerate(EARLY_WIN):
            plan(functools.partial(job, (i - 1) * len(EARLY_WIN) + n, clock["now"] + window[1]),
                 window)
        copies[0].start()
        normalize(tile(i, 1), LN_WIN, TR_WIN)
        pending = summarize(tile(i, 0), None, drain)
        copies[1].start()
        normalize(tile(i + 1, 0), LN_WIN, TR_WIN)
        pending = summarize(tile(i, 1), pending, drain)
        accumulate_kv(*pending)
        assert not ready

    def second_tiles():
        x_rest_cp.wait()
        summarize_pair(1, (mod_b_cp, wg_cp))

    def third_tiles():
        summarize_pair(2, (wu_cp, wd_cp))

    last = n_tiles // 2 - 1

    def last_tiles():
        for cp in (wq_cp, wo_cp, wr_cp, mod_b_cp):
            cp.wait()
        normalize(tile(last, 1), LN_WIN, TR_WIN)
        for p, window in enumerate(OUT_WIN):
            for c in range(n_chunks):
                plan(functools.partial(output_terms, p, c), window)
        for j in range(n_chunks):
            for g in range(n_chunks):
                fillers.append(functools.partial(folded_terms, 0, wq_s, j, g))
                fillers.extend([lambda: None] * FOLD_GAP)
        pending = summarize(tile(last, 0), None)
        accumulate_kv(*summarize(tile(last, 1), pending))
        assert not fillers

    def first_read_outs():
        row = lax.broadcasted_iota(I32, (PAIR, 128), 0)
        lane = lax.broadcasted_iota(I32, (PAIR, 128), 1)
        for p in range(n_pairs):
            kv = jnp.where(row % 2 == lane % 2, kv_v[p * PAIR:(p + 1) * PAIR, :], 0.0)
            kvm_v[p * HEAD_DIM:(p + 1) * HEAD_DIM, :] = _pack(kv)
            z = jnp.sum(z_v[p * 128:(p + 1) * 128, :], axis=1, keepdims=True)
            z_v[p * 128:(p + 1) * 128, :] = jnp.broadcast_to(z, (128, 128))
        for i in (GATE_A, SHIFT_B, SCALE_B, GATE_B):
            fillers.extend(modulation_rounds(i))
        fetch(tile(0, 0))
        fetch(tile(0, 1))
        attend(tile(0, 0), None)
        fetch(tile(1, 0))
        attend(tile(0, 1), functools.partial(residual, tile(0, 0)))
        assert not fillers
        derived_vectors()

    def attend_tiles():
        def body(i, carry):
            reset_clock()
            tiles = [tile(i - 1, 0), tile(i - 1, 1), tile(i, 0), tile(i, 1)]
            tiles.append(tile(jnp.minimum(i + 1, last), 0))
            for k in range(2):
                fetch(tiles[k + 3])
                finishing(tiles[k], FIN_WIN)
                attend(tiles[k + 2], functools.partial(residual, tiles[k + 1]))
            out_copy(i - 1).start()
            return carry
        lax.fori_loop(1, last + 1, body, 0)

    def last_tile():
        final = tile(last, 1)
        finishing(tile(last, 0), LAST_WIN)
        for g in range(n_chunks):
            residual(final, g, 0, HALF // 2)
        groups = HALF // 32
        for n, g in enumerate(side * 2 * groups + g for side in range(2) for g in range(groups)):
            plan(functools.partial(finish, final, g), (7 * (n // 3) - 1, 7 * (n // 3) + 9))
        for g in range(n_chunks):
            residual(final, g, HALF // 2, HALF // 2)
        for side in range(2):
            for g in range(groups):
                finish(final, (2 * side + 1) * groups + g)
        out_copy(last).start()

    def route():
        scores = r_v[...]
        row = lax.broadcasted_iota(I32, scores.shape, 0)
        lane = lax.broadcasted_iota(I32, scores.shape, 1)
        index = jnp.where(lane < TILE // 8, (row // 8) * TILE + lane * 8 + row % 8, seq)

        def arg_top(valid):
            best = jnp.max(jnp.where(valid, scores, -jnp.inf))
            first = jnp.min(jnp.where(valid & (scores == best), index, seq).astype(F32))
            return jnp.minimum(first.astype(I32), seq - 1)

        i0 = arg_top(index < seq)
        i1 = arg_top((index < seq) & (index != i0))

        sub = lax.broadcasted_iota(I32, (16, d), 0)
        x1 = jnp.where(sub == 0, x1_all[pl.ds(i0, 1), :], x1_all[pl.ds(i1, 1), :])
        xc, rstd = _centered(x1)
        h2 = xc * rstd * _rows(vec(SCALE_B), 16) + _rows(vec(SHIFT_B), 16)
        gate = _sigmoid(jnp.sum(h2 * _rows(vec(ROUTER), 16), axis=-1, keepdims=True))
        xs = h2.astype(BF16)
        for cp in (wg_cp, wu_cp, wd_cp):
            cp.wait()
        spans = [slice(f, f + FFN_CHUNK) for f in range(0, wd_v.shape[0], FFN_CHUNK)]
        y, hidden = 0.0, None
        for k in range(len(spans) + 1):
            if k < len(spans):
                g = _dot(xs, wg_v[:, spans[k]])
                u = _dot(xs, wu_v[:, spans[k]])
            if k > 0:
                y = y + _dot(hidden, wd_v[spans[k - 1], :])
            hidden = (g * _sigmoid(g) * u).astype(BF16)
        routed = x1 + _rows(vec(GATE_B), 16) * (h2 + y * gate)

        for i in range(last + 1):
            out_copy(i).wait()

        def patch(k, i):
            base = pl.multiple_of((i // 16) * 16, 16)
            old = out_v[pl.ds(base, 16), :].astype(F32)
            out_v[pl.ds(base, 16), :] = jnp.where(
                sub == i - base, routed[k:k + 1], old).astype(BF16)
            return base, copy(out_v.at[pl.ds(base, 16)], out_hbm.at[pl.ds(base, 16)],
                              sem.at[16 + k])

        base0, patch0 = patch(0, i0)
        base1, patch1 = patch(1, i1)
        patch0.start()

        @pl.when(base1 != base0)
        def _():
            patch1.start()
            patch1.wait()

        patch0.wait()

    for cp in (c_cp, wphi_cp, x_first_cp):
        cp.start()
    for j in range(n_chunks):
        for cp in kv_weight_copies(j) + mod_a_copies(j):
            cp.start()
    x_next_cp.start()
    x_rest_cp.start()
    kv_v[...] = jnp.zeros(kv_v.shape, F32)
    z_v[...] = jnp.zeros(z_v.shape, F32)
    r_v[...] = jnp.full(r_v.shape, -jnp.inf, F32)
    c_cp.wait()
    words = pltpu.bitcast(jnp.broadcast_to(c_v[:, :128].astype(F32), (8, 128)), I32)
    zero = jnp.minimum(lax.shift_right_logical(words, 1), 0)
    zero_v[...] = zero
    origin = jnp.max(zero)
    steps = (start_up, second_tiles, third_tiles, last_tiles, first_read_outs, attend_tiles,
             last_tile, route)
    for k, step in enumerate(steps):
        if ONLY is None or ONLY == k:
            with _scope(step.__name__):
                reset_clock()
                if k in SPLIT:
                    pl.when(origin <= k)(step)
                else:
                    step()
    if ONLY is not None:
        probe = pl.ds(pl.multiple_of(origin * 8, 8), 8)
        total = jnp.zeros((8, 128), F32)
        for ref in (wq_s, wk_s, wv_s, wo_s, n_s, *h_s, h_all, *o_s, *x1_v, x1_all, kv_v, kvm_v, z_v, r_v):
            total = total + ref[probe, 0:128].astype(F32)
        out_v[0:8, 0:128] = total.astype(BF16)
        last_copy = copy(out_v, out_hbm, sem.at[16])
        last_copy.start()
        last_copy.wait()


@jax.jit
def pallas_adaLN_cond__linear_kernel_hedgehog__moe_arch_mod__prompt_kernel(
    A_x: jax.Array,
    A_wqkv: jax.Array,
    A_w_phi: jax.Array,
    A_wo: jax.Array,
    B_x: jax.Array,
    B_w_r: jax.Array,
    B_w_gate: jax.Array,
    B_w_up: jax.Array,
    B_w_down: jax.Array,
    c: jax.Array,
    w_mod: jax.Array,
):
    del B_x
    batch, seq, d = A_x.shape
    assert batch == 1 and d == HEADS * HEAD_DIM and seq == 8 * TILE
    n_tiles = seq // TILE
    operands = (A_x.reshape(seq, d), A_wqkv, A_w_phi, A_wo, B_w_r, B_w_gate, B_w_up, B_w_down,
                c, w_mod)
    weight_terms = pltpu.VMEM((TERMS * d // 4, d // 2), I32)
    scratch = [pltpu.VMEM(a.shape, a.dtype) for a in operands] + [
        weight_terms, weight_terms, weight_terms, weight_terms,
        pltpu.VMEM((TERMS * HALF // 2, d // 2), I32),
        [pltpu.VMEM((TERMS * d // 4, HALF), I32)] * 2,
        pltpu.VMEM((n_tiles * TERMS * d // 4, HALF), I32),
        [pltpu.VMEM((TERMS * HALF // 2, d // 2), I32)] * 2,
        [pltpu.VMEM((TILE, d), F32)] * 2,
        pltpu.VMEM((seq, d), F32),
        pltpu.VMEM((8, 10 * d), F32),
        pltpu.VMEM((HEADS // 2 * PAIR, 128), F32),
        pltpu.VMEM((HEADS // 2 * HEAD_DIM, 128), I32),
        pltpu.VMEM((HEADS // 2 * 128, 128), F32),
        pltpu.VMEM((seq, d), BF16),
        pltpu.VMEM((n_tiles * 8, 128), F32),
        pltpu.VMEM((8, 128), I32),
        pltpu.VMEM((8, d), I32),
        pltpu.VMEM((d // 2, 128), I32),
        pltpu.SemaphoreType.DMA((26,)),
        pltpu.SemaphoreType.DMA((n_tiles // 2,)),
    ]
    out = pl.pallas_call(
        _kernel,
        out_shape=jax.ShapeDtypeStruct((seq, d), A_x.dtype),
        in_specs=[pl.BlockSpec(memory_space=pl.ANY)] * len(operands),
        out_specs=pl.BlockSpec(memory_space=pl.ANY),
        scratch_shapes=scratch,
        compiler_params=pltpu.CompilerParams(vmem_limit_bytes=110 * 2**20, flags=FLAGS or None),
        name="adaln_hedgehog_mod",
    )(*operands)
    return out.reshape(batch, seq, d)
```

```python
import collections
import functools
import math

import jax
import jax.numpy as jnp
from jax import lax
import jax.experimental.pallas as pl
import jax.experimental.pallas.tpu as pltpu

F32 = jnp.float32
BF16 = jnp.bfloat16
I32 = jnp.int32

HEADS = 32
HEAD_DIM = 32
PAIRS = HEADS // 2
PAIR = 2 * HEAD_DIM
TERMS = 7
TILE = 256
HALF = TILE // 2
CHUNK = 128
FFN_CHUNK = 512
LN_EPS = 1e-5
DEN_EPS = 1e-6
LOG2E = math.log2(math.e)

EARLY_WINDOWS = tuple((6 * n - 1, 6 * n + 16) for n in range(16))
OUTPUT_WINDOWS = tuple((55 + 6 * p, 67 + 6 * p) for p in range(8))
FINISH_WINDOWS = tuple((3 * g - 1, min(3 * g + 11, 55)) for g in range(16))
LAST_WINDOWS = tuple((7 * (g // 5), 7 * (g // 5) + 9) for g in range(16))
TAIL_WINDOWS = tuple((7 * (n // 3) - 1, 7 * (n // 3) + 9) for n in range(8))

QUERY, KEY, VALUE = range(3)
SHIFT_A, SCALE_A, GATE_A, SHIFT_B, SCALE_B, GATE_B, ROUTER, OUT_SCALE, OUT_SHIFT, SCORE = range(10)

Tile = collections.namedtuple("Tile", "x h h_all o x1 x1_all out score")


def _dot(a, b):
    return jnp.dot(a, b, preferred_element_type=F32)


def _dot_nt(a, b):
    return lax.dot_general(a, b, (((1,), (1,)), ((), ())), preferred_element_type=F32)


def _pack(v):
    return pltpu.bitcast(v.astype(BF16), I32)


def _pack_heads(v):
    starts = range(0, v.shape[0], PAIR)
    first = jnp.concatenate([v[s:s + HEAD_DIM] for s in starts], axis=0)
    second = jnp.concatenate([v[s + HEAD_DIM:s + PAIR] for s in starts], axis=0)
    return pltpu.pack_elementwise([first, second], packed_dtype=BF16).astype(I32)


def _pack_transposed(v):
    return pltpu.bitcast(v.astype(BF16).T, I32)


def _unpack(words):
    return pltpu.bitcast(words, BF16)


def _recip(v):
    r = pltpu.reciprocal(v, approx=True)
    return r * (2.0 - v * r)


def _sigmoid(v):
    return 1.0 / (1.0 + jnp.exp(-v))


def _rows(v, n):
    return jnp.concatenate([v] * (n // 8), axis=0)


def _centered(x, after=None):
    inv_d = 1.0 / x.shape[-1]
    if after is not None:
        head = x[:, :128] + _rows(pltpu.bitcast(after, F32), x.shape[0])
        x = jnp.concatenate([head, x[:, 128:]], axis=1)
    xc = x - jnp.sum(x, axis=-1, keepdims=True) * inv_d
    var = jnp.sum(xc * xc, axis=-1, keepdims=True) * inv_d
    return xc, lax.rsqrt(var + LN_EPS)


def _lhs_terms(a11, a12, a21, a22):
    return [a11 + a22, a21 + a22, a11, a22, a11 + a12, a21 - a11, a12 - a22]


def _rhs_terms(b11, b12, b21, b22):
    return [b11 + b22, b11, b12 - b22, b21 - b11, b22, b11 + b12, b21 + b22]


def _block_matmul(product):
    m1 = product(0)
    m4 = product(3)
    c11 = m1 + m4
    c11 = c11 + product(6)
    m5 = product(4)
    c11 = c11 - m5
    m3 = product(2)
    c12 = m3 + m5
    c22 = m1 + m3
    m2 = product(1)
    c21 = m2 + m4
    c22 = c22 - m2
    c22 = c22 + product(5)
    return c11, c12, c21, c22


def _head_reduce(op, tiles):
    while len(tiles) > 1:
        tiles = [op(tiles[i], tiles[i + 1]) for i in range(0, len(tiles), 2)]
    m = tiles[0]
    m = op(m, pltpu.roll(m, 4, 0))
    return op(m, pltpu.roll(m, 2, 0))


def _feature_map(p):
    tiles = [p[8 * j:8 * j + 8] for j in range(PAIR // 8)]
    hi = _head_reduce(jnp.maximum, tiles)
    lo = _head_reduce(jnp.minimum, tiles)
    e_pos = [jnp.exp2(t - hi) for t in tiles]
    e_neg = [jnp.exp2(lo - t) for t in tiles]
    r_pos = _recip(_head_reduce(jnp.add, e_pos))
    r_neg = _recip(_head_reduce(jnp.add, e_neg))
    return [e * r_pos for e in e_pos] + [e * r_neg for e in e_neg]


class _Pacer:
    def __init__(self, zero_ref):
        self.zero_ref = zero_ref
        self.now = 0
        self.last = None
        self.jobs, self.gates, self.fillers = {}, {}, []

    def reset(self):
        assert not self.jobs and not self.fillers
        self.last, self.gates = None, {}

    def token(self, values):
        tiles = [pltpu.bitcast(v[r:r + 8, c:c + 128], I32) for v in values
                 for r in range(0, v.shape[0], 8) for c in range(0, v.shape[1], 128)]
        while len(tiles) > 1:
            tiles = [tiles[j] | tiles[j + 1] if j + 1 < len(tiles) else tiles[j]
                     for j in range(0, len(tiles), 2)]
        return tiles[0] & self.zero_ref[...]

    def plan(self, job, window):
        start, end = (self.now + w for w in window)
        if start < self.now:
            self._run(job, end)
        else:
            self.jobs.setdefault(start, []).append((job, end))

    def _run(self, job, end):
        self.gates.setdefault(end, []).append(job(self.last))

    def dot(self, lhs, rhs):
        for zero in self.gates.pop(self.now, []):
            top = jnp.concatenate([lhs[:8, :128] | zero, lhs[:8, 128:]], axis=1)
            lhs = jnp.concatenate([top, lhs[8:]], axis=0)
        out = _dot(_unpack(lhs), _unpack(rhs))
        self.last = self.token([out[-8:]])
        for job, end in self.jobs.pop(self.now, []):
            self._run(job, end)
        self.now += 1
        if self.fillers:
            self.fillers.pop(0)()
        return out


def _kernel(x_hbm, wqkv_hbm, wphi_hbm, wo_hbm, wr_hbm, wg_hbm, wu_hbm, wd_hbm, c_hbm, wmod_hbm,
            out_hbm,
            x_v, wqkv_v, wphi_v, wo_v, wr_v, wg_v, wu_v, wd_v, c_v, wmod_v,
            wq_s, wk_s, wv_s, wo_s, phi_s, act_s, vec_s, norm_s, h_s, h_all, o_s, x1_s, x1_all,
            kv_s, kvm_s, z_s, score_s, zero_s, out_v,
            sem):
    seq, d = x_v.shape
    hd = d // 2
    last = seq // (2 * TILE) - 1
    n_chunks = hd // CHUNK
    h_rows = HALF // 2
    w_rows = hd // 2
    pacer = _Pacer(zero_s)

    copy = pltpu.make_async_copy

    def view(ref, index, size):
        start = index * size
        return ref.at[pl.ds(start if isinstance(start, int) else pl.multiple_of(start, size), size)]

    def x_copy(first, count, s):
        return copy(x_hbm.at[pl.ds(first, count)], x_v.at[pl.ds(first, count)], s)

    c_cp = copy(c_hbm, c_v, sem.at[0])
    wphi_cp = copy(wphi_hbm, wphi_v, sem.at[1])
    wr_cp = copy(wr_hbm, wr_v, sem.at[2])
    mod_b_cp = copy(wmod_hbm.at[:, pl.ds(2 * d, 4 * d)], wmod_v.at[:, pl.ds(2 * d, 4 * d)],
                    sem.at[3])
    wq_cp = copy(wqkv_hbm.at[:, pl.ds(0, d)], wqkv_v.at[:, pl.ds(0, d)], sem.at[4])
    wo_cp = copy(wo_hbm, wo_v, sem.at[5])
    wg_cp = copy(wg_hbm, wg_v, sem.at[6])
    wu_cp = copy(wu_hbm, wu_v, sem.at[7])
    wd_cp = copy(wd_hbm, wd_v, sem.at[8])
    x_first_cp = x_copy(0, 2 * TILE, sem.at[9])
    x_next_cp = x_copy(2 * TILE, TILE, sem.at[10])
    x_rest_cp = x_copy(3 * TILE, seq - 3 * TILE, sem.at[11])

    def weight_copies(j):
        spans = [(pl.ds(half * hd + j * CHUNK, CHUNK), pl.ds(d, 2 * d)) for half in range(2)]
        return [copy(wqkv_hbm.at[span], wqkv_v.at[span], sem.at[12 + j]) for span in spans]

    def mod_a_copies(j):
        spans = [pl.ds(part * hd + j * CHUNK, CHUNK) for part in range(4)]
        return [copy(wmod_hbm.at[:, span], wmod_v.at[:, span], sem.at[16 + j]) for span in spans]

    def out_copy(i):
        return copy(view(out_v, i, 2 * TILE), view(out_hbm, i, 2 * TILE), sem.at[20 + i])

    def tile(i, parity):
        t = 2 * i + parity
        return Tile(x=view(x_v, t, TILE), h=h_s[parity], h_all=view(h_all, t, TERMS * w_rows),
                    o=o_s[parity], x1=x1_s[parity], x1_all=view(x1_all, t, TILE),
                    out=view(out_v, t, TILE), score=view(score_s, t, 8))

    def feature_blocks():
        row = lax.broadcasted_iota(I32, (128, 128), 0)
        lane = lax.broadcasted_iota(I32, (128, 128), 1)
        same_head = row // HEAD_DIM == lane // HEAD_DIM
        row_f = lax.broadcasted_iota(I32, (128, HEAD_DIM), 0)
        lane_f = lax.broadcasted_iota(I32, (128, HEAD_DIM), 1)
        pick = jnp.where(row_f % HEAD_DIM == lane_f, 1.0, 0.0).astype(BF16)
        for g in range(d // 128):
            wphi = wphi_v[4 * g:4 * g + 4].reshape(128, HEAD_DIM)
            phi_s[g * 64:(g + 1) * 64, :] = _pack(jnp.where(same_head, _dot_nt(pick, wphi), 0.0))

    def projection_terms(col, j, g):
        def group(g):
            span = slice(col * d + g * CHUNK, col * d + (g + 1) * CHUNK)
            w = jnp.concatenate(
                [wqkv_v[r + j * CHUNK:r + (j + 1) * CHUNK, span] for r in (0, hd)], axis=0)
            if col == VALUE:
                return w.astype(F32).T
            return _dot_nt(_unpack(phi_s[g * 64:(g + 1) * 64, :]), w) * LOG2E

        top, bottom = group(g), group(g + n_chunks)
        terms = _lhs_terms(top[:, :CHUNK], top[:, CHUNK:], bottom[:, :CHUNK], bottom[:, CHUNK:])
        for i, term in enumerate(terms):
            r0 = i * w_rows + g * CHUNK // 2
            (wq_s, wk_s, wv_s)[col][r0:r0 + CHUNK // 2, j * CHUNK:(j + 1) * CHUNK] = (
                _pack_heads(term))

    def output_terms(p, c, after):
        def block(r0, c0):
            words = pltpu.bitcast(wo_v[r0:r0 + PAIR, c0:c0 + CHUNK], I32) | _rows(after, HEAD_DIM)
            return _unpack(words).astype(F32)

        blocks = (block(r + p * PAIR, k + c * CHUNK) for r in (0, hd) for k in (0, hd))
        packed = [_pack_heads(term) for term in _rhs_terms(*blocks)]
        for i, term in enumerate(packed):
            r0 = i * w_rows + p * HEAD_DIM
            wo_s[r0:r0 + HEAD_DIM, c * CHUNK:(c + 1) * CHUNK] = term
        return pacer.token([term[-8:] for term in packed])

    def vec(i):
        return vec_s[:, i * d:(i + 1) * d]

    def modulation_rounds(i):
        partial = {}

        def one(c0, half):
            span = slice(half * hd, (half + 1) * hd)
            m = _dot(_unpack(act_s[:, span]), wmod_v[span, c0:c0 + 128])[0:8]
            if half == 0:
                partial[c0] = 1.0 + m if i == SCALE_B else m
            else:
                vec_s[:, c0:c0 + 128] = partial[c0] + m

        return [functools.partial(one, c0, half)
                for c0 in range(i * d, (i + 1) * d, 128) for half in range(2)]

    def derived_vectors():
        router = jnp.broadcast_to(wr_v[...].astype(F32).reshape(1, d), (8, d))
        for i, v in ((ROUTER, router), (OUT_SCALE, vec(GATE_B) * vec(SCALE_B)),
                     (OUT_SHIFT, vec(GATE_B) * vec(SHIFT_B)), (SCORE, router * vec(SCALE_B))):
            vec_s[:, i * d:(i + 1) * d] = v

    def normed_rows(t, r0):
        xc, rstd = _centered(t.x[r0:r0 + 16, :].astype(F32))
        return xc * rstd

    def normalize(t):
        for r0 in range(0, HALF, 16):
            ha, hb = (normed_rows(t, r + r0) * _rows(vec(SCALE_A), 16) + _rows(vec(SHIFT_A), 16)
                      for r in (0, HALF))
            for j, term in enumerate(_rhs_terms(ha[:, :hd], hb[:, :hd], ha[:, hd:], hb[:, hd:])):
                norm_s[j * h_rows + r0 // 2:j * h_rows + r0 // 2 + 8, :] = _pack(term)
        for j in range(TERMS):
            term = _pack_transposed(_unpack(norm_s[j * h_rows:(j + 1) * h_rows, :]))
            t.h[j * w_rows:(j + 1) * w_rows, :] = term
            t.h_all[j * w_rows:(j + 1) * w_rows, :] = term

    def fetch(t):
        for j in range(TERMS):
            t.h[j * w_rows:(j + 1) * w_rows, :] = t.h_all[j * w_rows:(j + 1) * w_rows, :]

    def project(w_s, t, m):
        def product(j):
            r0 = j * w_rows + m * CHUNK // 2
            return pacer.dot(w_s[r0:r0 + CHUNK // 2, :], t.h[j * w_rows:(j + 1) * w_rows, :])

        c11, c12, c21, c22 = _block_matmul(product)
        halves = (jnp.concatenate([c11, c12], axis=1), jnp.concatenate([c21, c22], axis=1))
        return [(side * PAIRS // 2 + m * CHUNK // PAIR + j, block[j * PAIR:(j + 1) * PAIR])
                for side, block in enumerate(halves) for j in range(CHUNK // PAIR)]

    def key_features(p, pk):
        phi = jnp.concatenate(_feature_map(pk), axis=0)
        z_s[p * 128:(p + 1) * 128, :] += phi[:, :HALF] + phi[:, HALF:]
        return phi.astype(BF16)

    def accumulate_kv(phi, v):
        for phi_p, (p, v_p) in zip(phi, v, strict=True):
            kv_s[p * PAIR:(p + 1) * PAIR, :] += _dot_nt(v_p.astype(BF16), phi_p)

    def summarize(t, owed, between=lambda: None, flush=False):
        for m in range(n_chunks):
            pk = project(wk_s, t, m)
            if not (flush and m + 1 == n_chunks):
                while owed:
                    accumulate_kv(*owed.pop(0))
            between()
            owed.append(([key_features(*pair) for pair in pk], project(wv_s, t, m)))
            between()
        while flush and owed:
            accumulate_kv(*owed.pop(0))
        return owed

    def early_product(col, i):
        n = (col - KEY) * TERMS + i
        return x1_all.at[pl.ds(n // 4 * hd, hd), pl.ds(n % 4 * TILE, TILE)]

    def early_features(q, b):
        def block(col):
            return _block_matmul(lambda i: early_product(col, i)[q * PAIR:(q + 1) * PAIR, :])[b]

        return b // 2 * PAIRS // 2 + q, block(KEY), block(VALUE)

    def query_features(p, pq):
        phi = _feature_map(pq)
        z = [z_s[p * 128 + 8 * j:p * 128 + 8 * j + 8, :] for j in range(len(phi))]
        den = _head_reduce(
            jnp.add, [f * jnp.concatenate([zj, zj], axis=1) for f, zj in zip(phi, z)])
        return p, jnp.concatenate(phi, axis=0).astype(BF16), _recip(den + DEN_EPS)

    def queries(t, m):
        return [query_features(*pair) for pair in project(wq_s, t, m)]

    def read_out(t, m, features):
        o_t = [_dot(_unpack(kvm_s[p * HEAD_DIM:(p + 1) * HEAD_DIM, :]), phi) * _rows(inv, PAIR)
               for p, phi, inv in features]
        top = jnp.concatenate(o_t[:len(o_t) // 2], axis=0)
        bottom = jnp.concatenate(o_t[len(o_t) // 2:], axis=0)
        terms = _lhs_terms(top[:, :HALF], bottom[:, :HALF], top[:, HALF:], bottom[:, HALF:])
        for j, term in enumerate(terms):
            t.o[j * h_rows:(j + 1) * h_rows, m * CHUNK:(m + 1) * CHUNK] = _pack_transposed(term)

    def residual(t, g, first=0, count=HALF):
        def product(j):
            return pacer.dot(t.o[j * h_rows + first // 2:j * h_rows + (first + count) // 2, :],
                             wo_s[j * w_rows:(j + 1) * w_rows, g * CHUNK:(g + 1) * CHUNK])

        for b, attn in enumerate(_block_matmul(product)):
            span = (slice(b // 2 * HALF + first, b // 2 * HALF + first + count),
                    slice(b % 2 * hd + g * CHUNK, b % 2 * hd + (g + 1) * CHUNK))
            gate = vec_s[:, GATE_A * d + span[1].start:GATE_A * d + span[1].stop]
            x1 = t.x[span].astype(F32) + _rows(gate, count) * attn
            t.x1[span] = x1
            t.x1_all[span] = x1

    def finish(t, g, after=None):
        x1 = t.x1[16 * g:16 * g + 16, :]
        xc, rstd = _centered(x1, after)
        out = x1 + (xc * rstd * _rows(vec(OUT_SCALE), 16) + _rows(vec(OUT_SHIFT), 16))
        t.out[16 * g:16 * g + 16, :] = out.astype(BF16)
        score = jnp.sum(xc * _rows(vec(SCORE), 16), axis=-1, keepdims=True) * rstd
        lane = lax.broadcasted_iota(I32, (8, 128), 1)
        packed = t.score[...]
        for s in range(2):
            packed = jnp.where(lane == 2 * g + s, score[8 * s:8 * s + 8], packed)
        t.score[...] = packed
        return pacer.token([packed, out[:, -128:]])

    def finishing(t, groups, windows):
        for g, window in zip(groups, windows, strict=True):
            pacer.plan(functools.partial(finish, t, g), window)

    def attend(t, previous, after_first=lambda: None):
        ready = queries(t, 0)
        after_first()
        for m in range(n_chunks - 1):
            ahead = queries(t, m + 1)
            residual(previous, m)
            read_out(t, m, ready)
            ready = ahead
        read_out(t, n_chunks - 1, ready)
        residual(previous, n_chunks - 1)

    def start_up():
        early = (tile(0, 0), tile(0, 1))
        cf = c_v[...].astype(F32)
        act_s[...] = _pack(jnp.broadcast_to(cf * _sigmoid(cf), (16, d)))
        wphi_cp.wait()
        feature_blocks()

        def weight_terms(j):
            for cp in weight_copies(j):
                cp.wait()
            for g in range(n_chunks):
                projection_terms(KEY, j, g)
                projection_terms(VALUE, j, g)

        def activation_terms(j):
            for cp in mod_a_copies(j):
                cp.wait()
            parts = [slice(part * hd + j * CHUNK, part * hd + (j + 1) * CHUNK) for part in range(4)]
            m = _dot(_unpack(act_s[...]),
                     jnp.concatenate([wmod_v[:, part] for part in parts], axis=1))[0:8]
            vectors = [m[:, :128], m[:, 128:256], 1.0 + m[:, 256:384], 1.0 + m[:, 384:]]
            for part, v in zip(parts, vectors):
                vec_s[:, part] = v
            shifts, scales = vectors[:2], vectors[2:]
            for t in early:
                blocks = (t.x1[r:r + HALF, part] * _rows(scale, HALF) + _rows(shift, HALF)
                          for part, scale, shift in zip(parts, scales, shifts) for r in (0, HALF))
                for i, term in enumerate(_rhs_terms(*blocks)):
                    r0 = i * w_rows + j * CHUNK // 2
                    t.h_all[r0:r0 + CHUNK // 2, :] = _pack_transposed(term)

        x_first_cp.wait()
        for t in early:
            for r0 in range(0, TILE, 16):
                t.x1[r0:r0 + 16, :] = normed_rows(t, r0)
        weight_terms(0)
        activation_terms(0)
        for j in range(n_chunks):
            for i in range(TERMS):
                if i == 2 and j + 1 < n_chunks:
                    weight_terms(j + 1)
                if i == 5 and j + 1 < n_chunks:
                    activation_terms(j + 1)
                if i == 0 and j + 1 == n_chunks:
                    x_next_cp.wait()
                    normalize(tile(1, 0))
                r0 = i * w_rows + j * CHUNK // 2
                h = jnp.concatenate([t.h_all[r0:r0 + CHUNK // 2, :] for t in early], axis=1)
                for col, w_s in ((KEY, wk_s), (VALUE, wv_s)):
                    w = w_s[i * w_rows:(i + 1) * w_rows, j * CHUNK:(j + 1) * CHUNK]
                    product = _dot(_unpack(w), _unpack(h))
                    acc = early_product(col, i)
                    acc[...] = product + acc[...] if j else product
        for cp in (wq_cp, wo_cp, wr_cp):
            cp.start()

    def summarize_pair(i, copies):
        ready = []

        def job(n, end, after):
            p, pk, v = early_features(n // 4, n % 4)
            if after is not None:
                pk = pk + _rows(jnp.concatenate([pltpu.bitcast(after, F32)] * 2, axis=1), PAIR)
            phi = key_features(p, pk)
            ready.append((end, [phi], [(p, v)]))
            return pacer.token([pltpu.bitcast(phi[-16:], I32)])

        def drain():
            while ready and ready[0][0] <= pacer.now:
                accumulate_kv(*ready.pop(0)[1:])

        for n, window in enumerate(EARLY_WINDOWS):
            pacer.plan(functools.partial(
                job, (i - 1) * len(EARLY_WINDOWS) + n, pacer.now + window[1]), window)
        copies[0].start()
        normalize(tile(i, 1))
        owed = summarize(tile(i, 0), [], drain)
        copies[1].start()
        normalize(tile(i + 1, 0))
        summarize(tile(i, 1), owed, drain, flush=True)
        assert not ready

    def summarize_last_pair():
        for cp in (wq_cp, wo_cp, wr_cp, mod_b_cp):
            cp.wait()
        normalize(tile(last, 1))
        for p, window in enumerate(OUTPUT_WINDOWS):
            for c in range(n_chunks):
                pacer.plan(functools.partial(output_terms, p, c), window)
        for j in range(n_chunks):
            for g in range(n_chunks):
                pacer.fillers += [functools.partial(projection_terms, QUERY, j, g),
                                  lambda: None, lambda: None]
        summarize(tile(last, 1), summarize(tile(last, 0), []), flush=True)

    def attend_first_pair():
        row = lax.broadcasted_iota(I32, (PAIR, 128), 0)
        lane = lax.broadcasted_iota(I32, (PAIR, 128), 1)
        for p in range(PAIRS):
            kv = jnp.where(row % 2 == lane % 2, kv_s[p * PAIR:(p + 1) * PAIR, :], 0.0)
            kvm_s[p * HEAD_DIM:(p + 1) * HEAD_DIM, :] = _pack(kv)
            z = jnp.sum(z_s[p * 128:(p + 1) * 128, :], axis=1, keepdims=True)
            z_s[p * 128:(p + 1) * 128, :] = jnp.broadcast_to(z, (128, 128))
        for i in (GATE_A, SHIFT_B, SCALE_B, GATE_B):
            pacer.fillers += modulation_rounds(i)
        first = tile(0, 0)
        fetch(first)
        fetch(tile(0, 1))
        ready = queries(first, 0)
        for m in range(n_chunks - 1):
            ahead = queries(first, m + 1)
            read_out(first, m, ready)
            ready = ahead
        fetch(tile(1, 0))
        attend(tile(0, 1), first, lambda: read_out(first, n_chunks - 1, ready))
        derived_vectors()

    def attend_pairs():
        def body(i, carry):
            pacer.reset()
            tiles = [tile(i - 1, 0), tile(i - 1, 1), tile(i, 0), tile(i, 1),
                     tile(jnp.minimum(i + 1, last), 0)]
            for k in range(2):
                fetch(tiles[k + 3])
                finishing(tiles[k], range(TILE // 16), FINISH_WINDOWS)
                attend(tiles[k + 2], tiles[k + 1])
            out_copy(i - 1).start()
            return carry

        lax.fori_loop(1, last + 1, body, 0)

    def finish_last_pair():
        final = tile(last, 1)
        groups = [[(r + k * HALF // 2 + side * HALF) // 16 for side in range(2)
                   for r in range(0, HALF // 2, 16)] for k in range(2)]
        finishing(tile(last, 0), range(TILE // 16), LAST_WINDOWS)
        for g in range(n_chunks):
            residual(final, g, 0, HALF // 2)
        finishing(final, groups[0], TAIL_WINDOWS)
        for g in range(n_chunks):
            residual(final, g, HALF // 2, HALF // 2)
        for g in groups[1]:
            finish(final, g)
        out_copy(last).start()

    def route():
        scores = score_s[...]
        row = lax.broadcasted_iota(I32, scores.shape, 0)
        lane = lax.broadcasted_iota(I32, scores.shape, 1)
        index = jnp.where(
            lane < TILE // 8, (row // 8) * TILE + lane * 8 + row % 8, seq).astype(F32)

        def everywhere(op, v):
            return op(op(v, axis=0, keepdims=True), axis=1, keepdims=True)

        def arg_top(valid):
            best = everywhere(jnp.max, jnp.where(valid, scores, -jnp.inf))
            return everywhere(jnp.min, jnp.where(valid & (scores == best), index, seq - 1.0))

        first = arg_top(index < seq)
        second = arg_top((index < seq) & (index != first))
        i0, i1 = (jnp.max(v).astype(I32) for v in (first, second))

        sub = lax.broadcasted_iota(I32, (16, d), 0)
        x1 = jnp.where(sub == 0, x1_all[pl.ds(i0, 1), :], x1_all[pl.ds(i1, 1), :])
        xc, rstd = _centered(x1)
        h2 = xc * rstd * _rows(vec(SCALE_B), 16) + _rows(vec(SHIFT_B), 16)
        gate = _sigmoid(jnp.sum(h2 * _rows(vec(ROUTER), 16), axis=-1, keepdims=True))
        xs = h2.astype(BF16)
        for cp in (wg_cp, wu_cp, wd_cp):
            cp.wait()
        spans = [slice(f, f + FFN_CHUNK) for f in range(0, wd_v.shape[0], FFN_CHUNK)]
        y, hidden = 0.0, None
        for k in range(len(spans) + 1):
            if k < len(spans):
                g, u = _dot(xs, wg_v[:, spans[k]]), _dot(xs, wu_v[:, spans[k]])
            if k > 0:
                y = y + _dot(hidden, wd_v[spans[k - 1], :])
            hidden = (g * _sigmoid(g) * u).astype(BF16)
        routed = x1 + _rows(vec(GATE_B), 16) * (h2 + y * gate)

        for i in range(last + 1):
            out_copy(i).wait()

        def patch(k, i):
            base = pl.multiple_of((i // 16) * 16, 16)
            old = out_v[pl.ds(base, 16), :].astype(F32)
            out_v[pl.ds(base, 16), :] = jnp.where(
                sub == i - base, routed[k:k + 1], old).astype(BF16)
            return base, copy(out_v.at[pl.ds(base, 16)], out_hbm.at[pl.ds(base, 16)],
                              sem.at[24 + k])

        base0, patch0 = patch(0, i0)
        base1, patch1 = patch(1, i1)
        patch0.start()

        @pl.when(base1 != base0)
        def _():
            patch1.start()
            patch1.wait()

        patch0.wait()

    for cp in (c_cp, wphi_cp, x_first_cp):
        cp.start()
    for j in range(n_chunks):
        for cp in weight_copies(j) + mod_a_copies(j):
            cp.start()
    x_next_cp.start()
    x_rest_cp.start()
    kv_s[...] = jnp.zeros(kv_s.shape, F32)
    z_s[...] = jnp.zeros(z_s.shape, F32)
    score_s[...] = jnp.full(score_s.shape, -jnp.inf, F32)
    c_cp.wait()
    words = pltpu.bitcast(jnp.broadcast_to(c_v[:, :128].astype(F32), (8, 128)), I32)
    zero = jnp.minimum(lax.shift_right_logical(words, 1), 0)
    zero_s[...] = zero
    origin = jnp.max(zero)

    def own_block(k, step):
        pacer.reset()
        pl.when(origin <= k)(step)
        pacer.reset()

    start_up()
    x_rest_cp.wait()
    own_block(1, functools.partial(summarize_pair, 1, (mod_b_cp, wg_cp)))
    summarize_pair(2, (wu_cp, wd_cp))
    own_block(2, summarize_last_pair)
    attend_first_pair()
    attend_pairs()
    pacer.reset()
    finish_last_pair()
    route()


@jax.jit
def pallas_adaLN_cond__linear_kernel_hedgehog__moe_arch_mod__prompt_kernel(
    A_x: jax.Array,
    A_wqkv: jax.Array,
    A_w_phi: jax.Array,
    A_wo: jax.Array,
    B_x: jax.Array,
    B_w_r: jax.Array,
    B_w_gate: jax.Array,
    B_w_up: jax.Array,
    B_w_down: jax.Array,
    c: jax.Array,
    w_mod: jax.Array,
):
    del B_x
    batch, seq, d = A_x.shape
    assert batch == 1 and d == HEADS * HEAD_DIM and seq == 8 * TILE
    n_tiles = seq // TILE
    operands = (A_x.reshape(seq, d), A_wqkv, A_w_phi, A_wo, B_w_r, B_w_gate, B_w_up, B_w_down,
                c, w_mod)
    weight_terms = pltpu.VMEM((TERMS * d // 4, d // 2), I32)
    token_terms = pltpu.VMEM((TERMS * HALF // 2, d // 2), I32)
    scratch = [pltpu.VMEM(a.shape, a.dtype) for a in operands] + [
        weight_terms, weight_terms, weight_terms, weight_terms,
        pltpu.VMEM((d // 2, 128), I32),
        pltpu.VMEM((8, d), I32),
        pltpu.VMEM((8, 10 * d), F32),
        token_terms,
        [pltpu.VMEM((TERMS * d // 4, HALF), I32)] * 2,
        pltpu.VMEM((n_tiles * TERMS * d // 4, HALF), I32),
        [token_terms] * 2,
        [pltpu.VMEM((TILE, d), F32)] * 2,
        pltpu.VMEM((seq, d), F32),
        pltpu.VMEM((PAIRS * PAIR, 128), F32),
        pltpu.VMEM((PAIRS * HEAD_DIM, 128), I32),
        pltpu.VMEM((PAIRS * 128, 128), F32),
        pltpu.VMEM((n_tiles * 8, 128), F32),
        pltpu.VMEM((8, 128), I32),
        pltpu.VMEM((seq, d), A_x.dtype),
        pltpu.SemaphoreType.DMA((26,)),
    ]
    out = pl.pallas_call(
        _kernel,
        out_shape=jax.ShapeDtypeStruct((seq, d), A_x.dtype),
        in_specs=[pl.BlockSpec(memory_space=pl.ANY)] * len(operands),
        out_specs=pl.BlockSpec(memory_space=pl.ANY),
        scratch_shapes=scratch,
        compiler_params=pltpu.CompilerParams(
            vmem_limit_bytes=110 * 2**20,
            flags={"XLA_TPU_EVENLY_DISTRIBUTE_CRITICAL_NODES": True}),
        name="adaln_hedgehog_mod",
    )(*operands)
    return out.reshape(batch, seq, d)
```

```python
import collections
import functools
import math

import jax
import jax.numpy as jnp
from jax import lax
import jax.experimental.pallas as pl
import jax.experimental.pallas.tpu as pltpu

F32 = jnp.float32
BF16 = jnp.bfloat16
I32 = jnp.int32

HEADS = 32
HEAD_DIM = 32
PAIRS = HEADS // 2
PAIR = 2 * HEAD_DIM
TERMS = 7
TILE = 256
HALF = TILE // 2
CHUNK = 128
FFN_CHUNK = 512
LN_EPS = 1e-5
DEN_EPS = 1e-6
LOG2E = math.log2(math.e)

EARLY_WINDOWS = tuple((6 * n - 1, 6 * n + 16) for n in range(16))
OUTPUT_WINDOWS = tuple((55 + 6 * p, 67 + 6 * p) for p in range(8))
FINISH_WINDOWS = tuple((3 * g - 1, min(3 * g + 11, 55)) for g in range(16))
LAST_WINDOWS = tuple((7 * (g // 5), 7 * (g // 5) + 9) for g in range(16))
TAIL_WINDOWS = tuple((7 * (n // 3) - 1, 7 * (n // 3) + 9) for n in range(8))

QUERY, KEY, VALUE = range(3)
SHIFT_A, SCALE_A, GATE_A, SHIFT_B, SCALE_B, GATE_B, ROUTER, OUT_SCALE, OUT_SHIFT, SCORE = range(10)

Tile = collections.namedtuple("Tile", "x h h_all o x1 x1_all out score")


def _dot(a, b):
    return jnp.dot(a, b, preferred_element_type=F32)


def _dot_nt(a, b):
    return lax.dot_general(a, b, (((1,), (1,)), ((), ())), preferred_element_type=F32)


def _pack(v):
    return pltpu.bitcast(v.astype(BF16), I32)


def _pack_transposed(v):
    return pltpu.bitcast(v.astype(BF16).T, I32)


def _unpack(words):
    return pltpu.bitcast(words, BF16)


def _recip(v):
    r = pltpu.reciprocal(v, approx=True)
    return r * (2.0 - v * r)


def _sigmoid(v):
    return 1.0 / (1.0 + jnp.exp(-v))


def _rows(v, n):
    return jnp.concatenate([v] * (n // 8), axis=0)


def _centered(x, after=None):
    inv_d = 1.0 / x.shape[-1]
    if after is not None:
        head = x[:, :128] + _rows(pltpu.bitcast(after, F32), x.shape[0])
        x = jnp.concatenate([head, x[:, 128:]], axis=1)
    xc = x - jnp.sum(x, axis=-1, keepdims=True) * inv_d
    var = jnp.sum(xc * xc, axis=-1, keepdims=True) * inv_d
    return xc, lax.rsqrt(var + LN_EPS)


def _lhs_terms(a11, a12, a21, a22):
    return [a11 + a22, a21 + a22, a11, a22, a11 + a12, a21 - a11, a12 - a22]


def _rhs_terms(b11, b12, b21, b22):
    return [b11 + b22, b11, b12 - b22, b21 - b11, b22, b11 + b12, b21 + b22]


def _block_matmul(product):
    m5, m3 = product(4), product(2)
    c12 = m5 + m3
    m1 = product(0)
    c11, c22 = m1 - m5, m3 + m1
    c11 = c11 + product(6)
    m4 = product(3)
    c11 = c11 + m4
    m2 = product(1)
    c21, c22 = m4 + m2, c22 - m2
    c22 = c22 + product(5)
    return c11, c12, c21, c22


def _head_reduce(op, tiles):
    while len(tiles) > 1:
        tiles = [op(tiles[i], tiles[i + 1]) for i in range(0, len(tiles), 2)]
    m = tiles[0]
    m = op(m, pltpu.roll(m, 4, 0))
    return op(m, pltpu.roll(m, 2, 0))


def _feature_map(p):
    tiles = [p[8 * j:8 * j + 8] for j in range(PAIR // 8)]
    hi = _head_reduce(jnp.maximum, tiles)
    lo = _head_reduce(jnp.minimum, tiles)
    e_pos = [jnp.exp2(t - hi) for t in tiles]
    e_neg = [jnp.exp2(lo - t) for t in tiles]
    r_pos = _recip(_head_reduce(jnp.add, e_pos))
    r_neg = _recip(_head_reduce(jnp.add, e_neg))
    return [e * r_pos for e in e_pos] + [e * r_neg for e in e_neg]


class _Pacer:
    def __init__(self, zero_ref):
        self.zero_ref = zero_ref
        self.now = 0
        self.last = None
        self.jobs, self.gates, self.fillers = {}, {}, []

    def reset(self):
        assert not self.jobs and not self.fillers
        self.last, self.gates = None, {}

    def token(self, values):
        tiles = [pltpu.bitcast(v[r:r + 8, c:c + 128], I32) for v in values
                 for r in range(0, v.shape[0], 8) for c in range(0, v.shape[1], 128)]
        while len(tiles) > 1:
            tiles = [tiles[j] | tiles[j + 1] if j + 1 < len(tiles) else tiles[j]
                     for j in range(0, len(tiles), 2)]
        return tiles[0] & self.zero_ref[...]

    def plan(self, job, window):
        start, end = (self.now + w for w in window)
        if start < self.now:
            self._run(job, end)
        else:
            self.jobs.setdefault(start, []).append((job, end))

    def _run(self, job, end):
        self.gates.setdefault(end, []).append(job(self.last))

    def dot(self, lhs, rhs):
        for zero in self.gates.pop(self.now, []):
            top = jnp.concatenate([lhs[:8, :128] | zero, lhs[:8, 128:]], axis=1)
            lhs = jnp.concatenate([top, lhs[8:]], axis=0)
        out = _dot(_unpack(lhs), _unpack(rhs))
        self.last = self.token([out[-8:]])
        for job, end in self.jobs.pop(self.now, []):
            self._run(job, end)
        self.now += 1
        if self.fillers:
            self.fillers.pop(0)()
        return out


def _kernel(x_hbm, wqkv_hbm, wphi_hbm, wo_hbm, wr_hbm, wg_hbm, wu_hbm, wd_hbm, c_hbm, wmod_hbm,
            out_hbm,
            x_v, wqkv_v, wphi_v, wo_v, wr_v, wg_v, wu_v, wd_v, c_v, wmod_v,
            wq_s, wk_s, wv_s, wo_s, phi_s, act_s, vec_s, norm_s, h_s, h_all, o_s, x1_s, x1_all,
            kv_s, kvm_s, z_s, score_s, zero_s, out_v,
            sem):
    seq, d = x_v.shape
    hd = d // 2
    last = seq // (2 * TILE) - 1
    n_chunks = hd // CHUNK
    h_rows = HALF // 2
    w_rows = hd // 2
    pacer = _Pacer(zero_s)

    copy = pltpu.make_async_copy

    def view(ref, index, size):
        start = index * size
        return ref.at[pl.ds(start if isinstance(start, int) else pl.multiple_of(start, size), size)]

    def x_copy(first, count, s):
        return copy(x_hbm.at[pl.ds(first, count)], x_v.at[pl.ds(first, count)], s)

    c_cp = copy(c_hbm, c_v, sem.at[0])
    wphi_cp = copy(wphi_hbm, wphi_v, sem.at[1])
    wr_cp = copy(wr_hbm, wr_v, sem.at[2])
    mod_b_cp = copy(wmod_hbm.at[:, pl.ds(2 * d, 4 * d)], wmod_v.at[:, pl.ds(2 * d, 4 * d)],
                    sem.at[3])
    wq_cp = copy(wqkv_hbm.at[:, pl.ds(0, d)], wqkv_v.at[:, pl.ds(0, d)], sem.at[4])
    wo_cp = copy(wo_hbm, wo_v, sem.at[5])
    wg_cp = copy(wg_hbm, wg_v, sem.at[6])
    wu_cp = copy(wu_hbm, wu_v, sem.at[7])
    wd_cp = copy(wd_hbm, wd_v, sem.at[8])
    x_first_cp = x_copy(0, 2 * TILE, sem.at[9])
    x_next_cp = x_copy(2 * TILE, TILE, sem.at[10])
    x_rest_cp = x_copy(3 * TILE, seq - 3 * TILE, sem.at[11])

    def weight_copies(j):
        spans = [(pl.ds(half * hd + j * CHUNK, CHUNK), pl.ds(d, 2 * d)) for half in range(2)]
        return [copy(wqkv_hbm.at[span], wqkv_v.at[span], sem.at[12 + j]) for span in spans]

    def mod_a_copies(j):
        spans = [pl.ds(part * hd + j * CHUNK, CHUNK) for part in range(4)]
        return [copy(wmod_hbm.at[:, span], wmod_v.at[:, span], sem.at[16 + j]) for span in spans]

    def out_copy(i):
        return copy(view(out_v, i, 2 * TILE), view(out_hbm, i, 2 * TILE), sem.at[20 + i])

    def tile(i, parity):
        t = 2 * i + parity
        return Tile(x=view(x_v, t, TILE), h=h_s[parity], h_all=view(h_all, t, TERMS * w_rows),
                    o=o_s[parity], x1=x1_s[parity], x1_all=view(x1_all, t, TILE),
                    out=view(out_v, t, TILE), score=view(score_s, t, 8))

    def feature_blocks():
        row = lax.broadcasted_iota(I32, (128, 128), 0)
        lane = lax.broadcasted_iota(I32, (128, 128), 1)
        same_head = 2 * (row // PAIR) + row % 2 == lane // HEAD_DIM
        row_f = lax.broadcasted_iota(I32, (128, HEAD_DIM), 0)
        lane_f = lax.broadcasted_iota(I32, (128, HEAD_DIM), 1)
        pick = jnp.where(row_f % PAIR // 2 == lane_f, 1.0, 0.0).astype(BF16)
        for g in range(d // 128):
            wphi = wphi_v[4 * g:4 * g + 4].reshape(128, HEAD_DIM)
            phi_s[g * 64:(g + 1) * 64, :] = _pack(jnp.where(same_head, _dot_nt(pick, wphi), 0.0))

    def projection_terms(col, j, g):
        def group(g):
            span = slice(col * d + g * CHUNK, col * d + (g + 1) * CHUNK)
            w = jnp.concatenate(
                [wqkv_v[r + j * CHUNK:r + (j + 1) * CHUNK, span] for r in (0, hd)], axis=0)
            if col == VALUE:
                return w.astype(F32).T
            return _dot_nt(_unpack(phi_s[g * 64:(g + 1) * 64, :]), w) * LOG2E

        top, bottom = group(g), group(g + n_chunks)
        terms = _lhs_terms(top[:, :CHUNK], top[:, CHUNK:], bottom[:, :CHUNK], bottom[:, CHUNK:])
        for i, term in enumerate(terms):
            r0 = i * w_rows + g * CHUNK // 2
            (wq_s, wk_s, wv_s)[col][r0:r0 + CHUNK // 2, j * CHUNK:(j + 1) * CHUNK] = _pack(term)

    def output_terms(p, c, after):
        def block(r0, c0):
            words = pltpu.bitcast(wo_v[r0:r0 + PAIR, c0:c0 + CHUNK], I32) | _rows(after, HEAD_DIM)
            return _unpack(words).astype(F32)

        blocks = (block(r + p * PAIR, k + c * CHUNK) for r in (0, hd) for k in (0, hd))
        terms = _rhs_terms(*blocks)
        for i, term in enumerate(terms):
            r0 = i * w_rows + p * HEAD_DIM
            wo_s[r0:r0 + HEAD_DIM, c * CHUNK:(c + 1) * CHUNK] = _pack(term)
        return pacer.token([term[-8:] for term in terms])

    def vec(i):
        return vec_s[:, i * d:(i + 1) * d]

    def modulation_rounds(i):
        partial = {}

        def one(c0, half):
            span = slice(half * hd, (half + 1) * hd)
            m = _dot(_unpack(act_s[:, span]), wmod_v[span, c0:c0 + 128])[0:8]
            if half == 0:
                partial[c0] = 1.0 + m if i == SCALE_B else m
            else:
                vec_s[:, c0:c0 + 128] = partial[c0] + m

        return [functools.partial(one, c0, half)
                for c0 in range(i * d, (i + 1) * d, 128) for half in range(2)]

    def derived_vectors():
        router = jnp.broadcast_to(wr_v[...].astype(F32).reshape(1, d), (8, d))
        for i, v in ((ROUTER, router), (OUT_SCALE, vec(GATE_B) * vec(SCALE_B)),
                     (OUT_SHIFT, vec(GATE_B) * vec(SHIFT_B)), (SCORE, router * vec(SCALE_B))):
            vec_s[:, i * d:(i + 1) * d] = v

    def normed_rows(t, r0):
        xc, rstd = _centered(t.x[r0:r0 + 16, :].astype(F32))
        return xc * rstd

    def normalize(t):
        for r0 in range(0, HALF, 16):
            ha, hb = (normed_rows(t, r + r0) * _rows(vec(SCALE_A), 16) + _rows(vec(SHIFT_A), 16)
                      for r in (0, HALF))
            for j, term in enumerate(_rhs_terms(ha[:, :hd], hb[:, :hd], ha[:, hd:], hb[:, hd:])):
                norm_s[j * h_rows + r0 // 2:j * h_rows + r0 // 2 + 8, :] = _pack(term)
        for j in range(TERMS):
            term = _pack_transposed(_unpack(norm_s[j * h_rows:(j + 1) * h_rows, :]))
            t.h[j * w_rows:(j + 1) * w_rows, :] = term
            t.h_all[j * w_rows:(j + 1) * w_rows, :] = term

    def fetch(t):
        for j in range(TERMS):
            t.h[j * w_rows:(j + 1) * w_rows, :] = t.h_all[j * w_rows:(j + 1) * w_rows, :]

    def project(w_s, t, m):
        def product(j):
            r0 = j * w_rows + m * CHUNK // 2
            return pacer.dot(w_s[r0:r0 + CHUNK // 2, :], t.h[j * w_rows:(j + 1) * w_rows, :])

        c11, c12, c21, c22 = _block_matmul(product)
        halves = (jnp.concatenate([c11, c12], axis=1), jnp.concatenate([c21, c22], axis=1))
        return [(side * PAIRS // 2 + m * CHUNK // PAIR + j, block[j * PAIR:(j + 1) * PAIR])
                for side, block in enumerate(halves) for j in range(CHUNK // PAIR)]

    def key_features(p, pk):
        phi = jnp.concatenate(_feature_map(pk), axis=0)
        z_s[p * 128:(p + 1) * 128, :] += phi[:, :HALF] + phi[:, HALF:]
        return phi

    def accumulate_kv(phi, v):
        for phi_p, (p, v_p) in zip(phi, v, strict=True):
            kv_s[p * PAIR:(p + 1) * PAIR, :] += _dot_nt(v_p.astype(BF16), phi_p.astype(BF16))

    def summarize(t, owed, between=lambda: None, flush=False):
        for m in range(n_chunks):
            pk = project(wk_s, t, m)
            if not (flush and m + 1 == n_chunks):
                while owed:
                    accumulate_kv(*owed.pop(0))
            between()
            owed.append(([key_features(*pair) for pair in pk], project(wv_s, t, m)))
            between()
        while flush and owed:
            accumulate_kv(*owed.pop(0))
        return owed

    def early_product(col, i):
        n = (col - KEY) * TERMS + i
        return x1_all.at[pl.ds(n // 4 * hd, hd), pl.ds(n % 4 * TILE, TILE)]

    def early_features(q, b):
        def block(col):
            return _block_matmul(lambda i: early_product(col, i)[q * PAIR:(q + 1) * PAIR, :])[b]

        return b // 2 * PAIRS // 2 + q, block(KEY), block(VALUE)

    def query_features(p, pq):
        phi = _feature_map(pq)
        z = [z_s[p * 128 + 8 * j:p * 128 + 8 * j + 8, :] for j in range(len(phi))]
        den = _head_reduce(
            jnp.add, [f * jnp.concatenate([zj, zj], axis=1) for f, zj in zip(phi, z)])
        inv = _recip(den + DEN_EPS)
        even = lax.broadcasted_iota(I32, inv.shape, 0) % 2 == 0
        other = pltpu.roll(inv, 1, 0)
        per_head = [jnp.where(even, inv, other), jnp.where(even, other, inv)]
        return (p, jnp.concatenate(phi, axis=0).astype(BF16),
                jnp.concatenate([_rows(v, HEAD_DIM) for v in per_head], axis=0))

    def queries(t, m):
        return [query_features(*pair) for pair in project(wq_s, t, m)]

    def read_out(t, m, features):
        o_t = [_dot(_unpack(kvm_s[p * HEAD_DIM:(p + 1) * HEAD_DIM, :]), phi) * inv
               for p, phi, inv in features]
        top = jnp.concatenate(o_t[:len(o_t) // 2], axis=0)
        bottom = jnp.concatenate(o_t[len(o_t) // 2:], axis=0)
        terms = _lhs_terms(top[:, :HALF], bottom[:, :HALF], top[:, HALF:], bottom[:, HALF:])
        for j, term in enumerate(terms):
            t.o[j * h_rows:(j + 1) * h_rows, m * CHUNK:(m + 1) * CHUNK] = _pack_transposed(term)

    def residual(t, g, first=0, count=HALF):
        def product(j):
            return pacer.dot(t.o[j * h_rows + first // 2:j * h_rows + (first + count) // 2, :],
                             wo_s[j * w_rows:(j + 1) * w_rows, g * CHUNK:(g + 1) * CHUNK])

        for b, attn in enumerate(_block_matmul(product)):
            span = (slice(b // 2 * HALF + first, b // 2 * HALF + first + count),
                    slice(b % 2 * hd + g * CHUNK, b % 2 * hd + (g + 1) * CHUNK))
            gate = vec_s[:, GATE_A * d + span[1].start:GATE_A * d + span[1].stop]
            x1 = t.x[span].astype(F32) + _rows(gate, count) * attn
            t.x1[span] = x1
            t.x1_all[span] = x1

    def finish(t, g, after=None):
        x1 = t.x1[16 * g:16 * g + 16, :]
        xc, rstd = _centered(x1, after)
        out = x1 + (xc * rstd * _rows(vec(OUT_SCALE), 16) + _rows(vec(OUT_SHIFT), 16))
        t.out[16 * g:16 * g + 16, :] = out.astype(BF16)
        score = jnp.sum(xc * _rows(vec(SCORE), 16), axis=-1, keepdims=True) * rstd
        lane = lax.broadcasted_iota(I32, (8, 128), 1)
        packed = t.score[...]
        for s in range(2):
            packed = jnp.where(lane == 2 * g + s, score[8 * s:8 * s + 8], packed)
        t.score[...] = packed
        return pacer.token([packed, out[:, -128:]])

    def finishing(t, groups, windows):
        for g, window in zip(groups, windows, strict=True):
            pacer.plan(functools.partial(finish, t, g), window)

    def attend(t, previous, after_first=lambda: None):
        ready = queries(t, 0)
        after_first()
        for m in range(n_chunks - 1):
            ahead = queries(t, m + 1)
            residual(previous, m)
            read_out(t, m, ready)
            ready = ahead
        read_out(t, n_chunks - 1, ready)
        residual(previous, n_chunks - 1)

    def start_up():
        early = (tile(0, 0), tile(0, 1))
        cf = c_v[...].astype(F32)
        act_s[...] = _pack(jnp.broadcast_to(cf * _sigmoid(cf), (16, d)))
        wphi_cp.wait()
        feature_blocks()

        def weight_terms(j):
            for cp in weight_copies(j):
                cp.wait()
            for g in range(n_chunks):
                projection_terms(KEY, j, g)
                projection_terms(VALUE, j, g)

        def activation_terms(j):
            for cp in mod_a_copies(j):
                cp.wait()
            parts = [slice(part * hd + j * CHUNK, part * hd + (j + 1) * CHUNK) for part in range(4)]
            m = _dot(_unpack(act_s[...]),
                     jnp.concatenate([wmod_v[:, part] for part in parts], axis=1))[0:8]
            vectors = [m[:, :128], m[:, 128:256], 1.0 + m[:, 256:384], 1.0 + m[:, 384:]]
            for part, v in zip(parts, vectors):
                vec_s[:, part] = v
            shifts, scales = vectors[:2], vectors[2:]
            for t in early:
                blocks = (t.x1[r:r + HALF, part] * _rows(scale, HALF) + _rows(shift, HALF)
                          for part, scale, shift in zip(parts, scales, shifts) for r in (0, HALF))
                for i, term in enumerate(_rhs_terms(*blocks)):
                    r0 = i * w_rows + j * CHUNK // 2
                    t.h_all[r0:r0 + CHUNK // 2, :] = _pack_transposed(term)

        x_first_cp.wait()
        for t in early:
            for r0 in range(0, TILE, 16):
                t.x1[r0:r0 + 16, :] = normed_rows(t, r0)
        weight_terms(0)
        activation_terms(0)
        for j in range(n_chunks):
            for i in range(TERMS):
                if i == 2 and j + 1 < n_chunks:
                    weight_terms(j + 1)
                if i == 5 and j + 1 < n_chunks:
                    activation_terms(j + 1)
                if i == 0 and j + 1 == n_chunks:
                    x_next_cp.wait()
                    normalize(tile(1, 0))
                r0 = i * w_rows + j * CHUNK // 2
                h = jnp.concatenate([t.h_all[r0:r0 + CHUNK // 2, :] for t in early], axis=1)
                for col, w_s in ((KEY, wk_s), (VALUE, wv_s)):
                    w = w_s[i * w_rows:(i + 1) * w_rows, j * CHUNK:(j + 1) * CHUNK]
                    product = _dot(_unpack(w), _unpack(h))
                    acc = early_product(col, i)
                    acc[...] = product + acc[...] if j else product
        for cp in (wq_cp, wo_cp, wr_cp):
            cp.start()

    def summarize_pair(i, copies):
        ready = []

        def job(n, end, after):
            p, pk, v = early_features(n // 4, n % 4)
            if after is not None:
                pk = pk + _rows(jnp.concatenate([pltpu.bitcast(after, F32)] * 2, axis=1), PAIR)
            phi = key_features(p, pk)
            ready.append((end, [phi], [(p, v)]))
            return pacer.token([phi[PAIR - 8:PAIR], phi[-8:]])

        def drain():
            while ready and ready[0][0] <= pacer.now:
                accumulate_kv(*ready.pop(0)[1:])

        for n, window in enumerate(EARLY_WINDOWS):
            pacer.plan(functools.partial(
                job, (i - 1) * len(EARLY_WINDOWS) + n, pacer.now + window[1]), window)
        copies[0].start()
        normalize(tile(i, 1))
        owed = summarize(tile(i, 0), [], drain)
        copies[1].start()
        normalize(tile(i + 1, 0))
        summarize(tile(i, 1), owed, drain, flush=True)
        assert not ready

    def summarize_last_pair():
        for cp in (wq_cp, wo_cp, wr_cp, mod_b_cp):
            cp.wait()
        normalize(tile(last, 1))
        for p, window in enumerate(OUTPUT_WINDOWS):
            for c in range(n_chunks):
                pacer.plan(functools.partial(output_terms, p, c), window)
        for j in range(n_chunks):
            for g in range(n_chunks):
                pacer.fillers += [functools.partial(projection_terms, QUERY, j, g),
                                  lambda: None, lambda: None]
        summarize(tile(last, 1), summarize(tile(last, 0), []), flush=True)

    def attend_first_pair():
        row = lax.broadcasted_iota(I32, (PAIR, 128), 0)
        lane = lax.broadcasted_iota(I32, (PAIR, 128), 1)
        for p in range(PAIRS):
            kv = jnp.where(row // HEAD_DIM == lane % 2, kv_s[p * PAIR:(p + 1) * PAIR, :], 0.0)
            kvm_s[p * HEAD_DIM:(p + 1) * HEAD_DIM, :] = _pack(kv)
            z = jnp.sum(z_s[p * 128:(p + 1) * 128, :], axis=1, keepdims=True)
            z_s[p * 128:(p + 1) * 128, :] = jnp.broadcast_to(z, (128, 128))
        for i in (GATE_A, SHIFT_B, SCALE_B, GATE_B):
            pacer.fillers += modulation_rounds(i)
        first = tile(0, 0)
        fetch(first)
        fetch(tile(0, 1))
        ready = queries(first, 0)
        for m in range(n_chunks - 1):
            ahead = queries(first, m + 1)
            read_out(first, m, ready)
            ready = ahead
        fetch(tile(1, 0))
        attend(tile(0, 1), first, lambda: read_out(first, n_chunks - 1, ready))
        derived_vectors()

    def attend_pairs():
        def body(i, carry):
            pacer.reset()
            tiles = [tile(i - 1, 0), tile(i - 1, 1), tile(i, 0), tile(i, 1),
                     tile(jnp.minimum(i + 1, last), 0)]
            for k in range(2):
                fetch(tiles[k + 3])
                finishing(tiles[k], range(TILE // 16), FINISH_WINDOWS)
                attend(tiles[k + 2], tiles[k + 1])
            out_copy(i - 1).start()
            return carry

        lax.fori_loop(1, last + 1, body, 0)

    def finish_last_pair():
        final = tile(last, 1)
        groups = [[(r + k * HALF // 2 + side * HALF) // 16 for side in range(2)
                   for r in range(0, HALF // 2, 16)] for k in range(2)]
        finishing(tile(last, 0), range(TILE // 16), LAST_WINDOWS)
        for g in range(n_chunks):
            residual(final, g, 0, HALF // 2)
        finishing(final, groups[0], TAIL_WINDOWS)
        for g in range(n_chunks):
            residual(final, g, HALF // 2, HALF // 2)
        for g in groups[1]:
            finish(final, g)
        out_copy(last).start()

    def route():
        scores = score_s[...]
        row = lax.broadcasted_iota(I32, scores.shape, 0)
        lane = lax.broadcasted_iota(I32, scores.shape, 1)
        index = jnp.where(
            lane < TILE // 8, (row // 8) * TILE + lane * 8 + row % 8, seq).astype(F32)

        def everywhere(op, v):
            return op(op(v, axis=0, keepdims=True), axis=1, keepdims=True)

        def arg_top(valid):
            best = everywhere(jnp.max, jnp.where(valid, scores, -jnp.inf))
            return everywhere(jnp.min, jnp.where(valid & (scores == best), index, seq - 1.0))

        first = arg_top(index < seq)
        second = arg_top((index < seq) & (index != first))
        i0, i1 = (jnp.max(v).astype(I32) for v in (first, second))

        sub = lax.broadcasted_iota(I32, (16, d), 0)
        x1 = jnp.where(sub == 0, x1_all[pl.ds(i0, 1), :], x1_all[pl.ds(i1, 1), :])
        xc, rstd = _centered(x1)
        h2 = xc * rstd * _rows(vec(SCALE_B), 16) + _rows(vec(SHIFT_B), 16)
        gate = _sigmoid(jnp.sum(h2 * _rows(vec(ROUTER), 16), axis=-1, keepdims=True))
        xs = h2.astype(BF16)
        for cp in (wg_cp, wu_cp, wd_cp):
            cp.wait()
        spans = [slice(f, f + FFN_CHUNK) for f in range(0, wd_v.shape[0], FFN_CHUNK)]
        y, hidden = 0.0, None
        for k in range(len(spans) + 1):
            if k < len(spans):
                g, u = _dot(xs, wg_v[:, spans[k]]), _dot(xs, wu_v[:, spans[k]])
            if k > 0:
                y = y + _dot(hidden, wd_v[spans[k - 1], :])
            hidden = (g * _sigmoid(g) * u).astype(BF16)
        routed = x1 + _rows(vec(GATE_B), 16) * (h2 + y * gate)

        for i in range(last + 1):
            out_copy(i).wait()

        def patch(k, i):
            base = pl.multiple_of((i // 16) * 16, 16)
            old = out_v[pl.ds(base, 16), :].astype(F32)
            out_v[pl.ds(base, 16), :] = jnp.where(
                sub == i - base, routed[k:k + 1], old).astype(BF16)
            return base, copy(out_v.at[pl.ds(base, 16)], out_hbm.at[pl.ds(base, 16)],
                              sem.at[24 + k])

        base0, patch0 = patch(0, i0)
        base1, patch1 = patch(1, i1)
        patch0.start()

        @pl.when(base1 != base0)
        def _():
            patch1.start()
            patch1.wait()

        patch0.wait()

    for cp in (c_cp, wphi_cp, x_first_cp):
        cp.start()
    for j in range(n_chunks):
        for cp in weight_copies(j) + mod_a_copies(j):
            cp.start()
    x_next_cp.start()
    x_rest_cp.start()
    kv_s[...] = jnp.zeros(kv_s.shape, F32)
    z_s[...] = jnp.zeros(z_s.shape, F32)
    score_s[...] = jnp.full(score_s.shape, -jnp.inf, F32)
    c_cp.wait()
    words = pltpu.bitcast(jnp.broadcast_to(c_v[:, :128].astype(F32), (8, 128)), I32)
    zero = jnp.minimum(lax.shift_right_logical(words, 1), 0)
    zero_s[...] = zero
    origin = jnp.max(zero)

    def own_block(k, step):
        pacer.reset()
        pl.when(origin <= k)(step)
        pacer.reset()

    start_up()
    x_rest_cp.wait()
    own_block(1, functools.partial(summarize_pair, 1, (mod_b_cp, wg_cp)))
    summarize_pair(2, (wu_cp, wd_cp))
    own_block(2, summarize_last_pair)
    attend_first_pair()
    attend_pairs()
    pacer.reset()
    finish_last_pair()
    route()


@jax.jit
def pallas_adaLN_cond__linear_kernel_hedgehog__moe_arch_mod__prompt_kernel(
    A_x: jax.Array,
    A_wqkv: jax.Array,
    A_w_phi: jax.Array,
    A_wo: jax.Array,
    B_x: jax.Array,
    B_w_r: jax.Array,
    B_w_gate: jax.Array,
    B_w_up: jax.Array,
    B_w_down: jax.Array,
    c: jax.Array,
    w_mod: jax.Array,
):
    del B_x
    batch, seq, d = A_x.shape
    assert batch == 1 and d == HEADS * HEAD_DIM and seq == 8 * TILE
    n_tiles = seq // TILE
    operands = (A_x.reshape(seq, d), A_wqkv, A_w_phi, A_wo, B_w_r, B_w_gate, B_w_up, B_w_down,
                c, w_mod)
    weight_terms = pltpu.VMEM((TERMS * d // 4, d // 2), I32)
    token_terms = pltpu.VMEM((TERMS * HALF // 2, d // 2), I32)
    scratch = [pltpu.VMEM(a.shape, a.dtype) for a in operands] + [
        weight_terms, weight_terms, weight_terms, weight_terms,
        pltpu.VMEM((d // 2, 128), I32),
        pltpu.VMEM((8, d), I32),
        pltpu.VMEM((8, 10 * d), F32),
        token_terms,
        [pltpu.VMEM((TERMS * d // 4, HALF), I32)] * 2,
        pltpu.VMEM((n_tiles * TERMS * d // 4, HALF), I32),
        [token_terms] * 2,
        [pltpu.VMEM((TILE, d), F32)] * 2,
        pltpu.VMEM((seq, d), F32),
        pltpu.VMEM((PAIRS * PAIR, 128), F32),
        pltpu.VMEM((PAIRS * HEAD_DIM, 128), I32),
        pltpu.VMEM((PAIRS * 128, 128), F32),
        pltpu.VMEM((n_tiles * 8, 128), F32),
        pltpu.VMEM((8, 128), I32),
        pltpu.VMEM((seq, d), A_x.dtype),
        pltpu.SemaphoreType.DMA((26,)),
    ]
    out = pl.pallas_call(
        _kernel,
        out_shape=jax.ShapeDtypeStruct((seq, d), A_x.dtype),
        in_specs=[pl.BlockSpec(memory_space=pl.ANY)] * len(operands),
        out_specs=pl.BlockSpec(memory_space=pl.ANY),
        scratch_shapes=scratch,
        compiler_params=pltpu.CompilerParams(
            vmem_limit_bytes=110 * 2**20,
            flags={"XLA_TPU_EVENLY_DISTRIBUTE_CRITICAL_NODES": True}),
        name="adaln_hedgehog_mod",
    )(*operands)
    return out.reshape(batch, seq, d)
```

```python
import collections
import functools
import math

import jax
import jax.numpy as jnp
from jax import lax
import jax.experimental.pallas as pl
import jax.experimental.pallas.tpu as pltpu

F32 = jnp.float32
BF16 = jnp.bfloat16
I32 = jnp.int32

HEADS = 32
HEAD_DIM = 32
PAIRS = HEADS // 2
PAIR = 2 * HEAD_DIM
TERMS = 7
TILE = 256
HALF = TILE // 2
CHUNK = 128
FFN_CHUNK = 512
LN_EPS = 1e-5
DEN_EPS = 1e-6
LOG2E = math.log2(math.e)

EARLY_WINDOWS = tuple((6 * n - 1, 6 * n + 16) for n in range(16))
OUTPUT_WINDOWS = tuple((55 + 6 * p, 67 + 6 * p) for p in range(8))
FINISH_WINDOWS = tuple((3 * g - 1, min(3 * g + 11, 55)) for g in range(16))
LAST_WINDOWS = tuple((7 * (g // 5), 7 * (g // 5) + 9) for g in range(16))
TAIL_WINDOWS = tuple((7 * (n // 3) - 1, 7 * (n // 3) + 9) for n in range(8))

QUERY, KEY, VALUE = range(3)
SHIFT_A, SCALE_A, GATE_A, SHIFT_B, SCALE_B, GATE_B, ROUTER, OUT_SCALE, OUT_SHIFT, SCORE = range(10)

Tile = collections.namedtuple("Tile", "x h h_all o x1 x1_all out score")


def _dot(a, b):
    return jnp.dot(a, b, preferred_element_type=F32)


def _dot_nt(a, b):
    return lax.dot_general(a, b, (((1,), (1,)), ((), ())), preferred_element_type=F32)


def _pack(v):
    return pltpu.bitcast(v.astype(BF16), I32)


def _pack_transposed(v):
    return pltpu.bitcast(v.astype(BF16).T, I32)


def _unpack(words):
    return pltpu.bitcast(words, BF16)


def _recip(v):
    r = pltpu.reciprocal(v, approx=True)
    return r * (2.0 - v * r)


def _sigmoid(v):
    return 1.0 / (1.0 + jnp.exp(-v))


def _rows(v, n):
    return jnp.concatenate([v] * (n // 8), axis=0)


def _centered(x, after=None):
    inv_d = 1.0 / x.shape[-1]
    if after is not None:
        head = x[:, :128] + _rows(pltpu.bitcast(after, F32), x.shape[0])
        x = jnp.concatenate([head, x[:, 128:]], axis=1)
    xc = x - jnp.sum(x, axis=-1, keepdims=True) * inv_d
    var = jnp.sum(xc * xc, axis=-1, keepdims=True) * inv_d
    return xc, lax.rsqrt(var + LN_EPS)


def _lhs_terms(a11, a12, a21, a22):
    return [a11 + a22, a21 + a22, a11, a22, a11 + a12, a21 - a11, a12 - a22]


def _rhs_terms(b11, b12, b21, b22):
    return [b11 + b22, b11, b12 - b22, b21 - b11, b22, b11 + b12, b21 + b22]


def _block_matmul(product):
    m5, m3 = product(4), product(2)
    c12 = m5 + m3
    m1 = product(0)
    c11, c22 = m1 - m5, m3 + m1
    c11 = c11 + product(6)
    m4 = product(3)
    c11 = c11 + m4
    m2 = product(1)
    c21, c22 = m4 + m2, c22 - m2
    c22 = c22 + product(5)
    return c11, c12, c21, c22


def _head_reduce(op, tiles):
    while len(tiles) > 1:
        tiles = [op(tiles[i], tiles[i + 1]) for i in range(0, len(tiles), 2)]
    m = tiles[0]
    m = op(m, pltpu.roll(m, 4, 0))
    return op(m, pltpu.roll(m, 2, 0))


def _feature_map(p):
    tiles = [p[8 * j:8 * j + 8] for j in range(PAIR // 8)]
    hi = _head_reduce(jnp.maximum, tiles)
    lo = _head_reduce(jnp.minimum, tiles)
    e_pos = [jnp.exp2(t - hi) for t in tiles]
    e_neg = [jnp.exp2(lo - t) for t in tiles]
    r_pos = _recip(_head_reduce(jnp.add, e_pos))
    r_neg = _recip(_head_reduce(jnp.add, e_neg))
    return [e * r_pos for e in e_pos] + [e * r_neg for e in e_neg]


class _Pacer:
    def __init__(self, zero_ref):
        self.zero_ref = zero_ref
        self.now = 0
        self.last = None
        self.jobs, self.gates, self.fillers = {}, {}, []

    def reset(self):
        assert not self.jobs and not self.fillers
        self.last, self.gates = None, {}

    def token(self, values):
        tiles = [pltpu.bitcast(v[r:r + 8, c:c + 128], I32) for v in values
                 for r in range(0, v.shape[0], 8) for c in range(0, v.shape[1], 128)]
        while len(tiles) > 1:
            tiles = [tiles[j] | tiles[j + 1] if j + 1 < len(tiles) else tiles[j]
                     for j in range(0, len(tiles), 2)]
        return tiles[0] & self.zero_ref[...]

    def plan(self, job, window):
        start, end = (self.now + w for w in window)
        if start < self.now:
            self._run(job, end)
        else:
            self.jobs.setdefault(start, []).append((job, end))

    def _run(self, job, end):
        self.gates.setdefault(end, []).append(job(self.last))

    def dot(self, lhs, rhs):
        for zero in self.gates.pop(self.now, []):
            top = jnp.concatenate([lhs[:8, :128] | zero, lhs[:8, 128:]], axis=1)
            lhs = jnp.concatenate([top, lhs[8:]], axis=0)
        out = _dot(_unpack(lhs), _unpack(rhs))
        self.last = self.token([out[-8:]])
        for job, end in self.jobs.pop(self.now, []):
            self._run(job, end)
        self.now += 1
        if self.fillers:
            self.fillers.pop(0)()
        return out


def _kernel(x_hbm, wqkv_hbm, wphi_hbm, wo_hbm, wr_hbm, wg_hbm, wu_hbm, wd_hbm, c_hbm, wmod_hbm,
            out_hbm,
            x_v, wqkv_v, wphi_v, wo_v, wr_v, wg_v, wu_v, wd_v, c_v, wmod_v,
            wq_s, wk_s, wv_s, wo_s, phi_s, act_s, vec_s, norm_s, h_s, h_all, o_s, x1_s, x1_all,
            kv_s, kvm_s, z_s, score_s, zero_s, out_v,
            sem):
    seq, d = x_v.shape
    hd = d // 2
    last = seq // (2 * TILE) - 1
    n_chunks = hd // CHUNK
    h_rows = HALF // 2
    w_rows = hd // 2
    pacer = _Pacer(zero_s)

    copy = pltpu.make_async_copy

    def view(ref, index, size):
        start = index * size
        return ref.at[pl.ds(start if isinstance(start, int) else pl.multiple_of(start, size), size)]

    def x_copy(first, count, s):
        return copy(x_hbm.at[pl.ds(first, count)], x_v.at[pl.ds(first, count)], s)

    c_cp = copy(c_hbm, c_v, sem.at[0])
    wphi_cp = copy(wphi_hbm, wphi_v, sem.at[1])
    wr_cp = copy(wr_hbm, wr_v, sem.at[2])
    mod_b_cp = copy(wmod_hbm.at[:, pl.ds(2 * d, 4 * d)], wmod_v.at[:, pl.ds(2 * d, 4 * d)],
                    sem.at[3])
    wq_cp = copy(wqkv_hbm.at[:, pl.ds(0, d)], wqkv_v.at[:, pl.ds(0, d)], sem.at[4])
    wo_cp = copy(wo_hbm, wo_v, sem.at[5])
    wg_cp = copy(wg_hbm, wg_v, sem.at[6])
    wu_cp = copy(wu_hbm, wu_v, sem.at[7])
    wd_cp = copy(wd_hbm, wd_v, sem.at[8])
    x_first_cp = x_copy(0, 2 * TILE, sem.at[9])
    x_next_cp = x_copy(2 * TILE, TILE, sem.at[10])
    x_rest_cp = x_copy(3 * TILE, seq - 3 * TILE, sem.at[11])

    def weight_copies(j):
        spans = [(pl.ds(half * hd + j * CHUNK, CHUNK), pl.ds(d, 2 * d)) for half in range(2)]
        return [copy(wqkv_hbm.at[span], wqkv_v.at[span], sem.at[12 + j]) for span in spans]

    def mod_a_copies(j):
        spans = [pl.ds(part * hd + j * CHUNK, CHUNK) for part in range(4)]
        return [copy(wmod_hbm.at[:, span], wmod_v.at[:, span], sem.at[16 + j]) for span in spans]

    def out_copy(i):
        return copy(view(out_v, i, 2 * TILE), view(out_hbm, i, 2 * TILE), sem.at[20 + i])

    def tile(i, parity):
        t = 2 * i + parity
        return Tile(x=view(x_v, t, TILE), h=h_s[parity], h_all=view(h_all, t, TERMS * w_rows),
                    o=o_s[parity], x1=x1_s[parity], x1_all=view(x1_all, t, TILE),
                    out=view(out_v, t, TILE), score=view(score_s, t, 8))

    def feature_blocks():
        row = lax.broadcasted_iota(I32, (128, 128), 0)
        lane = lax.broadcasted_iota(I32, (128, 128), 1)
        same_head = 2 * (row // PAIR) + row % 2 == lane // HEAD_DIM
        row_f = lax.broadcasted_iota(I32, (128, HEAD_DIM), 0)
        lane_f = lax.broadcasted_iota(I32, (128, HEAD_DIM), 1)
        pick = jnp.where(row_f % PAIR // 2 == lane_f, 1.0, 0.0).astype(BF16)
        for g in range(d // 128):
            wphi = wphi_v[4 * g:4 * g + 4].reshape(128, HEAD_DIM)
            phi_s[g * 64:(g + 1) * 64, :] = _pack(jnp.where(same_head, _dot_nt(pick, wphi), 0.0))

    def projection_terms(col, j, g):
        def group(g):
            span = slice(col * d + g * CHUNK, col * d + (g + 1) * CHUNK)
            w = jnp.concatenate(
                [wqkv_v[r + j * CHUNK:r + (j + 1) * CHUNK, span] for r in (0, hd)], axis=0)
            if col == VALUE:
                return w.astype(F32).T
            return _dot_nt(_unpack(phi_s[g * 64:(g + 1) * 64, :]), w) * LOG2E

        top, bottom = group(g), group(g + n_chunks)
        terms = _lhs_terms(top[:, :CHUNK], top[:, CHUNK:], bottom[:, :CHUNK], bottom[:, CHUNK:])
        for i, term in enumerate(terms):
            r0 = i * w_rows + g * CHUNK // 2
            (wq_s, wk_s, wv_s)[col][r0:r0 + CHUNK // 2, j * CHUNK:(j + 1) * CHUNK] = _pack(term)

    def output_terms(p, c, after):
        def block(r0, c0):
            words = pltpu.bitcast(wo_v[r0:r0 + PAIR, c0:c0 + CHUNK], I32) | _rows(after, HEAD_DIM)
            return _unpack(words).astype(F32)

        blocks = (block(r + p * PAIR, k + c * CHUNK) for r in (0, hd) for k in (0, hd))
        terms = _rhs_terms(*blocks)
        for i, term in enumerate(terms):
            r0 = i * w_rows + p * HEAD_DIM
            wo_s[r0:r0 + HEAD_DIM, c * CHUNK:(c + 1) * CHUNK] = _pack(term)
        return pacer.token([term[-8:] for term in terms])

    def vec(i):
        return vec_s[:, i * d:(i + 1) * d]

    def modulation_rounds(i):
        partial = {}

        def one(c0, half):
            span = slice(half * hd, (half + 1) * hd)
            m = _dot(_unpack(act_s[:, span]), wmod_v[span, c0:c0 + 128])[0:8]
            if half == 0:
                partial[c0] = 1.0 + m if i == SCALE_B else m
            else:
                vec_s[:, c0:c0 + 128] = partial[c0] + m

        return [functools.partial(one, c0, half)
                for c0 in range(i * d, (i + 1) * d, 128) for half in range(2)]

    def derived_vectors():
        router = jnp.broadcast_to(wr_v[...].astype(F32).reshape(1, d), (8, d))
        for i, v in ((ROUTER, router), (OUT_SCALE, vec(GATE_B) * vec(SCALE_B)),
                     (OUT_SHIFT, vec(GATE_B) * vec(SHIFT_B)), (SCORE, router * vec(SCALE_B))):
            vec_s[:, i * d:(i + 1) * d] = v

    def normed_rows(t, r0):
        xc, rstd = _centered(t.x[r0:r0 + 16, :].astype(F32))
        return xc * rstd

    def normalize(t):
        for r0 in range(0, HALF, 16):
            ha, hb = (normed_rows(t, r + r0) * _rows(vec(SCALE_A), 16) + _rows(vec(SHIFT_A), 16)
                      for r in (0, HALF))
            for j, term in enumerate(_rhs_terms(ha[:, :hd], hb[:, :hd], ha[:, hd:], hb[:, hd:])):
                norm_s[j * h_rows + r0 // 2:j * h_rows + r0 // 2 + 8, :] = _pack(term)
        for j in range(TERMS):
            term = _pack_transposed(_unpack(norm_s[j * h_rows:(j + 1) * h_rows, :]))
            t.h[j * w_rows:(j + 1) * w_rows, :] = term
            t.h_all[j * w_rows:(j + 1) * w_rows, :] = term

    def fetch(t):
        for j in range(TERMS):
            t.h[j * w_rows:(j + 1) * w_rows, :] = t.h_all[j * w_rows:(j + 1) * w_rows, :]

    def project(w_s, t, m):
        def product(j):
            r0 = j * w_rows + m * CHUNK // 2
            return pacer.dot(w_s[r0:r0 + CHUNK // 2, :], t.h[j * w_rows:(j + 1) * w_rows, :])

        c11, c12, c21, c22 = _block_matmul(product)
        halves = (jnp.concatenate([c11, c12], axis=1), jnp.concatenate([c21, c22], axis=1))
        return [(side * PAIRS // 2 + m * CHUNK // PAIR + j, block[j * PAIR:(j + 1) * PAIR])
                for side, block in enumerate(halves) for j in range(CHUNK // PAIR)]

    def key_features(p, pk):
        phi = jnp.concatenate(_feature_map(pk), axis=0)
        z_s[p * 128:(p + 1) * 128, :] += phi[:, :HALF] + phi[:, HALF:]
        return phi

    def accumulate_kv(phi, v):
        for phi_p, (p, v_p) in zip(phi, v, strict=True):
            kv_s[p * PAIR:(p + 1) * PAIR, :] += _dot_nt(v_p.astype(BF16), phi_p.astype(BF16))

    def summarize(t, owed, between=lambda: None, flush=False):
        for m in range(n_chunks):
            pk = project(wk_s, t, m)
            if not (flush and m + 1 == n_chunks):
                while owed:
                    accumulate_kv(*owed.pop(0))
            between()
            owed.append(([key_features(*pair) for pair in pk], project(wv_s, t, m)))
            between()
        while flush and owed:
            accumulate_kv(*owed.pop(0))
        return owed

    def early_product(col, i):
        n = (col - KEY) * TERMS + i
        return x1_all.at[pl.ds(n // 4 * hd, hd), pl.ds(n % 4 * TILE, TILE)]

    def early_features(q, b):
        def block(col):
            return _block_matmul(lambda i: early_product(col, i)[q * PAIR:(q + 1) * PAIR, :])[b]

        return b // 2 * PAIRS // 2 + q, block(KEY), block(VALUE)

    def query_features(p, pq):
        phi = _feature_map(pq)
        z = [z_s[p * 128 + 8 * j:p * 128 + 8 * j + 8, :] for j in range(len(phi))]
        den = _head_reduce(
            jnp.add, [f * jnp.concatenate([zj, zj], axis=1) for f, zj in zip(phi, z)])
        inv = _recip(den + DEN_EPS)
        even = lax.broadcasted_iota(I32, inv.shape, 0) % 2 == 0
        other = pltpu.roll(inv, 1, 0)
        per_head = [jnp.where(even, inv, other), jnp.where(even, other, inv)]
        return (p, jnp.concatenate(phi, axis=0).astype(BF16),
                jnp.concatenate([_rows(v, HEAD_DIM) for v in per_head], axis=0))

    def queries(t, m):
        return [query_features(*pair) for pair in project(wq_s, t, m)]

    def read_out(t, m, features):
        o_t = [_dot(_unpack(kvm_s[p * HEAD_DIM:(p + 1) * HEAD_DIM, :]), phi) * inv
               for p, phi, inv in features]
        top = jnp.concatenate(o_t[:len(o_t) // 2], axis=0)
        bottom = jnp.concatenate(o_t[len(o_t) // 2:], axis=0)
        terms = _lhs_terms(top[:, :HALF], bottom[:, :HALF], top[:, HALF:], bottom[:, HALF:])
        for j, term in enumerate(terms):
            t.o[j * h_rows:(j + 1) * h_rows, m * CHUNK:(m + 1) * CHUNK] = _pack_transposed(term)

    def residual(t, g, first=0, count=HALF):
        def product(j):
            return pacer.dot(t.o[j * h_rows + first // 2:j * h_rows + (first + count) // 2, :],
                             wo_s[j * w_rows:(j + 1) * w_rows, g * CHUNK:(g + 1) * CHUNK])

        for b, attn in enumerate(_block_matmul(product)):
            span = (slice(b // 2 * HALF + first, b // 2 * HALF + first + count),
                    slice(b % 2 * hd + g * CHUNK, b % 2 * hd + (g + 1) * CHUNK))
            gate = vec_s[:, GATE_A * d + span[1].start:GATE_A * d + span[1].stop]
            x1 = t.x[span].astype(F32) + _rows(gate, count) * attn
            t.x1[span] = x1
            t.x1_all[span] = x1

    def finish(t, g, after=None):
        x1 = t.x1[16 * g:16 * g + 16, :]
        xc, rstd = _centered(x1, after)
        out = x1 + (xc * rstd * _rows(vec(OUT_SCALE), 16) + _rows(vec(OUT_SHIFT), 16))
        t.out[16 * g:16 * g + 16, :] = out.astype(BF16)
        score = jnp.sum(xc * _rows(vec(SCORE), 16), axis=-1, keepdims=True) * rstd
        lane = lax.broadcasted_iota(I32, (8, 128), 1)
        packed = t.score[...]
        for s in range(2):
            packed = jnp.where(lane == 2 * g + s, score[8 * s:8 * s + 8], packed)
        t.score[...] = packed
        return pacer.token([packed, out[:, -128:]])

    def finishing(t, groups, windows):
        for g, window in zip(groups, windows, strict=True):
            pacer.plan(functools.partial(finish, t, g), window)

    def attend(t, previous, after_first=lambda: None):
        ready = queries(t, 0)
        after_first()
        for m in range(n_chunks - 1):
            ahead = queries(t, m + 1)
            residual(previous, m)
            read_out(t, m, ready)
            ready = ahead
        read_out(t, n_chunks - 1, ready)
        residual(previous, n_chunks - 1)

    def start_up():
        early = (tile(0, 0), tile(0, 1))
        cf = c_v[...].astype(F32)
        act_s[...] = _pack(jnp.broadcast_to(cf * _sigmoid(cf), (16, d)))
        wphi_cp.wait()
        feature_blocks()

        def weight_terms(j):
            for cp in weight_copies(j):
                cp.wait()
            for g in range(n_chunks):
                projection_terms(KEY, j, g)
                projection_terms(VALUE, j, g)

        def activation_terms(j):
            for cp in mod_a_copies(j):
                cp.wait()
            parts = [slice(part * hd + j * CHUNK, part * hd + (j + 1) * CHUNK) for part in range(4)]
            m = _dot(_unpack(act_s[...]),
                     jnp.concatenate([wmod_v[:, part] for part in parts], axis=1))[0:8]
            vectors = [m[:, :128], m[:, 128:256], 1.0 + m[:, 256:384], 1.0 + m[:, 384:]]
            for part, v in zip(parts, vectors):
                vec_s[:, part] = v
            shifts, scales = vectors[:2], vectors[2:]
            for t in early:
                blocks = (t.x1[r:r + HALF, part] * _rows(scale, HALF) + _rows(shift, HALF)
                          for part, scale, shift in zip(parts, scales, shifts) for r in (0, HALF))
                for i, term in enumerate(_rhs_terms(*blocks)):
                    r0 = i * w_rows + j * CHUNK // 2
                    t.h_all[r0:r0 + CHUNK // 2, :] = _pack_transposed(term)

        x_first_cp.wait()
        for t in early:
            for r0 in range(0, TILE, 16):
                t.x1[r0:r0 + 16, :] = normed_rows(t, r0)
        weight_terms(0)
        activation_terms(0)
        for j in range(n_chunks):
            for i in range(TERMS):
                if i == 2 and j + 1 < n_chunks:
                    weight_terms(j + 1)
                if i == 5 and j + 1 < n_chunks:
                    activation_terms(j + 1)
                if i == 0 and j + 1 == n_chunks:
                    x_next_cp.wait()
                    normalize(tile(1, 0))
                r0 = i * w_rows + j * CHUNK // 2
                h = jnp.concatenate([t.h_all[r0:r0 + CHUNK // 2, :] for t in early], axis=1)
                for col, w_s in ((KEY, wk_s), (VALUE, wv_s)):
                    w = w_s[i * w_rows:(i + 1) * w_rows, j * CHUNK:(j + 1) * CHUNK]
                    product = _dot(_unpack(w), _unpack(h))
                    acc = early_product(col, i)
                    acc[...] = product + acc[...] if j else product
        for cp in (wq_cp, wo_cp, wr_cp):
            cp.start()

    def summarize_pair(i, copies):
        ready = []

        def job(n, end, after):
            p, pk, v = early_features(n // 4, n % 4)
            if after is not None:
                pk = pk + _rows(jnp.concatenate([pltpu.bitcast(after, F32)] * 2, axis=1), PAIR)
            phi = key_features(p, pk)
            ready.append((end, [phi], [(p, v)]))
            return pacer.token([phi[PAIR - 8:PAIR], phi[-8:]])

        def drain():
            while ready and ready[0][0] <= pacer.now:
                accumulate_kv(*ready.pop(0)[1:])

        for n, window in enumerate(EARLY_WINDOWS):
            pacer.plan(functools.partial(
                job, (i - 1) * len(EARLY_WINDOWS) + n, pacer.now + window[1]), window)
        copies[0].start()
        normalize(tile(i, 1))
        owed = summarize(tile(i, 0), [], drain)
        copies[1].start()
        normalize(tile(i + 1, 0))
        summarize(tile(i, 1), owed, drain, flush=True)
        assert not ready

    def summarize_last_pair():
        for cp in (wq_cp, wo_cp, wr_cp, mod_b_cp):
            cp.wait()
        normalize(tile(last, 1))
        for p, window in enumerate(OUTPUT_WINDOWS):
            for c in range(n_chunks):
                pacer.plan(functools.partial(output_terms, p, c), window)
        for j in range(n_chunks):
            for g in range(n_chunks):
                pacer.fillers += [functools.partial(projection_terms, QUERY, j, g),
                                  lambda: None, lambda: None]
        summarize(tile(last, 1), summarize(tile(last, 0), []), flush=True)

    def attend_first_pair():
        row = lax.broadcasted_iota(I32, (PAIR, 128), 0)
        lane = lax.broadcasted_iota(I32, (PAIR, 128), 1)
        for p in range(PAIRS):
            kv = jnp.where(row // HEAD_DIM == lane % 2, kv_s[p * PAIR:(p + 1) * PAIR, :], 0.0)
            kvm_s[p * HEAD_DIM:(p + 1) * HEAD_DIM, :] = _pack(kv)
            z = jnp.sum(z_s[p * 128:(p + 1) * 128, :], axis=1, keepdims=True)
            z_s[p * 128:(p + 1) * 128, :] = jnp.broadcast_to(z, (128, 128))
        for i in (GATE_A, SHIFT_B, SCALE_B, GATE_B):
            pacer.fillers += modulation_rounds(i)
        first = tile(0, 0)
        fetch(first)
        fetch(tile(0, 1))
        ready = queries(first, 0)
        for m in range(n_chunks - 1):
            ahead = queries(first, m + 1)
            read_out(first, m, ready)
            ready = ahead
        fetch(tile(1, 0))
        attend(tile(0, 1), first, lambda: read_out(first, n_chunks - 1, ready))
        derived_vectors()

    def attend_pairs():
        def body(i, carry):
            pacer.reset()
            tiles = [tile(i - 1, 0), tile(i - 1, 1), tile(i, 0), tile(i, 1),
                     tile(jnp.minimum(i + 1, last), 0)]
            for k in range(2):
                fetch(tiles[k + 3])
                finishing(tiles[k], range(TILE // 16), FINISH_WINDOWS)
                attend(tiles[k + 2], tiles[k + 1])
            out_copy(i - 1).start()
            return carry

        lax.fori_loop(1, last + 1, body, 0)

    def finish_last_pair():
        for cp in (wg_cp, wu_cp, wd_cp):
            cp.wait()
        final = tile(last, 1)
        groups = [[(r + k * HALF // 2 + side * HALF) // 16 for side in range(2)
                   for r in range(0, HALF // 2, 16)] for k in range(2)]
        finishing(tile(last, 0), range(TILE // 16), LAST_WINDOWS)
        for g in range(n_chunks):
            residual(final, g, 0, HALF // 2)
        finishing(final, groups[0], TAIL_WINDOWS)
        for g in range(n_chunks):
            residual(final, g, HALF // 2, HALF // 2)
        for g in groups[1]:
            finish(final, g)

    def route():
        scores = score_s[...]
        row = lax.broadcasted_iota(I32, scores.shape, 0)
        lane = lax.broadcasted_iota(I32, scores.shape, 1)
        index = jnp.where(
            lane < TILE // 8, (row // 8) * TILE + lane * 8 + row % 8, seq).astype(F32)

        def everywhere(op, v):
            return op(op(v, axis=0, keepdims=True), axis=1, keepdims=True)

        valid = index < seq
        best = everywhere(jnp.max, jnp.where(valid, scores, -jnp.inf))
        tied = valid & (scores == best)
        below = valid & jnp.logical_not(tied)
        runner_up = everywhere(jnp.max, jnp.where(below, scores, -jnp.inf))
        first = everywhere(jnp.min, jnp.where(tied, index, seq - 1.0))
        second = everywhere(jnp.min, jnp.where(
            tied & (index != first), index,
            jnp.where(below & (scores == runner_up), index + seq, 2 * seq - 1.0)))
        i0, i1 = first.astype(I32)[0, 0], second.astype(I32)[0, 0] % seq

        sub = lax.broadcasted_iota(I32, (16, d), 0)
        x1 = jnp.where(sub == 0, x1_all[pl.ds(i0, 1), :], x1_all[pl.ds(i1, 1), :])
        xc, rstd = _centered(x1)
        h2 = xc * rstd * _rows(vec(SCALE_B), 16) + _rows(vec(SHIFT_B), 16)
        gate = _sigmoid(jnp.sum(h2 * _rows(vec(ROUTER), 16), axis=-1, keepdims=True))
        xs = h2.astype(BF16)
        out_copy(last).start()
        spans = [slice(f, f + FFN_CHUNK) for f in range(0, wd_v.shape[0], FFN_CHUNK)]
        y, hidden = 0.0, None
        for k in range(len(spans) + 1):
            if k < len(spans):
                g, u = _dot(xs, wg_v[:, spans[k]]), _dot(xs, wu_v[:, spans[k]])
            if k > 0:
                y = y + _dot(hidden, wd_v[spans[k - 1], :])
            hidden = (g * _sigmoid(g) * u).astype(BF16)
        routed = x1 + _rows(vec(GATE_B), 16) * (h2 + y * gate)

        for i in range(last + 1):
            out_copy(i).wait()

        def patch(k, i):
            base = pl.multiple_of((i // 16) * 16, 16)
            old = out_v[pl.ds(base, 16), :].astype(F32)
            out_v[pl.ds(base, 16), :] = jnp.where(
                sub == i - base, routed[k:k + 1], old).astype(BF16)
            return base, copy(out_v.at[pl.ds(base, 16)], out_hbm.at[pl.ds(base, 16)],
                              sem.at[24 + k])

        base0, patch0 = patch(0, i0)
        base1, patch1 = patch(1, i1)
        patch0.start()

        @pl.when(base1 != base0)
        def _():
            patch1.start()
            patch1.wait()

        patch0.wait()

    for cp in (c_cp, wphi_cp, x_first_cp):
        cp.start()
    for j in range(n_chunks):
        for cp in weight_copies(j) + mod_a_copies(j):
            cp.start()
    x_next_cp.start()
    x_rest_cp.start()
    kv_s[...] = jnp.zeros(kv_s.shape, F32)
    z_s[...] = jnp.zeros(z_s.shape, F32)
    score_s[...] = jnp.full(score_s.shape, -jnp.inf, F32)
    c_cp.wait()
    words = pltpu.bitcast(jnp.broadcast_to(c_v[:, :128].astype(F32), (8, 128)), I32)
    zero = jnp.minimum(lax.shift_right_logical(words, 1), 0)
    zero_s[...] = zero
    origin = jnp.max(zero)

    def own_block(k, step):
        pacer.reset()
        pl.when(origin <= k)(step)
        pacer.reset()

    start_up()
    x_rest_cp.wait()
    own_block(1, functools.partial(summarize_pair, 1, (mod_b_cp, wg_cp)))
    summarize_pair(2, (wu_cp, wd_cp))
    own_block(2, summarize_last_pair)
    attend_first_pair()
    attend_pairs()
    pacer.reset()
    finish_last_pair()
    route()


@jax.jit
def pallas_adaLN_cond__linear_kernel_hedgehog__moe_arch_mod__prompt_kernel(
    A_x: jax.Array,
    A_wqkv: jax.Array,
    A_w_phi: jax.Array,
    A_wo: jax.Array,
    B_x: jax.Array,
    B_w_r: jax.Array,
    B_w_gate: jax.Array,
    B_w_up: jax.Array,
    B_w_down: jax.Array,
    c: jax.Array,
    w_mod: jax.Array,
):
    del B_x
    batch, seq, d = A_x.shape
    assert batch == 1 and d == HEADS * HEAD_DIM and seq == 8 * TILE
    n_tiles = seq // TILE
    operands = (A_x.reshape(seq, d), A_wqkv, A_w_phi, A_wo, B_w_r, B_w_gate, B_w_up, B_w_down,
                c, w_mod)
    weight_terms = pltpu.VMEM((TERMS * d // 4, d // 2), I32)
    token_terms = pltpu.VMEM((TERMS * HALF // 2, d // 2), I32)
    scratch = [pltpu.VMEM(a.shape, a.dtype) for a in operands] + [
        weight_terms, weight_terms, weight_terms, weight_terms,
        pltpu.VMEM((d // 2, 128), I32),
        pltpu.VMEM((8, d), I32),
        pltpu.VMEM((8, 10 * d), F32),
        token_terms,
        [pltpu.VMEM((TERMS * d // 4, HALF), I32)] * 2,
        pltpu.VMEM((n_tiles * TERMS * d // 4, HALF), I32),
        [token_terms] * 2,
        [pltpu.VMEM((TILE, d), F32)] * 2,
        pltpu.VMEM((seq, d), F32),
        pltpu.VMEM((PAIRS * PAIR, 128), F32),
        pltpu.VMEM((PAIRS * HEAD_DIM, 128), I32),
        pltpu.VMEM((PAIRS * 128, 128), F32),
        pltpu.VMEM((n_tiles * 8, 128), F32),
        pltpu.VMEM((8, 128), I32),
        pltpu.VMEM((seq, d), A_x.dtype),
        pltpu.SemaphoreType.DMA((26,)),
    ]
    out = pl.pallas_call(
        _kernel,
        out_shape=jax.ShapeDtypeStruct((seq, d), A_x.dtype),
        in_specs=[pl.BlockSpec(memory_space=pl.ANY)] * len(operands),
        out_specs=pl.BlockSpec(memory_space=pl.ANY),
        scratch_shapes=scratch,
        compiler_params=pltpu.CompilerParams(
            vmem_limit_bytes=110 * 2**20,
            flags={"XLA_TPU_EVENLY_DISTRIBUTE_CRITICAL_NODES": True}),
        name="adaln_hedgehog_mod",
    )(*operands)
    return out.reshape(batch, seq, d)
```

```python
import collections
import functools
import math

import jax
import jax.numpy as jnp
from jax import lax
import jax.experimental.pallas as pl
import jax.experimental.pallas.tpu as pltpu

F32 = jnp.float32
BF16 = jnp.bfloat16
I32 = jnp.int32

HEADS = 32
HEAD_DIM = 32
PAIRS = HEADS // 2
PAIR = 2 * HEAD_DIM
TERMS = 7
TILE = 256
HALF = TILE // 2
CHUNK = 128
FFN_CHUNK = 512
LN_EPS = 1e-5
DEN_EPS = 1e-6
LOG2E = math.log2(math.e)

EARLY_WINDOWS = tuple((6 * n - 1, 6 * n + 16) for n in range(16))
OUTPUT_WINDOWS = tuple((55 + 6 * p, 67 + 6 * p) for p in range(8))
FINISH_WINDOWS = tuple((3 * g - 1, min(3 * g + 11, 55)) for g in range(16))
LAST_WINDOWS = tuple((7 * (g // 5), 7 * (g // 5) + 9) for g in range(16))
TAIL_WINDOWS = tuple((7 * (n // 3) - 1, 7 * (n // 3) + 9) for n in range(8))

QUERY, KEY, VALUE = range(3)
SHIFT_A, SCALE_A, GATE_A, SHIFT_B, SCALE_B, GATE_B, ROUTER, OUT_SCALE, OUT_SHIFT, SCORE = range(10)

Tile = collections.namedtuple("Tile", "x h h_all o x1 x1_all out score")


def _dot(a, b):
    return jnp.dot(a, b, preferred_element_type=F32)


def _dot_nt(a, b):
    return lax.dot_general(a, b, (((1,), (1,)), ((), ())), preferred_element_type=F32)


def _pack(v):
    return pltpu.bitcast(v.astype(BF16), I32)


def _pack_transposed(v):
    return pltpu.bitcast(v.astype(BF16).T, I32)


def _unpack(words):
    return pltpu.bitcast(words, BF16)


def _recip(v):
    r = pltpu.reciprocal(v, approx=True)
    return r * (2.0 - v * r)


def _sigmoid(v):
    return 1.0 / (1.0 + jnp.exp(-v))


def _rows(v, n):
    return jnp.concatenate([v] * (n // 8), axis=0)


def _centered(x, after=None):
    inv_d = 1.0 / x.shape[-1]
    if after is not None:
        head = x[:, :128] + _rows(pltpu.bitcast(after, F32), x.shape[0])
        x = jnp.concatenate([head, x[:, 128:]], axis=1)
    xc = x - jnp.sum(x, axis=-1, keepdims=True) * inv_d
    var = jnp.sum(xc * xc, axis=-1, keepdims=True) * inv_d
    return xc, lax.rsqrt(var + LN_EPS)


def _lhs_terms(a11, a12, a21, a22):
    return [a11 + a22, a21 + a22, a11, a22, a11 + a12, a21 - a11, a12 - a22]


def _rhs_terms(b11, b12, b21, b22):
    return [b11 + b22, b11, b12 - b22, b21 - b11, b22, b11 + b12, b21 + b22]


def _block_matmul(product):
    m5, m3 = product(4), product(2)
    c12 = m5 + m3
    m1 = product(0)
    c11, c22 = m1 - m5, m3 + m1
    c11 = c11 + product(6)
    m4 = product(3)
    c11 = c11 + m4
    m2 = product(1)
    c21, c22 = m4 + m2, c22 - m2
    c22 = c22 + product(5)
    return c11, c12, c21, c22


def _head_reduce(op, tiles):
    while len(tiles) > 1:
        tiles = [op(tiles[i], tiles[i + 1]) for i in range(0, len(tiles), 2)]
    m = tiles[0]
    m = op(m, pltpu.roll(m, 4, 0))
    return op(m, pltpu.roll(m, 2, 0))


def _feature_map(p):
    tiles = [p[8 * j:8 * j + 8] for j in range(PAIR // 8)]
    hi = _head_reduce(jnp.maximum, tiles)
    lo = _head_reduce(jnp.minimum, tiles)
    e_pos = [jnp.exp2(t - hi) for t in tiles]
    e_neg = [jnp.exp2(lo - t) for t in tiles]
    r_pos = _recip(_head_reduce(jnp.add, e_pos))
    r_neg = _recip(_head_reduce(jnp.add, e_neg))
    return [e * r_pos for e in e_pos] + [e * r_neg for e in e_neg]


class _Pacer:
    def __init__(self, zero_ref):
        self.zero_ref = zero_ref
        self.now = 0
        self.last = None
        self.jobs, self.gates, self.fillers = {}, {}, []

    def reset(self):
        assert not self.jobs and not self.fillers
        self.last, self.gates = None, {}

    def token(self, values):
        tiles = [pltpu.bitcast(v[r:r + 8, c:c + 128], I32) for v in values
                 for r in range(0, v.shape[0], 8) for c in range(0, v.shape[1], 128)]
        while len(tiles) > 1:
            tiles = [tiles[j] | tiles[j + 1] if j + 1 < len(tiles) else tiles[j]
                     for j in range(0, len(tiles), 2)]
        return tiles[0] & self.zero_ref[...]

    def plan(self, job, window):
        start, end = (self.now + w for w in window)
        if start < self.now:
            self._run(job, end)
        else:
            self.jobs.setdefault(start, []).append((job, end))

    def _run(self, job, end):
        self.gates.setdefault(end, []).append(job(self.last))

    def dot(self, lhs, rhs):
        for zero in self.gates.pop(self.now, []):
            top = jnp.concatenate([lhs[:8, :128] | zero, lhs[:8, 128:]], axis=1)
            lhs = jnp.concatenate([top, lhs[8:]], axis=0)
        out = _dot(_unpack(lhs), _unpack(rhs))
        self.last = self.token([out[-8:]])
        for job, end in self.jobs.pop(self.now, []):
            self._run(job, end)
        self.now += 1
        if self.fillers:
            self.fillers.pop(0)()
        return out


def _kernel(x_hbm, wqkv_hbm, wphi_hbm, wo_hbm, wr_hbm, wg_hbm, wu_hbm, wd_hbm, c_hbm, wmod_hbm,
            out_hbm,
            x_v, wqkv_v, wphi_v, wo_v, wr_v, wg_v, wu_v, wd_v, c_v, wmod_v,
            wq_s, wk_s, wv_s, wo_s, phi_s, act_s, vec_s, norm_s, h_s, h_all, o_s, x1_s, x1_all,
            kv_s, kvm_s, z_s, score_s, zero_s, out_v,
            sem):
    seq, d = x_v.shape
    hd = d // 2
    last = seq // (2 * TILE) - 1
    n_chunks = hd // CHUNK
    h_rows = HALF // 2
    w_rows = hd // 2
    pacer = _Pacer(zero_s)

    copy = pltpu.make_async_copy

    def view(ref, index, size):
        start = index * size
        return ref.at[pl.ds(start if isinstance(start, int) else pl.multiple_of(start, size), size)]

    def x_copy(first, count, s):
        return copy(x_hbm.at[pl.ds(first, count)], x_v.at[pl.ds(first, count)], s)

    c_cp = copy(c_hbm, c_v, sem.at[0])
    wphi_cp = copy(wphi_hbm, wphi_v, sem.at[1])
    wr_cp = copy(wr_hbm, wr_v, sem.at[2])
    mod_b_cp = copy(wmod_hbm.at[:, pl.ds(2 * d, 4 * d)], wmod_v.at[:, pl.ds(2 * d, 4 * d)],
                    sem.at[3])
    wq_cp = copy(wqkv_hbm.at[:, pl.ds(0, d)], wqkv_v.at[:, pl.ds(0, d)], sem.at[4])
    wo_cp = copy(wo_hbm, wo_v, sem.at[5])
    wg_cp = copy(wg_hbm, wg_v, sem.at[6])
    wu_cp = copy(wu_hbm, wu_v, sem.at[7])
    wd_cp = copy(wd_hbm, wd_v, sem.at[8])
    x_first_cp = x_copy(0, 2 * TILE, sem.at[9])
    x_next_cp = x_copy(2 * TILE, TILE, sem.at[10])
    x_rest_cp = x_copy(3 * TILE, seq - 3 * TILE, sem.at[11])

    def weight_copies(j):
        spans = [(pl.ds(half * hd + j * CHUNK, CHUNK), pl.ds(d, 2 * d)) for half in range(2)]
        return [copy(wqkv_hbm.at[span], wqkv_v.at[span], sem.at[12 + j]) for span in spans]

    def mod_a_copies(j):
        spans = [pl.ds(part * hd + j * CHUNK, CHUNK) for part in range(4)]
        return [copy(wmod_hbm.at[:, span], wmod_v.at[:, span], sem.at[16 + j]) for span in spans]

    def out_copy(i):
        return copy(view(out_v, i, 2 * TILE), view(out_hbm, i, 2 * TILE), sem.at[20 + i])

    def tile(i, parity):
        t = 2 * i + parity
        return Tile(x=view(x_v, t, TILE), h=h_s[parity], h_all=view(h_all, t, TERMS * w_rows),
                    o=o_s[parity], x1=x1_s[parity], x1_all=view(x1_all, t, TILE),
                    out=view(out_v, t, TILE), score=view(score_s, t, 8))

    def feature_blocks():
        row = lax.broadcasted_iota(I32, (128, 128), 0)
        lane = lax.broadcasted_iota(I32, (128, 128), 1)
        same_head = 2 * (row // PAIR) + row % 2 == lane // HEAD_DIM
        row_f = lax.broadcasted_iota(I32, (128, HEAD_DIM), 0)
        lane_f = lax.broadcasted_iota(I32, (128, HEAD_DIM), 1)
        pick = jnp.where(row_f % PAIR // 2 == lane_f, 1.0, 0.0).astype(BF16)
        for g in range(d // 128):
            wphi = wphi_v[4 * g:4 * g + 4].reshape(128, HEAD_DIM)
            phi_s[g * 64:(g + 1) * 64, :] = _pack(jnp.where(same_head, _dot_nt(pick, wphi), 0.0))

    def projection_terms(col, j, g):
        def group(g):
            span = slice(col * d + g * CHUNK, col * d + (g + 1) * CHUNK)
            w = jnp.concatenate(
                [wqkv_v[r + j * CHUNK:r + (j + 1) * CHUNK, span] for r in (0, hd)], axis=0)
            if col == VALUE:
                return w.astype(F32).T
            return _dot_nt(_unpack(phi_s[g * 64:(g + 1) * 64, :]), w) * LOG2E

        top, bottom = group(g), group(g + n_chunks)
        terms = _lhs_terms(top[:, :CHUNK], top[:, CHUNK:], bottom[:, :CHUNK], bottom[:, CHUNK:])
        for i, term in enumerate(terms):
            r0 = i * w_rows + g * CHUNK // 2
            (wq_s, wk_s, wv_s)[col][r0:r0 + CHUNK // 2, j * CHUNK:(j + 1) * CHUNK] = _pack(term)

    def output_terms(p, c, after):
        def block(r0, c0):
            words = pltpu.bitcast(wo_v[r0:r0 + PAIR, c0:c0 + CHUNK], I32) | _rows(after, HEAD_DIM)
            return _unpack(words).astype(F32)

        blocks = (block(r + p * PAIR, k + c * CHUNK) for r in (0, hd) for k in (0, hd))
        terms = _rhs_terms(*blocks)
        for i, term in enumerate(terms):
            r0 = i * w_rows + p * HEAD_DIM
            wo_s[r0:r0 + HEAD_DIM, c * CHUNK:(c + 1) * CHUNK] = _pack(term)
        return pacer.token([term[-8:] for term in terms])

    def vec(i):
        return vec_s[:, i * d:(i + 1) * d]

    def modulation_rounds(i):
        partial = {}

        def one(c0, half):
            span = slice(half * hd, (half + 1) * hd)
            m = _dot(_unpack(act_s[:, span]), wmod_v[span, c0:c0 + 128])[0:8]
            if half == 0:
                partial[c0] = 1.0 + m if i == SCALE_B else m
            else:
                vec_s[:, c0:c0 + 128] = partial[c0] + m

        return [functools.partial(one, c0, half)
                for c0 in range(i * d, (i + 1) * d, 128) for half in range(2)]

    def derived_vectors():
        router = jnp.broadcast_to(wr_v[...].astype(F32).reshape(1, d), (8, d))
        for i, v in ((ROUTER, router), (OUT_SCALE, vec(GATE_B) * vec(SCALE_B)),
                     (OUT_SHIFT, vec(GATE_B) * vec(SHIFT_B)), (SCORE, router * vec(SCALE_B))):
            vec_s[:, i * d:(i + 1) * d] = v

    def normed_rows(t, r0):
        xc, rstd = _centered(t.x[r0:r0 + 16, :].astype(F32))
        return xc * rstd

    def normalize(t):
        for r0 in range(0, HALF, 16):
            ha, hb = (normed_rows(t, r + r0) * _rows(vec(SCALE_A), 16) + _rows(vec(SHIFT_A), 16)
                      for r in (0, HALF))
            for j, term in enumerate(_rhs_terms(ha[:, :hd], hb[:, :hd], ha[:, hd:], hb[:, hd:])):
                norm_s[j * h_rows + r0 // 2:j * h_rows + r0 // 2 + 8, :] = _pack(term)
        for j in range(TERMS):
            term = _pack_transposed(_unpack(norm_s[j * h_rows:(j + 1) * h_rows, :]))
            t.h[j * w_rows:(j + 1) * w_rows, :] = term
            t.h_all[j * w_rows:(j + 1) * w_rows, :] = term

    def fetch(t):
        for j in range(TERMS):
            t.h[j * w_rows:(j + 1) * w_rows, :] = t.h_all[j * w_rows:(j + 1) * w_rows, :]

    def project(w_s, t, m):
        def product(j):
            r0 = j * w_rows + m * CHUNK // 2
            return pacer.dot(w_s[r0:r0 + CHUNK // 2, :], t.h[j * w_rows:(j + 1) * w_rows, :])

        c11, c12, c21, c22 = _block_matmul(product)
        halves = (jnp.concatenate([c11, c12], axis=1), jnp.concatenate([c21, c22], axis=1))
        return [(side * PAIRS // 2 + m * CHUNK // PAIR + j, block[j * PAIR:(j + 1) * PAIR])
                for side, block in enumerate(halves) for j in range(CHUNK // PAIR)]

    def key_features(p, pk):
        phi = jnp.concatenate(_feature_map(pk), axis=0)
        z_s[p * 128:(p + 1) * 128, :] += phi[:, :HALF] + phi[:, HALF:]
        return phi

    def accumulate_kv(phi, v):
        for phi_p, (p, v_p) in zip(phi, v, strict=True):
            kv_s[p * PAIR:(p + 1) * PAIR, :] += _dot_nt(v_p.astype(BF16), phi_p.astype(BF16))

    def summarize(t, owed, between=lambda: None, flush=False):
        for m in range(n_chunks):
            pk = project(wk_s, t, m)
            if not (flush and m + 1 == n_chunks):
                while owed:
                    accumulate_kv(*owed.pop(0))
            between()
            owed.append(([key_features(*pair) for pair in pk], project(wv_s, t, m)))
            between()
        while flush and owed:
            accumulate_kv(*owed.pop(0))
        return owed

    def early_product(col, i):
        n = (col - KEY) * TERMS + i
        return x1_all.at[pl.ds(n // 4 * hd, hd), pl.ds(n % 4 * TILE, TILE)]

    def early_features(q, b):
        def block(col):
            return _block_matmul(lambda i: early_product(col, i)[q * PAIR:(q + 1) * PAIR, :])[b]

        return b // 2 * PAIRS // 2 + q, block(KEY), block(VALUE)

    def query_features(p, pq):
        phi = _feature_map(pq)
        z = [z_s[p * 128 + 8 * j:p * 128 + 8 * j + 8, :] for j in range(len(phi))]
        den = _head_reduce(
            jnp.add, [f * jnp.concatenate([zj, zj], axis=1) for f, zj in zip(phi, z)])
        inv = _recip(den + DEN_EPS)
        even = lax.broadcasted_iota(I32, inv.shape, 0) % 2 == 0
        other = pltpu.roll(inv, 1, 0)
        per_head = [jnp.where(even, inv, other), jnp.where(even, other, inv)]
        return (p, jnp.concatenate(phi, axis=0).astype(BF16),
                jnp.concatenate([_rows(v, HEAD_DIM) for v in per_head], axis=0))

    def queries(t, m):
        return [query_features(*pair) for pair in project(wq_s, t, m)]

    def read_out(t, m, features):
        o_t = [_dot(_unpack(kvm_s[p * HEAD_DIM:(p + 1) * HEAD_DIM, :]), phi) * inv
               for p, phi, inv in features]
        top = jnp.concatenate(o_t[:len(o_t) // 2], axis=0)
        bottom = jnp.concatenate(o_t[len(o_t) // 2:], axis=0)
        terms = _lhs_terms(top[:, :HALF], bottom[:, :HALF], top[:, HALF:], bottom[:, HALF:])
        for j, term in enumerate(terms):
            t.o[j * h_rows:(j + 1) * h_rows, m * CHUNK:(m + 1) * CHUNK] = _pack_transposed(term)

    def residual(t, g, first=0, count=HALF):
        def product(j):
            return pacer.dot(t.o[j * h_rows + first // 2:j * h_rows + (first + count) // 2, :],
                             wo_s[j * w_rows:(j + 1) * w_rows, g * CHUNK:(g + 1) * CHUNK])

        for b, attn in enumerate(_block_matmul(product)):
            span = (slice(b // 2 * HALF + first, b // 2 * HALF + first + count),
                    slice(b % 2 * hd + g * CHUNK, b % 2 * hd + (g + 1) * CHUNK))
            gate = vec_s[:, GATE_A * d + span[1].start:GATE_A * d + span[1].stop]
            x1 = t.x[span].astype(F32) + _rows(gate, count) * attn
            t.x1[span] = x1
            t.x1_all[span] = x1

    def finish(t, g, after=None):
        x1 = t.x1[16 * g:16 * g + 16, :]
        xc, rstd = _centered(x1, after)
        out = x1 + (xc * rstd * _rows(vec(OUT_SCALE), 16) + _rows(vec(OUT_SHIFT), 16))
        t.out[16 * g:16 * g + 16, :] = out.astype(BF16)
        score = jnp.sum(xc * _rows(vec(SCORE), 16), axis=-1, keepdims=True) * rstd
        lane = lax.broadcasted_iota(I32, (8, 128), 1)
        packed = t.score[...]
        for s in range(2):
            packed = jnp.where(lane == 2 * g + s, score[8 * s:8 * s + 8], packed)
        t.score[...] = packed
        return pacer.token([packed, out[:, -128:]])

    def finishing(t, groups, windows):
        for g, window in zip(groups, windows, strict=True):
            pacer.plan(functools.partial(finish, t, g), window)

    def attend(t, previous, after_first=lambda: None):
        ready = queries(t, 0)
        after_first()
        for m in range(n_chunks - 1):
            ahead = queries(t, m + 1)
            residual(previous, m)
            read_out(t, m, ready)
            ready = ahead
        read_out(t, n_chunks - 1, ready)
        residual(previous, n_chunks - 1)

    def start_up():
        early = (tile(0, 0), tile(0, 1))
        cf = c_v[...].astype(F32)
        act_s[...] = _pack(jnp.broadcast_to(cf * _sigmoid(cf), (16, d)))
        wphi_cp.wait()
        feature_blocks()

        def weight_terms(j):
            for cp in weight_copies(j):
                cp.wait()
            for g in range(n_chunks):
                projection_terms(KEY, j, g)
                projection_terms(VALUE, j, g)

        def activation_terms(j, between=()):
            for cp in mod_a_copies(j):
                cp.wait()
            parts = [slice(part * hd + j * CHUNK, part * hd + (j + 1) * CHUNK) for part in range(4)]
            vectors = []
            between = list(between)
            for n, part in enumerate(parts):
                m = float(n >= 2)
                for span in (slice(0, hd), slice(hd, d)):
                    if between:
                        between.pop(0)()
                    m = m + _dot(_unpack(act_s[:, span]), wmod_v[span, part])[0:8]
                vectors.append(m)
            for part, v in zip(parts, vectors):
                vec_s[:, part] = v
            shifts, scales = vectors[:2], vectors[2:]
            for t in early:
                blocks = (t.x1[r:r + HALF, part] * _rows(scale, HALF) + _rows(shift, HALF)
                          for part, scale, shift in zip(parts, scales, shifts) for r in (0, HALF))
                for i, term in enumerate(_rhs_terms(*blocks)):
                    r0 = i * w_rows + j * CHUNK // 2
                    t.h_all[r0:r0 + CHUNK // 2, :] = _pack_transposed(term)

        x_first_cp.wait()
        for t in early:
            for r0 in range(0, TILE, 16):
                t.x1[r0:r0 + 16, :] = normed_rows(t, r0)
        weight_terms(0)
        activation_terms(0)

        def accumulate(j, i, col, r0=0, n=hd):
            h0 = i * w_rows + j * CHUNK // 2
            h = jnp.concatenate([t.h_all[h0:h0 + CHUNK // 2, :] for t in early], axis=1)
            w = (wk_s if col == KEY else wv_s)[
                i * w_rows + r0 // 2:i * w_rows + (r0 + n) // 2, j * CHUNK:(j + 1) * CHUNK]
            product = _dot(_unpack(w), _unpack(h))
            acc = early_product(col, i)
            acc[r0:r0 + n, :] = product + acc[r0:r0 + n, :] if j else product

        for j in range(n_chunks):
            for i in range(TERMS):
                if i == 2 and j + 1 < n_chunks:
                    weight_terms(j + 1)
                if i == 0 and j + 1 == n_chunks:
                    x_next_cp.wait()
                    normalize(tile(1, 0))
                if i == (4 if j else 5) and j + 1 < n_chunks:
                    activation_terms(j + 1, [functools.partial(accumulate, j, i, col, r0, CHUNK)
                                             for col in (KEY, VALUE) for r0 in range(0, hd, CHUNK)])
                else:
                    accumulate(j, i, KEY)
                    accumulate(j, i, VALUE)
        for cp in (wq_cp, wo_cp, wr_cp):
            cp.start()

    def summarize_pair(i, copies):
        ready = []

        def job(n, end, after):
            p, pk, v = early_features(n // 4, n % 4)
            if after is not None:
                pk = pk + _rows(jnp.concatenate([pltpu.bitcast(after, F32)] * 2, axis=1), PAIR)
            phi = key_features(p, pk)
            ready.append((end, [phi], [(p, v)]))
            return pacer.token([phi[PAIR - 8:PAIR], phi[-8:]])

        def drain():
            while ready and ready[0][0] <= pacer.now:
                accumulate_kv(*ready.pop(0)[1:])

        for n, window in enumerate(EARLY_WINDOWS):
            pacer.plan(functools.partial(
                job, (i - 1) * len(EARLY_WINDOWS) + n, pacer.now + window[1]), window)
        copies[0].start()
        normalize(tile(i, 1))
        owed = summarize(tile(i, 0), [], drain)
        copies[1].start()
        normalize(tile(i + 1, 0))
        summarize(tile(i, 1), owed, drain, flush=True)
        assert not ready

    def summarize_last_pair():
        for cp in (wq_cp, wo_cp, wr_cp, mod_b_cp):
            cp.wait()
        normalize(tile(last, 1))
        for p, window in enumerate(OUTPUT_WINDOWS):
            for c in range(n_chunks):
                pacer.plan(functools.partial(output_terms, p, c), window)
        for j in range(n_chunks):
            for g in range(n_chunks):
                pacer.fillers += [functools.partial(projection_terms, QUERY, j, g),
                                  lambda: None, lambda: None]
        summarize(tile(last, 1), summarize(tile(last, 0), []), flush=True)

    def attend_first_pair():
        row = lax.broadcasted_iota(I32, (PAIR, 128), 0)
        lane = lax.broadcasted_iota(I32, (PAIR, 128), 1)
        for p in range(PAIRS):
            kv = jnp.where(row // HEAD_DIM == lane % 2, kv_s[p * PAIR:(p + 1) * PAIR, :], 0.0)
            kvm_s[p * HEAD_DIM:(p + 1) * HEAD_DIM, :] = _pack(kv)
            z = jnp.sum(z_s[p * 128:(p + 1) * 128, :], axis=1, keepdims=True)
            z_s[p * 128:(p + 1) * 128, :] = jnp.broadcast_to(z, (128, 128))
        for i in (GATE_A, SHIFT_B, SCALE_B, GATE_B):
            pacer.fillers += modulation_rounds(i)
        first = tile(0, 0)
        fetch(first)
        fetch(tile(0, 1))
        ready = queries(first, 0)
        for m in range(n_chunks - 1):
            ahead = queries(first, m + 1)
            read_out(first, m, ready)
            ready = ahead
        fetch(tile(1, 0))
        attend(tile(0, 1), first, lambda: read_out(first, n_chunks - 1, ready))
        derived_vectors()

    def attend_pairs():
        def body(i, carry):
            pacer.reset()
            tiles = [tile(i - 1, 0), tile(i - 1, 1), tile(i, 0), tile(i, 1),
                     tile(jnp.minimum(i + 1, last), 0)]
            for k in range(2):
                fetch(tiles[k + 3])
                finishing(tiles[k], range(TILE // 16), FINISH_WINDOWS)
                attend(tiles[k + 2], tiles[k + 1])
            out_copy(i - 1).start()
            return carry

        lax.fori_loop(1, last + 1, body, 0)

    def finish_last_pair():
        for cp in (wg_cp, wu_cp, wd_cp):
            cp.wait()
        final = tile(last, 1)
        groups = [[(r + k * HALF // 2 + side * HALF) // 16 for side in range(2)
                   for r in range(0, HALF // 2, 16)] for k in range(2)]
        finishing(tile(last, 0), range(TILE // 16), LAST_WINDOWS)
        for g in range(n_chunks):
            residual(final, g, 0, HALF // 2)
        finishing(final, groups[0], TAIL_WINDOWS)
        for g in range(n_chunks):
            residual(final, g, HALF // 2, HALF // 2)
        for g in groups[1]:
            finish(final, g)

    def route():
        scores = score_s[...]
        row = lax.broadcasted_iota(I32, scores.shape, 0)
        lane = lax.broadcasted_iota(I32, scores.shape, 1)
        index = jnp.where(
            lane < TILE // 8, (row // 8) * TILE + lane * 8 + row % 8, seq).astype(F32)

        def everywhere(op, v):
            return op(op(v, axis=0, keepdims=True), axis=1, keepdims=True)

        valid = index < seq
        best = everywhere(jnp.max, jnp.where(valid, scores, -jnp.inf))
        tied = valid & (scores == best)
        below = valid & jnp.logical_not(tied)
        runner_up = everywhere(jnp.max, jnp.where(below, scores, -jnp.inf))
        first = everywhere(jnp.min, jnp.where(tied, index, seq - 1.0))
        second = everywhere(jnp.min, jnp.where(
            tied & (index != first), index,
            jnp.where(below & (scores == runner_up), index + seq, 2 * seq - 1.0)))
        i0, i1 = first.astype(I32)[0, 0], second.astype(I32)[0, 0] % seq

        sub = lax.broadcasted_iota(I32, (16, d), 0)
        x1 = jnp.where(sub == 0, x1_all[pl.ds(i0, 1), :], x1_all[pl.ds(i1, 1), :])
        xc, rstd = _centered(x1)
        h2 = xc * rstd * _rows(vec(SCALE_B), 16) + _rows(vec(SHIFT_B), 16)
        gate = _sigmoid(jnp.sum(h2 * _rows(vec(ROUTER), 16), axis=-1, keepdims=True))
        xs = h2.astype(BF16)
        out_copy(last).start()
        spans = [slice(f, f + FFN_CHUNK) for f in range(0, wd_v.shape[0], FFN_CHUNK)]
        y, hidden = 0.0, None
        for k in range(len(spans) + 1):
            if k < len(spans):
                g, u = _dot(xs, wg_v[:, spans[k]]), _dot(xs, wu_v[:, spans[k]])
            if k > 0:
                y = y + _dot(hidden, wd_v[spans[k - 1], :])
            hidden = (g * _sigmoid(g) * u).astype(BF16)
        routed = x1 + _rows(vec(GATE_B), 16) * (h2 + y * gate)

        for i in range(last + 1):
            out_copy(i).wait()

        def patch(k, i):
            base = pl.multiple_of((i // 16) * 16, 16)
            old = out_v[pl.ds(base, 16), :].astype(F32)
            out_v[pl.ds(base, 16), :] = jnp.where(
                sub == i - base, routed[k:k + 1], old).astype(BF16)
            return base, copy(out_v.at[pl.ds(base, 16)], out_hbm.at[pl.ds(base, 16)],
                              sem.at[24 + k])

        base0, patch0 = patch(0, i0)
        base1, patch1 = patch(1, i1)
        patch0.start()

        @pl.when(base1 != base0)
        def _():
            patch1.start()
            patch1.wait()

        patch0.wait()

    for cp in (c_cp, wphi_cp, x_first_cp):
        cp.start()
    for j in range(n_chunks):
        for cp in weight_copies(j) + mod_a_copies(j):
            cp.start()
    x_next_cp.start()
    x_rest_cp.start()
    kv_s[...] = jnp.zeros(kv_s.shape, F32)
    z_s[...] = jnp.zeros(z_s.shape, F32)
    score_s[...] = jnp.full(score_s.shape, -jnp.inf, F32)
    c_cp.wait()
    words = pltpu.bitcast(jnp.broadcast_to(c_v[:, :128].astype(F32), (8, 128)), I32)
    zero = jnp.minimum(lax.shift_right_logical(words, 1), 0)
    zero_s[...] = zero
    origin = jnp.max(zero)

    def own_block(k, step):
        pacer.reset()
        pl.when(origin <= k)(step)
        pacer.reset()

    start_up()
    x_rest_cp.wait()
    own_block(1, functools.partial(summarize_pair, 1, (mod_b_cp, wg_cp)))
    summarize_pair(2, (wu_cp, wd_cp))
    own_block(2, summarize_last_pair)
    attend_first_pair()
    attend_pairs()
    pacer.reset()
    finish_last_pair()
    route()


@jax.jit
def pallas_adaLN_cond__linear_kernel_hedgehog__moe_arch_mod__prompt_kernel(
    A_x: jax.Array,
    A_wqkv: jax.Array,
    A_w_phi: jax.Array,
    A_wo: jax.Array,
    B_x: jax.Array,
    B_w_r: jax.Array,
    B_w_gate: jax.Array,
    B_w_up: jax.Array,
    B_w_down: jax.Array,
    c: jax.Array,
    w_mod: jax.Array,
):
    del B_x
    batch, seq, d = A_x.shape
    assert batch == 1 and d == HEADS * HEAD_DIM and seq == 8 * TILE
    n_tiles = seq // TILE
    operands = (A_x.reshape(seq, d), A_wqkv, A_w_phi, A_wo, B_w_r, B_w_gate, B_w_up, B_w_down,
                c, w_mod)
    weight_terms = pltpu.VMEM((TERMS * d // 4, d // 2), I32)
    token_terms = pltpu.VMEM((TERMS * HALF // 2, d // 2), I32)
    scratch = [pltpu.VMEM(a.shape, a.dtype) for a in operands] + [
        weight_terms, weight_terms, weight_terms, weight_terms,
        pltpu.VMEM((d // 2, 128), I32),
        pltpu.VMEM((8, d), I32),
        pltpu.VMEM((8, 10 * d), F32),
        token_terms,
        [pltpu.VMEM((TERMS * d // 4, HALF), I32)] * 2,
        pltpu.VMEM((n_tiles * TERMS * d // 4, HALF), I32),
        [token_terms] * 2,
        [pltpu.VMEM((TILE, d), F32)] * 2,
        pltpu.VMEM((seq, d), F32),
        pltpu.VMEM((PAIRS * PAIR, 128), F32),
        pltpu.VMEM((PAIRS * HEAD_DIM, 128), I32),
        pltpu.VMEM((PAIRS * 128, 128), F32),
        pltpu.VMEM((n_tiles * 8, 128), F32),
        pltpu.VMEM((8, 128), I32),
        pltpu.VMEM((seq, d), A_x.dtype),
        pltpu.SemaphoreType.DMA((26,)),
    ]
    out = pl.pallas_call(
        _kernel,
        out_shape=jax.ShapeDtypeStruct((seq, d), A_x.dtype),
        in_specs=[pl.BlockSpec(memory_space=pl.ANY)] * len(operands),
        out_specs=pl.BlockSpec(memory_space=pl.ANY),
        scratch_shapes=scratch,
        compiler_params=pltpu.CompilerParams(
            vmem_limit_bytes=110 * 2**20,
            flags={"XLA_TPU_EVENLY_DISTRIBUTE_CRITICAL_NODES": True}),
        name="adaln_hedgehog_mod",
    )(*operands)
    return out.reshape(batch, seq, d)
```
